```python
import jax
import jax.numpy as jnp

def _softmax(x, axis=-1):
    return jax.nn.softmax(x, axis=axis)

def _gelu(x):
    return jax.nn.gelu(x, approximate=True)

def _silu(x):
    return jax.nn.silu(x)

def _sigmoid(x):
    return jax.nn.sigmoid(x)

def _layernorm(x, axis=-1, eps=1e-05):
    m = jnp.mean(x, axis=axis, keepdims=True)
    v = jnp.var(x, axis=axis, keepdims=True)
    return (x - m) / jnp.sqrt(v + eps)

def _scatter_add(tgt, idx, src, axis=0):
    return tgt.at[idx].add(src)

def _segment_sum(src, seg, n):
    return jax.ops.segment_sum(src, seg, n)

class _Rng:

    def __init__(self, key):
        self._k = key

    def _next(self):
        self._k, sub = jax.random.split(self._k)
        return sub

    def normal(self, shape):
        return jax.random.normal(self._next(), shape, dtype=jnp.bfloat16)

    def randint(self, lo, hi, shape):
        return jax.random.randint(self._next(), shape, lo, hi, dtype=jnp.int32)

    def uniform(self, shape, lo=0.0, hi=1.0):
        return jax.random.uniform(self._next(), shape, jnp.bfloat16, lo, hi)

    def permutation(self, n):
        return jax.random.permutation(self._next(), n)
kernel_name = 'standalone__conformer_family_branchformer__speech'

def setup_inputs():
    _rng = _Rng(jax.random.key(int.from_bytes(__import__("os").urandom(4), "little")))
    _w = lambda a: (lambda t: t.astype(jnp.bfloat16) if jnp.issubdtype(t.dtype, jnp.floating) else t)(jnp.asarray(a))
    B, T, D, K = (2, 4000, 512, 31)
    s = float(D) ** (-0.5)
    return {'x': _w((lambda *s: _rng.normal(s) * 0.05)(B, T, D)), 'w_q': _w((lambda *s: _rng.normal(s) * 0.05)(D, D) * s), 'w_k': _w((lambda *s: _rng.normal(s) * 0.05)(D, D) * s), 'w_v': _w((lambda *s: _rng.normal(s) * 0.05)(D, D) * s), 'w_ao': _w((lambda *s: _rng.normal(s) * 0.05)(D, D) * s), 'w_up': _w((lambda *s: _rng.normal(s) * 0.05)(D, 2 * D) * s), 'dw': _w((lambda *s: _rng.normal(s) * 0.05)(K, D) * (1.0 / K)), 'w_dn': _w((lambda *s: _rng.normal(s) * 0.05)(D, D) * s), 'w_merge': _w((lambda *s: _rng.normal(s) * 0.05)(2 * D, D) * s)}

def reference(x, w_q, w_k, w_v, w_ao, w_up, dw, w_dn, w_merge):
    B, T, D = x.shape
    K = dw.shape[0]
    xa = _layernorm(x, axis=-1)
    q = jnp.einsum('btd,de->bte', xa, w_q)
    k = jnp.einsum('btd,de->bte', xa, w_k)
    v = jnp.einsum('btd,de->bte', xa, w_v)
    logits = jnp.einsum('btd,bsd->bts', q, k) * float(D) ** (-0.5)
    attn = _softmax(logits, axis=-1)
    ya = jnp.einsum('bts,bsd->btd', attn, v)
    ya = jnp.einsum('btd,de->bte', ya, w_ao)
    xc = _layernorm(x, axis=-1)
    h = _gelu(jnp.einsum('btd,de->bte', xc, w_up))
    u = h[..., :D].copy()
    g = _layernorm(h[..., D:], axis=-1)
    pad = K // 2
    gp = jnp.pad(g, ((0, 0), (pad, pad), (0, 0)))
    conv = jnp.zeros_like(g)
    for i in range(K):
        conv = conv + gp[:, i:i + T, :] * dw[i][None, None, :]
    yc = jnp.einsum('btd,de->bte', u * conv, w_dn)
    merged = jnp.concatenate([ya, yc], axis=-1)
    out = jnp.einsum('btf,fd->btd', merged, w_merge)
    return x + out
```

```python
import functools
import jax
import jax.numpy as jnp
import numpy as np
from jax import lax
import jax.experimental.pallas as pl
import jax.experimental.pallas.tpu as pltpu

LOG2E = 1.4426950408889634
NT = (((1,), (1,)), ((), ()))
NN = (((1,), (0,)), ((), ()))
bf = jnp.bfloat16
f32 = jnp.float32
HALO = 16
PERM = (0, 2, 6, 5, 3, 4, 1)


def _ln(x, eps=1e-5):
    m = jnp.mean(x, axis=-1, keepdims=True)
    d = x - m
    v = jnp.mean(d * d, axis=-1, keepdims=True)
    return d * lax.rsqrt(v + eps)


def _gelu(x):
    c = float(np.sqrt(2.0 / np.pi))
    return 0.5 * x * (1.0 + jnp.tanh(c * (x + 0.044715 * (x * x * x))))


def _dot(a, b, dims=NN):
    return lax.dot_general(a, b, dims, preferred_element_type=f32)


def rows(*p):
    return jnp.concatenate(p, axis=0)


def cols(*p):
    return jnp.concatenate(p, axis=1)


def alpha(z):
    (a, b), (c, d) = z
    return [a + d, c + d, a, d, a + b, c - a, b - d]


def beta(z):
    t = alpha(z)
    return [t[k] for k in PERM]


def gamma(n):
    return [[n[0] + n[3] - n[4] + n[6], n[2] + n[4]], [n[1] + n[3], n[0] - n[1] + n[2] + n[5]]]


def tr(z):
    return [list(r) for r in zip(*z)]


def lvl1(g):
    return [[rows(*[cols(g[2 * r1 + r2][2 * c1], g[2 * r1 + r2][2 * c1 + 1]) for r2 in range(2)])
             for c1 in range(2)] for r1 in range(2)]


def unlvl1(z):
    out = [[None] * 4 for _ in range(4)]
    for r1 in range(2):
        for c1 in range(2):
            v = z[r1][c1]
            n, m = v.shape[0] // 2, v.shape[1] // 2
            for r2 in range(2):
                for c2 in range(2):
                    out[2 * r1 + r2][2 * c1 + c2] = v[r2 * n:(r2 + 1) * n, c2 * m:(c2 + 1) * m]
    return out


def two(f, g):
    l1 = [[f([[g[2 * r1 + r2][2 * c1 + c2] for c1 in range(2)] for r1 in range(2)])
           for c2 in range(2)] for r2 in range(2)]
    return [f([[l1[r2][c2][a] for c2 in range(2)] for r2 in range(2)]) for a in range(7)]


def gamma2(n):
    inner = [gamma(n[a]) for a in range(7)]
    out = [[None] * 4 for _ in range(4)]
    for r2 in range(2):
        for c2 in range(2):
            z = gamma([inner[a][r2][c2] for a in range(7)])
            for r1 in range(2):
                for c1 in range(2):
                    out[2 * r1 + r2][2 * c1 + c2] = z[r1][c1]
    return out


def grid4(w):
    n, m = w.shape[0] // 4, w.shape[1] // 4
    return [[w[i * n:(i + 1) * n, j * m:(j + 1) * m] for j in range(4)] for i in range(4)]


def make(H=144, LQ=1, LV=1, LP=1, LF=1, C=256, CV=256, CR=72, NXC=5, FLAGS=None,
         QS=2, GJ=(0, 0, 1, 1), UJ=1, WQ=1.0, TIE=True):
    def kern(x_hbm, wq_hbm, wk_hbm, wv_hbm, wao_hbm, wup_hbm, dw_hbm, wdn_hbm, wm_hbm,
             o_hbm,
             x_v, wq, wk, wv, wao, wup, dwv, wdn, wm,
             wp_s, wf_s, xa_s, x1_s, x2_s, g_s, dw_s, ob_s,
             wsem, xsem, osem, *, B, T, D, K, NP):
        TQ = T // 4
        NL = D // 128
        pad = K // 2
        nb = -(-TQ // H)
        RX = TQ // NXC
        use0 = LP == 0
        use1 = 1 in (LQ, LV, LP)
        use2 = 2 in (LQ, LV, LP)

        wc = {n: pltpu.make_async_copy(s, d, wsem.at[k]) for k, (n, s, d) in enumerate(
            [("v", wv_hbm, wv), ("ao", wao_hbm, wao), ("m", wm_hbm, wm), ("dn", wdn_hbm, wdn),
             ("q", wq_hbm, wq), ("k", wk_hbm, wk), ("up", wup_hbm, wup), ("dw", dw_hbm, dwv)])}

        def xcopy(b, h, c):
            return pltpu.make_async_copy(x_hbm.at[b, pl.ds(h * TQ + c * RX, RX), :],
                                         x_v.at[b, pl.ds(h * TQ + c * RX, RX), :],
                                         xsem.at[h * NXC + c])

        def xrest(b):
            return pltpu.make_async_copy(x_hbm.at[b], x_v.at[b], xsem.at[4 * NXC + b - 1])

        def ln_rows(b, slot, r, n):
            xs = [_ln(x_v[b, pl.ds(h * TQ + r, n), :].astype(f32)) for h in range(4)]
            g = [[v[:, c * 128:(c + 1) * 128] for c in range(4)] for v in xs]
            if use0:
                for h in range(4):
                    xa_s[slot, h, pl.ds(r, n), :] = xs[h].astype(bf)
            l1 = [[alpha([[g[2 * r1 + r2][2 * c1 + c2] for c1 in range(2)] for r1 in range(2)])
                   for c2 in range(2)] for r2 in range(2)]
            for a in range(7):
                if use1:
                    for r2 in range(2):
                        x1_s[slot, 2 * a + r2, pl.ds(r, n), :] = cols(l1[r2][0][a], l1[r2][1][a]).astype(bf)
                if use2:
                    for k, v in enumerate(alpha([[l1[r2][c2][a] for c2 in range(2)] for r2 in range(2)])):
                        x2_s[slot, 7 * a + k, pl.ds(r, n), :] = v.astype(bf)
            return [v[:, :128] for v in xs]

        def set_proj(n, w):
            if LP == 0:
                wp_s[n] = w.astype(bf)
            elif LP == 1:
                for k, v in enumerate(beta(lvl1(grid4(w)))):
                    wp_s[n, k] = v.astype(bf)
            else:
                for a, row in enumerate(two(beta, grid4(w))):
                    for k, v in enumerate(row):
                        wp_s[n, 7 * a + k] = v.astype(bf)

        def set_fin(n, w):
            if LF == 0:
                wf_s[n * D:(n + 1) * D, :] = w.astype(bf)
            else:
                for k, v in enumerate(beta(lvl1(grid4(w)))):
                    wf_s[k, n * (D // 2):(n + 1) * (D // 2), :] = v.astype(bf)

        wc["v"].start(); wc["ao"].start()
        wc["m"].start(); wc["dn"].start()
        for slot in range(2):
            if use0:
                for h in range(4):
                    xa_s[slot, h, TQ:NP, :] = jnp.zeros((NP - TQ, D), bf)
            if use1:
                for k in range(14):
                    x1_s[slot, k, TQ:NP, :] = jnp.zeros((NP - TQ, D // 2), bf)
            if use2:
                for k in range(49):
                    x2_s[slot, k, TQ:NP, :] = jnp.zeros((NP - TQ, D // 4), bf)
        for c in range(NL):
            g_s[0, c, 0:HALO, :] = jnp.zeros((HALO, 128), f32)
            g_s[3, c, HALO + TQ:2 * HALO + TQ, :] = jnp.zeros((HALO, 128), f32)
            dw_s[c] = jnp.zeros((32, 128), f32)
        wc["v"].wait(); wc["ao"].wait()
        wc["q"].start(); wc["k"].start()
        t = _dot(wv[...], wao[...]).astype(bf)
        wc["m"].wait(); wc["dn"].wait()
        wc["up"].start(); wc["dw"].start()
        for h in range(4):
            xcopy(0, h, 0).start()
        set_fin(0, _dot(t, wm[0:D, :]))
        set_fin(1, _dot(wdn[...], wm[D:2 * D, :]))
        wc["q"].wait(); wc["k"].wait()
        for c in range(1, min(3, NXC)):
            for h in range(4):
                xcopy(0, h, c).start()
        set_proj(0, _dot(wq[...], wk[...], NT) * (LOG2E * D ** -0.5))
        wc["up"].wait(); wc["dw"].wait()
        set_proj(1, wup[:, 0:D].astype(f32))
        set_proj(2, wup[:, D:2 * D].astype(f32))
        for c in range(NL):
            dw_s[c, 0:K, :] = dwv[:, c * 128:(c + 1) * 128].astype(f32)

        def ln_body(c, _):
            @pl.when(c + 3 < NXC)
            def _():
                for h in range(4):
                    xcopy(0, h, c + 3).start()
            for h in range(4):
                xcopy(0, h, c).wait()
            ln_rows(0, 0, pl.multiple_of(c * RX, 8), RX)
            return 0
        with jax.named_scope("ln0"):
            lax.fori_loop(0, NXC, ln_body, 0)
        for b in range(1, B):
            xrest(b).start()

        def ocopy(b, r, h):
            return pltpu.make_async_copy(ob_s.at[h], o_hbm.at[b, pl.ds(h * TQ + r, H), :], osem.at[h])

        @jax.named_scope("step")
        def step(it, _):
            b = it // nb
            i = it % nb
            slot = b % 2
            r = pl.multiple_of(jnp.minimum(i * H, TQ - H), 8)
            never = it < 0

            def tie(a, tok, row=0):
                if not TIE:
                    return a
                n = tok.shape[0]
                parts = [jnp.where(never, tok.astype(a.dtype), a[row:row + n, :128])]
                if row:
                    parts.insert(0, a[:row, :128])
                if row + n < a.shape[0]:
                    parts.append(a[row + n:, :128])
                head = rows(*parts) if len(parts) > 1 else parts[0]
                return cols(head, a[:, 128:]) if a.shape[1] > 128 else head

            def tie_many(ops, ks, toks):
                for n, tk in enumerate(toks):
                    k = ks[n % len(ks)]
                    ops[k] = tie(ops[k], tk)

            @pl.when(i == 0)
            def _():
                xe = rows(*[x_v[b, pl.ds(h * TQ + o, HALO), :] for h in range(4) for o in (0, TQ - HALO)])
                ge = _ln(_gelu(_dot(_ln(xe.astype(f32)).astype(bf), wup[:, D:2 * D])))
                for h in range(4):
                    for c in range(NL):
                        sl = slice(c * 128, (c + 1) * 128)
                        g_s[h, c, HALO:2 * HALO, :] = ge[2 * h * HALO:(2 * h + 1) * HALO, sl]
                        if h < 3:
                            g_s[h + 1, c, 0:HALO, :] = ge[(2 * h + 1) * HALO:(2 * h + 2) * HALO, sl]

            def proj(n, r0, tok=None):
                first = (lambda v: tie(v, tok)) if tok is not None else (lambda v: v)
                if LP == 0:
                    ys = [_dot(first(xa_s[slot, h, pl.ds(r0, H), :]), wp_s[n]) for h in range(4)]
                    return [[y[:, c * 128:(c + 1) * 128] for c in range(4)] for y in ys]
                if LP == 1:
                    return unlvl1(gamma([_dot(first(rows(x1_s[slot, 2 * k, pl.ds(r0, H), :],
                                                         x1_s[slot, 2 * k + 1, pl.ds(r0, H), :])), wp_s[n, k])
                                         for k in range(7)]))
                return gamma2([[_dot(first(x2_s[slot, 7 * a + k, pl.ds(r0, H), :]), wp_s[n, 7 * a + k])
                                for k in range(7)] for a in range(7)])

            gpre = proj(2, r + HALO)
            q = proj(0, r)
            if LQ == 1:
                qc = [v.astype(bf) for v in beta(tr(lvl1(q)))]
            else:
                qc = [v.astype(bf) for row in two(beta, tr(q)) for v in row]
            gtok = []
            for h in range(4):
                gg = _ln(_gelu(cols(*gpre[h])))
                for c in range(NL):
                    g_s[h, c, pl.ds(r + 2 * HALO, H), :] = gg[:, c * 128:(c + 1) * 128]
                gtok.append(gg[:, :128])
            for h in range(3):
                for c in range(NL):
                    g_s[h, c, HALO + TQ:2 * HALO + TQ, :] = g_s[h + 1, c, HALO:2 * HALO, :]

            qch = [(r2, j) for j in range(NP // C) for r2 in range(2)] if LQ == 1 else [(None, j) for j in range(NP // C)]
            vch = [(r2, j) for j in range(NP // CV) for r2 in range(2)] if LV == 1 else [(None, j) for j in range(NP // CV)]
            nk, nv = len(qch), len(vch)
            pieces = [(h, c, rr) for h in range(4) for c in range(NL) for rr in range(0, H, CR)]
            wts = [0.0] * QS + [WQ / nk] * (nk - QS) + [1.0 / nv] * nv
            edges = np.cumsum(wts) / sum(wts) * len(pieces)
            sched = [[] for _ in range(nk + nv)]
            for n, p in enumerate(pieces):
                sched[int(np.searchsorted(edges, n + 0.5))].append(p)
            cv = {}

            def conv_piece(h, c, rr):
                w = dw_s[c]
                acc = None
                for tt in range(K):
                    term = g_s[h, c, pl.ds(r + (rr + HALO - pad + tt), CR), :] * w[tt:tt + 1, :]
                    acc = term if acc is None else acc + term
                cv[h, c, rr] = acc
                return acc

            def conv_toks(s):
                ts = [conv_piece(*p) for p in sched[s]]
                k = H // CR
                return [rows(*ts[n:n + k]) for n in range(0, len(ts), k)]

            S = [[[None] * (NP // 128) for _ in range(4)] for _ in range(4)]
            m = [None] * 4
            l = [None] * 4
            ctoks = []
            last = None
            for jj, (r2, j) in enumerate(qch):
                ks = slice(j * C, (j + 1) * C)
                qq = list(qc)
                n_ops = len(qq)
                tie_many(qq, (2, 3) if LQ == 1 else (21, 22, 23, 24), [gtok[h] for h in range(4) if GJ[h] == jj])
                if jj > 0:
                    if LQ == 1:
                        tie_many(qq, (5, 6), [rows(l[0], l[1]), rows(l[2], l[3])])
                    else:
                        tie_many(qq, (35, 36, 37, 38), l)
                tie_many(qq, (4,) if LQ == 1 else tuple(range(28, 35)), ctoks)
                new = [[] for _ in range(4)]
                if LQ == 1:
                    mm = [_dot(qq[k], x1_s[slot, 2 * k + r2, ks, :], NT) for k in range(7)]
                    last = mm[4][:H, :128]
                    z = tr(gamma(mm))
                    blocks = [(2 * r1 + a, 2 * c1 + r2, z[r1][c1][a * H:(a + 1) * H])
                              for r1 in range(2) for c1 in range(2) for a in range(2)]
                else:
                    mm = [[_dot(qq[7 * a + k], x2_s[slot, 7 * a + k, ks, :], NT) for k in range(7)] for a in range(7)]
                    last = mm[4][4][:, :128]
                    z = tr(gamma2(mm))
                    blocks = [(h, n, z[h][n]) for h in range(4) for n in range(4)]
                for h, n, v in blocks:
                    for t_ in range(C // 128):
                        tl = v[:, t_ * 128:(t_ + 1) * 128]
                        c0 = j * C + t_ * 128
                        if c0 + 128 > TQ:
                            tl = jnp.where(c0 + lax.broadcasted_iota(jnp.int32, (H, 128), 1) < TQ, tl, -jnp.inf)
                        S[h][n][c0 // 128] = tl
                        new[h].append(tl)
                ctoks = conv_toks(jj)
                for h in range(4):
                    mx = functools.reduce(jnp.maximum, new[h])
                    if m[h] is None:
                        mn, ln_ = mx, None
                    else:
                        mn = jnp.maximum(m[h], mx)
                        ln_ = l[h] * jnp.exp2(m[h] - mn)
                    for tl in new[h]:
                        e = jnp.exp2(tl - mn)
                        ln_ = e if ln_ is None else ln_ + e
                    m[h], l[h] = mn, ln_
            upre = proj(1, r, last)
            sh = []
            for h in range(4):
                mr = jnp.max(m[h], axis=-1, keepdims=True)
                lr = jnp.sum(l[h] * jnp.exp2(m[h] - mr), axis=-1, keepdims=True)
                sh.append(mr + jnp.log2(lr))

            acc = [None] * (7 if LV == 1 else 49)
            for jj, (r2, j) in enumerate(vch):
                ks = slice(j * CV, (j + 1) * CV)
                tt_ = range(j * CV // 128, (j + 1) * CV // 128)
                pe = lambda h, n: jnp.exp2(cols(*[S[h][n][t_] for t_ in tt_]) - sh[h])
                if LV == 1:
                    pc = [v.astype(bf) for v in alpha([[rows(pe(2 * r1, 2 * c1 + r2), pe(2 * r1 + 1, 2 * c1 + r2))
                                                        for c1 in range(2)] for r1 in range(2)])]
                    rhs = [x1_s[slot, 2 * PERM[k] + r2, ks, :] for k in range(7)]
                else:
                    pc = [v.astype(bf) for row in two(alpha, [[pe(h, n) for n in range(4)] for h in range(4)]) for v in row]
                    rhs = [x2_s[slot, 7 * PERM[a] + PERM[k], ks, :] for a in range(7) for k in range(7)]
                tie_many(pc, (6, 5) if LV == 1 else tuple(range(42, 49)), ctoks)
                if jj == UJ:
                    u = [[_gelu(upre[h][c]) for c in range(4)] for h in range(4)]
                    if LV == 1:
                        tie_many(pc, (1, 2, 3, 4), [rows(u[2 * a][c], u[2 * a + 1][c]) for a in range(2) for c in range(4)])
                    else:
                        tie_many(pc, tuple(range(24, 40)), [v for row in u for v in row])
                for k in range(len(acc)):
                    d = _dot(pc[k], rhs[k])
                    acc[k] = d if acc[k] is None else acc[k] + d
                ctoks = conv_toks(nk + jj)
            if LV == 1:
                o = unlvl1(gamma(acc))
            else:
                o = gamma2([acc[7 * a:7 * a + 7] for a in range(7)])

            @pl.when(it > 0)
            def _():
                for h in range(4):
                    ocopy(0, 0, h).wait()

            @pl.when(it == 0)
            def _():
                for bb in range(1, B):
                    xrest(bb).wait()
            ltok = ln_rows(jnp.minimum(b + 1, B - 1), 1 - slot, r, H)
            uc = [[u[h][c] * rows(*[cv[h, c, rr] for rr in range(0, H, CR)]) for c in range(4)] for h in range(4)]
            if LF == 0:
                out = [_dot(cols(*o[h]).astype(bf), wf_s[0:D, :])
                       + _dot(tie(cols(*uc[h]).astype(bf), ltok[h]), wf_s[D:2 * D, :]) for h in range(4)]
            else:
                ops = [cols(a.astype(bf), c.astype(bf)) for a, c in zip(alpha(lvl1(o)), alpha(lvl1(uc)))]
                tie_many(ops, (3, 4, 5, 6), ltok)
                out = [cols(*row) for row in unlvl1(gamma([_dot(ops[k], wf_s[k]) for k in range(7)]))]
            for h in range(4):
                ob_s[h] = (x_v[b, pl.ds(h * TQ + r, H), :].astype(f32) + out[h]).astype(ob_s.dtype)
            for h in range(4):
                ocopy(b, r, h).start()
            return 0

        lax.fori_loop(0, B * nb, step, 0)
        for h in range(4):
            ocopy(0, 0, h).wait()

    @jax.jit
    def fn(x, w_q, w_k, w_v, w_ao, w_up, dw, w_dn, w_merge):
        B, T, D = x.shape
        K = dw.shape[0]
        TQ = T // 4
        NP = -(-(TQ + HALO) // max(C, CV)) * max(C, CV)
        ws = (w_q, w_k, w_v, w_ao, w_up, dw, w_dn, w_merge)
        anyspec = pl.BlockSpec(memory_space=pl.ANY)
        tiny = (1, 1, 16, 128)
        return pl.pallas_call(
            functools.partial(kern, B=B, T=T, D=D, K=K, NP=NP),
            in_specs=[anyspec] * 9,
            out_specs=anyspec,
            out_shape=jax.ShapeDtypeStruct(x.shape, x.dtype),
            scratch_shapes=[pltpu.VMEM(x.shape, x.dtype)] + [pltpu.VMEM(w.shape, w.dtype) for w in ws] + [
                pltpu.VMEM([(3, D, D), (3, 7, D // 2, D // 2), (3, 49, D // 4, D // 4)][LP], bf),
                pltpu.VMEM([(2 * D, D), (7, D, D // 2)][LF], bf),
                pltpu.VMEM((2, 4, NP, D) if LP == 0 else tiny, bf),
                pltpu.VMEM((2, 14, NP, D // 2) if 1 in (LQ, LV, LP) else tiny, bf),
                pltpu.VMEM((2, 49, NP, D // 4) if 2 in (LQ, LV, LP) else tiny, bf),
                pltpu.VMEM((4, D // 128, TQ + 2 * HALO, 128), f32),
                pltpu.VMEM((D // 128, 32, 128), f32),
                pltpu.VMEM((4, H, D), x.dtype),
                pltpu.SemaphoreType.DMA((8,)),
                pltpu.SemaphoreType.DMA((4 * NXC + B - 1,)),
                pltpu.SemaphoreType.DMA((4,)),
            ],
            compiler_params=pltpu.CompilerParams(vmem_limit_bytes=112 * 1024 * 1024, flags=FLAGS),
        )(x, *ws)
    return fn


_impl = make(LV=2, CV=512, UJ=0)


def pallas_standalone__conformer_family_branchformer__speech_kernel(x, w_q, w_k, w_v, w_ao, w_up, dw, w_dn, w_merge):
    return _impl(x, w_q, w_k, w_v, w_ao, w_up, dw, w_dn, w_merge)
```

```python
import functools
import jax
import jax.numpy as jnp
import numpy as np
from jax import lax
import jax.experimental.pallas as pl
import jax.experimental.pallas.tpu as pltpu

LOG2E = 1.4426950408889634
NT = (((1,), (1,)), ((), ()))
NN = (((1,), (0,)), ((), ()))
bf = jnp.bfloat16
f32 = jnp.float32
i32 = jnp.int32
HALO = 16
PERM = (0, 2, 6, 5, 3, 4, 1)


def _ln(x, eps=1e-5):
    m = jnp.mean(x, axis=-1, keepdims=True)
    d = x - m
    v = jnp.mean(d * d, axis=-1, keepdims=True)
    return d * lax.rsqrt(v + eps)


def _gelu2(x):
    c = float(np.sqrt(2.0 / np.pi))
    return x * jnp.tanh((x * x * (0.044715 * c) + c) * x) + x


def _dot(a, b, dims=NN):
    return lax.dot_general(a, b, dims, preferred_element_type=f32)


def rows(*p):
    return jnp.concatenate(p, axis=0)


def cols(*p):
    return jnp.concatenate(p, axis=1)


def pk(v):
    return pltpu.bitcast(v.astype(bf), i32)


def up(v):
    return pltpu.bitcast(v, bf)


def alpha(z):
    (a, b), (c, d) = z
    return [a + d, c + d, a, d, a + b, c - a, b - d]


def alpha_one(k, z):
    return [lambda: z(0, 0) + z(1, 1), lambda: z(1, 0) + z(1, 1), lambda: z(0, 0), lambda: z(1, 1),
            lambda: z(0, 0) + z(0, 1), lambda: z(1, 0) - z(0, 0), lambda: z(0, 1) - z(1, 1)][k]()


def beta(z):
    t = alpha(z)
    return [t[k] for k in PERM]


def gamma(n):
    return [[n[0] + n[3] - n[4] + n[6], n[2] + n[4]], [n[1] + n[3], n[0] - n[1] + n[2] + n[5]]]


def tr(z):
    return [list(r) for r in zip(*z)]


def lvl1(g):
    return [[rows(*[cols(g[2 * r1 + r2][2 * c1], g[2 * r1 + r2][2 * c1 + 1]) for r2 in range(2)])
             for c1 in range(2)] for r1 in range(2)]


def unlvl1(z):
    out = [[None] * 4 for _ in range(4)]
    for r1 in range(2):
        for c1 in range(2):
            v = z[r1][c1]
            n, m = v.shape[0] // 2, v.shape[1] // 2
            for r2 in range(2):
                for c2 in range(2):
                    out[2 * r1 + r2][2 * c1 + c2] = v[r2 * n:(r2 + 1) * n, c2 * m:(c2 + 1) * m]
    return out


def two(f, g):
    l1 = [[f([[g[2 * r1 + r2][2 * c1 + c2] for c1 in range(2)] for r1 in range(2)])
           for c2 in range(2)] for r2 in range(2)]
    return [f([[l1[r2][c2][a] for c2 in range(2)] for r2 in range(2)]) for a in range(7)]


def alpha2_direct(g):
    terms = [[(0, 0, 1), (1, 1, 1)], [(1, 0, 1), (1, 1, 1)], [(0, 0, 1)], [(1, 1, 1)],
             [(0, 0, 1), (0, 1, 1)], [(1, 0, 1), (0, 0, -1)], [(0, 1, 1), (1, 1, -1)]]

    def pair(u, v):
        (x, sx), (y, sy) = u, v
        if sx > 0:
            return (x + y if sy > 0 else x - y), 1
        return (y - x, 1) if sy > 0 else (x + y, -1)

    out = []
    for a in range(7):
        for k in range(7):
            t = [[(g[2 * r1 + r2][2 * c1 + c2], s1 * s2) for r2, c2, s2 in terms[k]] for r1, c1, s1 in terms[a]]
            if len(t) == 2 and len(t[0]) == 2:
                v, sign = pair(pair(t[0][0], t[1][1]), pair(t[0][1], t[1][0]))
            else:
                f = [e for row in t for e in row]
                v, sign = pair(*f) if len(f) == 2 else f[0]
            assert sign > 0
            out.append(v)
    return out


def gamma2(n):
    inner = [gamma(n[a]) for a in range(7)]
    out = [[None] * 4 for _ in range(4)]
    for r2 in range(2):
        for c2 in range(2):
            z = gamma([inner[a][r2][c2] for a in range(7)])
            for r1 in range(2):
                for c1 in range(2):
                    out[2 * r1 + r2][2 * c1 + c2] = z[r1][c1]
    return out


def toks(a):
    return [a[k:k + 8, :128] for k in range(0, a.shape[0], 8)]


def take(q, n):
    out = q[:n]
    del q[:n]
    return out


def spread(q, n):
    q0 = list(q)
    del q[:]
    return [q0[k * len(q0) // n:(k + 1) * len(q0) // n] for k in range(n)]


def tie(never, a, ts):
    if not ts:
        return a
    nr, nc = a.shape[0] // 8, a.shape[1] // 128
    cells = {}
    for j, t in enumerate(ts):
        p = j * nr * nc // len(ts)
        cells[p] = jnp.maximum(cells[p], t) if p in cells else t
    out = []
    for p in range(nr):
        row = []
        for c in range(nc):
            v = a[8 * p:8 * p + 8, 128 * c:128 * c + 128]
            t = cells.get(p * nc + c)
            if t is not None:
                v = jnp.where(never, t if t.dtype == a.dtype else pltpu.bitcast(t, a.dtype), v)
            row.append(v)
        out.append(cols(*row))
    return rows(*out)


def quad(w):
    n, m = w.shape[0] // 2, w.shape[1] // 2
    return [[w[i * n:(i + 1) * n, j * m:(j + 1) * m] for j in range(2)] for i in range(2)]


DEFAULTS = {
    1: dict(VCH=(2, 2, 2, 2), CR=72, T2=True, SK=3, CQ=(1, 2), U0=1, UK=3, UG=2,
            PA=(5, 6), PW=(2, 7), CJ=(0, 0, 3, 3, 3, 3, 2, 2), CW=(0, 2), US=0, USK=4, UJ=1, UW=(0, 7), YM=False),
    2: dict(VCH=(2, 2, 4), CR=72, T2=True, SK=3, CQ=(1, 1, 2), U0=1, UK=3, UG=2,
            PA=(5, 6), PW=(3, 7), CJ=(0, 2, 6), CW=(0, 3), US=0, USK=4, UJ=1, UW=(0, 7), YM=True),
}


def make(H=144, C=256, LV=2, FLAGS=None, FO=(1, 3, 6, 0, 2, 4, 5), STG=True, LR=16, L0=0, LE=9, L1=48, GR=16, G0=1, GE=7, **kw):
    cfg = dict(DEFAULTS[LV], **kw)
    VCH, CR, T2, SK, CQ, U0, UK, UG = (cfg[k] for k in "VCH CR T2 SK CQ U0 UK UG".split())
    PA, PW, CJ, CW, US, USK, UJ, UW, YM = (cfg[k] for k in "PA PW CJ CW US USK UJ UW YM".split())
    NX = 32
    def kern(x_hbm, wq_hbm, wk_hbm, wv_hbm, wao_hbm, wup_hbm, dw_hbm, wdn_hbm, wm_hbm,
             o_hbm,
             x_v, wq, wk, wup, dwv, wa, wb,
             wp_s, wf_s, x_s, qc_s, g_s, dw_s, ob_s,
             wsem, xsem, osem, *, B, TQ, D, K, NP):
        NL = D // 128
        pad = K // 2
        nb = -(-TQ // H)
        HL = TQ - (nb - 1) * H
        H2 = H // 2

        wc = {n: pltpu.make_async_copy(s, d, wsem.at[k]) for k, (n, s, d) in enumerate(
            [("v", wv_hbm, wa.at[0]), ("ao", wao_hbm, wb.at[0]), ("m0", wm_hbm.at[0:D], wb.at[1]),
             ("dn", wdn_hbm, wa.at[2]), ("m1", wm_hbm.at[D:2 * D], wb.at[2]),
             ("q", wq_hbm, wq), ("k", wk_hbm, wk), ("up", wup_hbm, wup), ("dw", dw_hbm, dwv)])}
        cuts = [0, 2 * H, 4 * H, 6 * H, TQ]
        xc = [pltpu.make_async_copy(x_hbm.at[0, :, pl.ds(a, e - a), :], x_v.at[0, :, pl.ds(a, e - a), :], xsem.at[n])
              for n, (a, e) in enumerate(zip(cuts[:-1], cuts[1:]))]
        xrest = pltpu.make_async_copy(x_hbm.at[pl.ds(1, B - 1)], x_v.at[pl.ds(1, B - 1), :, pl.ds(0, TQ), :],
                                      xsem.at[len(xc)])

        def ln_part(b, r, n):
            r = pl.multiple_of(r, 16)
            dst = pl.ds(pl.multiple_of(r // 2, 8), n // 2)
            tmp = pl.ds(pl.multiple_of(jnp.minimum(r, 0), 8), n)
            xs = [_ln(x_v[b, h, pl.ds(r, n), :].astype(f32)) for h in range(4)]
            if STG:
                for h in range(4):
                    for c in range(2):
                        x_s[NX + 2 * h + c, tmp, :] = pltpu.bitcast(xs[h][:, c * 256:(c + 1) * 256], i32)
                tile = lambda h, c: pltpu.bitcast(x_s[NX + 2 * h + c // 2, tmp, (c % 2) * 128:(c % 2 + 1) * 128], f32)
            else:
                tile = lambda h, c: xs[h][:, c * 128:(c + 1) * 128]
            left = None
            for a in range(7):
                l1 = [[alpha_one(a, lambda r1, c1: tile(2 * r1 + r2, 2 * c1 + c2)) for c2 in range(2)] for r2 in range(2)]
                for r2 in range(2):
                    x_s[2 * a + r2, dst, :] = pk(cols(*l1[r2]))
                l2 = [v for k, v in enumerate(alpha(l1)) if k not in (2, 3)]
                if left is not None:
                    l2 = [left] + l2
                left = l2.pop() if len(l2) % 2 else None
                for k in range(len(l2) // 2):
                    x_s[14 + 5 * a // 2 + k, dst, :] = pk(cols(l2[2 * k], l2[2 * k + 1]))
            x_s[NX - 1, dst, :] = pk(cols(left, left))

        def set_proj(n, w):
            for k, v in enumerate(beta(quad(w))):
                wp_s[n, k] = pk(v)

        def proj(n, r0, first=lambda k, v: v):
            r2_ = r0 // 2 if isinstance(r0, int) else pl.multiple_of(r0 // 2, 8)
            return gamma([_dot(up(first(k, rows(x_s[2 * k, pl.ds(r2_, H2), :], x_s[2 * k + 1, pl.ds(r2_, H2), :]))),
                               up(wp_s[n, k])) for k in range(7)])

        for c in (wc["q"], wc["k"], xc[0], wc["up"], wc["dw"]):
            c.start()
        for b in range(B):
            for h in range(4):
                x_v[b, h, TQ:nb * H, :] = jnp.zeros((nb * H - TQ, D), x_v.dtype)
        for k in range(NX):
            x_s[k, nb * H2:NP // 2, :] = jnp.zeros((NP // 2 - nb * H2, D // 2), i32)
        for c in range(NL):
            for h in range(4):
                g_s[nb, h, c, HALO + H:, :] = jnp.zeros((HALO, 128), f32)
            dw_s[c] = jnp.zeros((32, 128), f32)
        for c in (wc["q"], wc["k"]):
            c.wait()
        xc[1].start()
        set_proj(0, _dot(wq[...], wk[...], NT) * (LOG2E * D ** -0.5))
        for c in (xc[0], wc["up"], wc["dw"]):
            c.wait()
        xc[2].start()
        set_proj(1, wup[:, 0:D].astype(f32))
        set_proj(2, wup[:, D:2 * D].astype(f32))
        for c in range(NL):
            dw_s[c, 0:K, :] = dwv[:, c * 128:(c + 1) * 128].astype(f32) * 0.5

        def prepare(b):
            pl.loop(0, H, step=L1)(lambda p: ln_part(b, p, L1))

            @pl.loop(0, nb)
            def _(i):
                for k in range(1, len(xc)):
                    @pl.when((b == 0) & (i == 2 * k - 1))
                    def _():
                        xc[k].wait()
                        for c in ((xc[3], wc["v"], wc["ao"]), (wc["m0"], wc["dn"], wc["m1"]), (xrest,))[k - 1]:
                            c.start()
                r = pl.multiple_of(i * H, 16)
                never = i < 0
                zero8 = pl.multiple_of(jnp.minimum(i, 0), 8)
                nxt = jnp.minimum(i + 1, nb - 1) * H
                lnq = [[] for _ in range(14)]
                for n, p in enumerate(range(0, H, LR)):
                    lnq[L0 + n * (LE - L0) * LR // H].append(p)

                def interleave(n, v):
                    for p in lnq[n]:
                        ln_part(b, nxt + p, LR)
                    return v

                gpre = unlvl1(proj(2, r, lambda k, v: interleave(k, v)))
                gq = []
                for p in range(0, H, GR):
                    for h in range(4):
                        gg = _ln(_gelu2(cols(*[t[p:p + GR] for t in gpre[h]])), 4e-5)
                        for c in range(NL):
                            t = gg[:, c * 128:(c + 1) * 128]
                            g_s[i + 1, h, c, HALO + p:HALO + p + GR, :] = t
                            if p == 0:
                                g_s[i, h, c, HALO + H:, :] = t[:HALO]
                            if p + GR == H:
                                g_s[i + 2, h, c, 0:HALO, :] = t[GR - HALO:]
                    gq.append(g_s[i + 1, 0, 0, pl.ds(zero8 + HALO, 8), :])
                gq = [[]] * G0 + spread(gq, GE - G0) + [[]] * (7 - GE)
                qn = beta(tr(proj(0, r, lambda k, v: tie(never, interleave(7 + k, v), gq[k]))))
                for k in range(7):
                    qc_s[i, k] = pk(qn[k])

            zero = jnp.zeros((HALO, 128), f32)
            for c in range(NL):
                for h in range(4):
                    g_s[nb, h, c, HALO + HL:2 * HALO + HL, :] = g_s[1, h + 1, c, HALO:2 * HALO, :] if h < 3 else zero
                    g_s[1, h, c, 0:HALO, :] = g_s[nb, h - 1, c, HL:HL + HALO, :] if h else zero

        def merge_weights():
            for n in ("v", "ao", "m0", "dn", "m1"):
                wc[n].wait()

            @pl.loop(0, 3)
            def _(n):
                w = _dot(wa[n], wb[n])

                @pl.when(n == 0)
                def _():
                    wa[1] = w.astype(bf)

                @pl.when(n > 0)
                def _():
                    for k, v in enumerate(beta(quad(w))):
                        wf_s[k, pl.ds(pl.multiple_of((n - 1) * (D // 4), 8), D // 4), :] = pk(v)

        def ocopy(b, r, n):
            return pltpu.make_async_copy(ob_s.at[:, pl.ds(0, n), :], o_hbm.at[b, :, pl.ds(r, n), :], osem.at[0])

        @jax.named_scope("step")
        def step(b, i):
            r = pl.multiple_of(i * H, 16)
            never = i < 0

            cv = [[None] * NL for _ in range(4)]
            convq = []
            for h in range(4):
                for c in range(NL):
                    w = dw_s[c]
                    ps = []
                    for rr in range(0, H, CR):
                        acc = None
                        for tt in sorted(range(K), key=lambda t: (t % 8, t)):
                            term = g_s[i + 1, h, c, pl.ds(rr + HALO - pad + tt, CR), :] * w[tt:tt + 1, :]
                            acc = term if acc is None else acc + term
                        ps.append(acc)
                        convq.append(toks(acc))
                    cv[h][c] = rows(*ps)

            qch = [(r2, j) for j in range(NP // C) for r2 in range(2)]
            qc = [qc_s[i, k] for k in range(7)]
            E = [[[None] * (NP // 128) for _ in range(4)] for _ in range(4)]
            m = [None] * 4
            l = [None] * 4
            statq = []
            for jj, (r2, j) in enumerate(qch):
                ks = slice(j * C // 2, (j + 1) * C // 2)
                st = [[]] * SK + spread(statq, 7 - SK)
                mm = []
                for k in range(7):
                    ts = st[k] + sum(take(convq, CQ.count(k)), [])
                    mm.append(_dot(up(tie(never, qc[k], ts)), up(x_s[2 * k + r2, ks, :]), NT))
                z = unlvl1(tr(gamma(mm)))
                for h in range(4):
                    new = []
                    for c1 in range(2):
                        v = cols(z[h][2 * c1], z[h][2 * c1 + 1])
                        for t_ in range(C // 128):
                            tl = v[:, t_ * 128:(t_ + 1) * 128]
                            c0 = j * C + t_ * 128
                            if c0 + 128 > TQ:
                                tl = jnp.where(c0 + lax.broadcasted_iota(i32, (H, 128), 1) < TQ, tl, -jnp.inf)
                            new.append((2 * c1 + r2, c0 // 128, tl))
                    mx = functools.reduce(jnp.maximum, [v for _, _, v in new])
                    if m[h] is None:
                        mn, ln_ = mx, None
                    else:
                        mn = jnp.maximum(m[h], mx)
                        ln_ = l[h] * jnp.exp2(m[h] - mn)
                    for n, t_, tl in new:
                        e = jnp.exp2(tl - mn)
                        E[h][n][t_] = (e, mn) if T2 else tl
                        ln_ = e if ln_ is None else ln_ + e
                    m[h], l[h] = mn, ln_
                tl_ = [toks(v) for v in l]
                statq = [tl_[2 * r1 + a][p] for a in range(2) for p in range(H // 8) for r1 in range(2)]
            sh = []
            for h in range(4):
                mr = jnp.max(m[h], axis=-1, keepdims=True)
                lr = jnp.sum(l[h] * jnp.exp2(m[h] - mr), axis=-1, keepdims=True)
                sh.append(mr + jnp.log2(lr))
            corr = {}

            def prob(h, n, t_):
                if not T2:
                    return jnp.exp2(E[h][n][t_] - sh[h])
                e, mn = E[h][n][t_]
                if (h, id(mn)) not in corr:
                    corr[h, id(mn)] = jnp.exp2(mn - sh[h])
                return e * corr[h, id(mn)]

            vt = np.cumsum((0,) + tuple(VCH))
            vch = [(r2, vt[j], vt[j + 1]) for j in range(len(VCH)) for r2 in range(2 if LV == 1 else 1)]
            NPR = 7 ** LV

            def pv_ops(jj):
                r2, ta, te = vch[jj]
                pe = lambda h, n: cols(*[prob(h, n, t_) for t_ in range(ta, te)])
                if LV == 1:
                    pc = alpha([[rows(pe(2 * r1, 2 * c1 + r2), pe(2 * r1 + 1, 2 * c1 + r2)) for c1 in range(2)]
                                for r1 in range(2)])
                    return pc, [pc[a][p:p + 8, t_ * 128:(t_ + 1) * 128]
                                for p in range(0, 2 * H, 8) for t_ in range(te - ta) for a in PA]
                g = [[pe(h, n) for n in range(4)] for h in range(4)]
                if not YM:
                    l1 = [[alpha([[g[2 * r1 + r_][2 * c1 + c2] for c1 in range(2)] for r1 in range(2)])
                           for c2 in range(2)] for r_ in range(2)]
                    pc = [v for a in range(7) for v in alpha([[l1[r_][c2][a] for c2 in range(2)] for r_ in range(2)])]
                    return pc, [l1[r_][c2][a][p:p + 8, t_ * 128:(t_ + 1) * 128] for p in range(0, H, 8)
                                for r_ in range(2) for c2 in range(2) for t_ in range(te - ta) for a in PA]
                return alpha2_direct(g), [g[h][n][p:p + 8, t_ * 128:(t_ + 1) * 128] for p in range(0, H, 8)
                                          for h in range(4) for n in range(4) for t_ in range(te - ta)]

            def pv_rhs(jj, k):
                r2, ta, te = vch[jj]
                ks = slice(ta * 64, te * 64)
                if LV == 1:
                    return x_s[2 * PERM[k] + r2, ks, :]
                a, k = PERM[k // 7], PERM[k % 7]
                n = 4 * a if k == 2 else 4 * a + 3 if k == 3 else 28 + 5 * a + (k if k < 2 else k - 2)
                return x_s[n // 2, ks, (n % 2) * 128:(n % 2 + 1) * 128]

            pc, pq = pv_ops(0)
            st = [[]] * U0 + spread(statq, UK) + [[]] * (7 - UK - U0)
            pp = [[]] * (7 - UG) + spread(pq, UG) if UG else [[]] * 7
            upre = unlvl1(proj(1, r, lambda k, v: tie(never, v, st[k] + pp[k])))
            u, uq = None, []

            acc = [None] * NPR
            nv = len(vch)
            f7 = NPR // 7
            win = lambda q, a, e: [[]] * (a * f7) + spread(q, (e - a) * f7) + [[]] * ((7 - e) * f7)
            assert US < UJ < nv
            for jj in range(nv):
                pcn, pq = pv_ops(jj + 1) if jj + 1 < nv else (None, [])
                pp = win(pq, *PW)
                ug = win(uq if jj == UJ else [], *UW)
                cg = win(take(convq, CJ[jj]), *CW)
                for k in range(NPR):
                    ts = pp[k] + ug[k] + sum(cg[k], [])
                    d = _dot(tie(never, pc[k], ts).astype(bf), up(pv_rhs(jj, k)))
                    if k == USK * f7:
                        d0 = d
                    acc[k] = d if acc[k] is None else acc[k] + d
                pc = pcn
                if jj == US:
                    u = [[_gelu2(jnp.where(never, d0[:H, :128], upre[h][c])) for c in range(4)] for h in range(4)]
                    uq = [t for row in u for v in row for t in toks(v)]
            o = gamma(acc) if LV == 1 else lvl1(gamma2([acc[7 * a:7 * a + 7] for a in range(7)]))
            uc = [[u[h][c] * cv[h][c] for c in range(4)] for h in range(4)]
            ao, au = alpha(o), alpha(lvl1(uc))

            pl.when((i == 0) & (b > 0))(lambda: ocopy(0, 0, HL).wait())
            pl.when(i > 0)(lambda: ocopy(0, 0, H).wait())
            fo = [None] * 7
            for k in FO:
                fo[k] = _dot(cols(ao[k], au[k]).astype(bf), up(wf_s[k]))
            out = unlvl1(gamma(fo))
            for h in range(4):
                ob_s[h] = (x_v[b, h, pl.ds(r, H), :].astype(f32) + cols(*out[h])).astype(ob_s.dtype)
            pl.when(i < nb - 1)(lambda: ocopy(b, r, H).start())
            pl.when(i == nb - 1)(lambda: ocopy(b, r, HL).start())

        @pl.loop(0, B)
        def _(b):
            pl.when(b == 1)(lambda: xrest.wait())
            prepare(b)
            pl.when(b == 0)(merge_weights)
            pl.loop(0, nb)(functools.partial(step, b))

        ocopy(0, 0, HL).wait()

    @jax.jit
    def fn(x, w_q, w_k, w_v, w_ao, w_up, dw, w_dn, w_merge):
        B, T, D = x.shape
        K = dw.shape[0]
        TQ = T // 4
        TP = -(-TQ // H) * H
        NP = 128 * sum(VCH)
        assert NP >= TP + HALO and NP % C == 0
        ws = (w_q, w_k, w_v, w_ao, w_up, dw, w_dn, w_merge)
        anyspec = pl.BlockSpec(memory_space=pl.ANY)
        out = pl.pallas_call(
            functools.partial(kern, B=B, TQ=TQ, D=D, K=K, NP=NP),
            in_specs=[anyspec] * 9,
            out_specs=anyspec,
            out_shape=jax.ShapeDtypeStruct((B, 4, TQ, D), x.dtype),
            scratch_shapes=[pltpu.VMEM((B, 4, TP, D), x.dtype)] + [
                pltpu.VMEM(w.shape, w.dtype) for w in (w_q, w_k, w_up, dw)] + [
                pltpu.VMEM((3, D, D), bf),
                pltpu.VMEM((3, D, D), bf),
                pltpu.VMEM((3, 7, D // 4, D // 2), i32),
                pltpu.VMEM((7, D // 2, D // 2), i32),
                pltpu.VMEM((NX + 8, NP // 2, D // 2), i32),
                pltpu.VMEM((TP // H, 7, H, D // 2), i32),
                pltpu.VMEM((TP // H + 2, 4, D // 128, H + 2 * HALO, 128), f32),
                pltpu.VMEM((D // 128, 32, 128), f32),
                pltpu.VMEM((4, H, D), x.dtype),
                pltpu.SemaphoreType.DMA((9,)),
                pltpu.SemaphoreType.DMA((5,)),
                pltpu.SemaphoreType.DMA((1,)),
            ],
            compiler_params=pltpu.CompilerParams(vmem_limit_bytes=112 * 1024 * 1024, flags=FLAGS),
        )(x.reshape(B, 4, TQ, D), *ws)
        return out.reshape(B, T, D)
    return fn


_impl = make(LE=7)


def pallas_standalone__conformer_family_branchformer__speech_kernel(x, w_q, w_k, w_v, w_ao, w_up, dw, w_dn, w_merge):
    return _impl(x, w_q, w_k, w_v, w_ao, w_up, dw, w_dn, w_merge)
```

```python
import functools
import jax
import jax.numpy as jnp
import numpy as np
from jax import lax
import jax.experimental.pallas as pl
import jax.experimental.pallas.tpu as pltpu

LOG2E = 1.4426950408889634
NT = (((1,), (1,)), ((), ()))
NN = (((1,), (0,)), ((), ()))
bf = jnp.bfloat16
f32 = jnp.float32
i32 = jnp.int32
HALO = 16
PERM = (0, 2, 6, 5, 3, 4, 1)


def _ln(x, eps=1e-5):
    m = jnp.mean(x, axis=-1, keepdims=True)
    d = x - m
    v = jnp.mean(d * d, axis=-1, keepdims=True)
    return d * lax.rsqrt(v + eps)


def _gelu2(x):
    c = float(np.sqrt(2.0 / np.pi))
    return x * jnp.tanh((x * x * (0.044715 * c) + c) * x) + x


def _dot(a, b, dims=NN):
    return lax.dot_general(a, b, dims, preferred_element_type=f32)


def rows(*p):
    return jnp.concatenate(p, axis=0)


def cols(*p):
    return jnp.concatenate(p, axis=1)


def pk(v):
    return pltpu.bitcast(v.astype(bf), i32)


def up(v):
    return pltpu.bitcast(v, bf)


def alpha(z):
    (a, b), (c, d) = z
    return [a + d, c + d, a, d, a + b, c - a, b - d]


def alpha_one(k, z):
    return [lambda: z(0, 0) + z(1, 1), lambda: z(1, 0) + z(1, 1), lambda: z(0, 0), lambda: z(1, 1),
            lambda: z(0, 0) + z(0, 1), lambda: z(1, 0) - z(0, 0), lambda: z(0, 1) - z(1, 1)][k]()


def beta(z):
    t = alpha(z)
    return [t[k] for k in PERM]


def gamma(n):
    return [[n[0] + n[3] - n[4] + n[6], n[2] + n[4]], [n[1] + n[3], n[0] - n[1] + n[2] + n[5]]]


def tr(z):
    return [list(r) for r in zip(*z)]


def lvl1(g):
    return [[rows(*[cols(g[2 * r1 + r2][2 * c1], g[2 * r1 + r2][2 * c1 + 1]) for r2 in range(2)])
             for c1 in range(2)] for r1 in range(2)]


def unlvl1(z):
    out = [[None] * 4 for _ in range(4)]
    for r1 in range(2):
        for c1 in range(2):
            v = z[r1][c1]
            n, m = v.shape[0] // 2, v.shape[1] // 2
            for r2 in range(2):
                for c2 in range(2):
                    out[2 * r1 + r2][2 * c1 + c2] = v[r2 * n:(r2 + 1) * n, c2 * m:(c2 + 1) * m]
    return out


def two(f, g):
    l1 = [[f([[g[2 * r1 + r2][2 * c1 + c2] for c1 in range(2)] for r1 in range(2)])
           for c2 in range(2)] for r2 in range(2)]
    return [f([[l1[r2][c2][a] for c2 in range(2)] for r2 in range(2)]) for a in range(7)]


def alpha2_direct(g):
    terms = [[(0, 0, 1), (1, 1, 1)], [(1, 0, 1), (1, 1, 1)], [(0, 0, 1)], [(1, 1, 1)],
             [(0, 0, 1), (0, 1, 1)], [(1, 0, 1), (0, 0, -1)], [(0, 1, 1), (1, 1, -1)]]

    def pair(u, v):
        (x, sx), (y, sy) = u, v
        if sx > 0:
            return (x + y if sy > 0 else x - y), 1
        return (y - x, 1) if sy > 0 else (x + y, -1)

    out = []
    for a in range(7):
        for k in range(7):
            t = [[(g[2 * r1 + r2][2 * c1 + c2], s1 * s2) for r2, c2, s2 in terms[k]] for r1, c1, s1 in terms[a]]
            if len(t) == 2 and len(t[0]) == 2:
                v, sign = pair(pair(t[0][0], t[1][1]), pair(t[0][1], t[1][0]))
            else:
                f = [e for row in t for e in row]
                v, sign = pair(*f) if len(f) == 2 else f[0]
            assert sign > 0
            out.append(v)
    return out


def gamma2(n):
    inner = [gamma(n[a]) for a in range(7)]
    out = [[None] * 4 for _ in range(4)]
    for r2 in range(2):
        for c2 in range(2):
            z = gamma([inner[a][r2][c2] for a in range(7)])
            for r1 in range(2):
                for c1 in range(2):
                    out[2 * r1 + r2][2 * c1 + c2] = z[r1][c1]
    return out


def toks(a):
    return [a[k:k + 8, :128] for k in range(0, a.shape[0], 8)]


def take(q, n):
    out = q[:n]
    del q[:n]
    return out


def spread(q, n):
    q0 = list(q)
    del q[:]
    return [q0[k * len(q0) // n:(k + 1) * len(q0) // n] for k in range(n)]


def tie(never, a, ts):
    if not ts:
        return a
    nr, nc = a.shape[0] // 8, a.shape[1] // 128
    cells = {}
    for j, t in enumerate(ts):
        p = j * nr * nc // len(ts)
        cells[p] = jnp.maximum(cells[p], t) if p in cells else t
    out = []
    for p in range(nr):
        row = []
        for c in range(nc):
            v = a[8 * p:8 * p + 8, 128 * c:128 * c + 128]
            t = cells.get(p * nc + c)
            if t is not None:
                v = jnp.where(never, t if t.dtype == a.dtype else pltpu.bitcast(t, a.dtype), v)
            row.append(v)
        out.append(cols(*row))
    return rows(*out)


def quad(w):
    n, m = w.shape[0] // 2, w.shape[1] // 2
    return [[w[i * n:(i + 1) * n, j * m:(j + 1) * m] for j in range(2)] for i in range(2)]


DEFAULTS = {
    1: dict(VCH=(2, 2, 2, 2), CR=72, T2=True, SK=3, CQ=(1, 2), U0=1, UK=3, UG=2,
            PA=(5, 6), PW=(2, 7), CJ=(0, 0, 3, 3, 3, 3, 2, 2), CW=(0, 2), US=0, USK=4, UJ=1, UW=(0, 7), YM=False),
    2: dict(VCH=(2, 2, 4), CR=72, T2=True, SK=3, CQ=(1, 1, 2), U0=0, UK=3, UG=2,
            PA=(5, 6), PW=(4, 7), CJ=(0, 2, 6), CW=(0, 3), US=0, USK=4, UJ=1, UW=(1, 3), YM=True),
}


def make(H=144, C=256, LV=2, FLAGS=None, FO=(1, 3, 0, 2, 4, 5, 6), STG=False, L0=2, LE=9, GR=24, GH=False, G0=1, GE=7, **kw):
    cfg = dict(DEFAULTS[LV], **kw)
    VCH, CR, T2, SK, CQ, U0, UK, UG = (cfg[k] for k in "VCH CR T2 SK CQ U0 UK UG".split())
    PA, PW, CJ, CW, US, USK, UJ, UW, YM = (cfg[k] for k in "PA PW CJ CW US USK UJ UW YM".split())
    NX = 32
    def kern(x_hbm, wq_hbm, wk_hbm, wv_hbm, wao_hbm, wup_hbm, dw_hbm, wdn_hbm, wm_hbm,
             o_hbm,
             x_v, wq, wk, wup, dwv, wa, wb,
             wp_s, wf_s, xa_s, x_s, qc_s, g_s, dw_s, ob_s,
             wsem, xsem, osem, *, B, TQ, D, K, NP):
        NL = D // 128
        pad = K // 2
        nb = -(-TQ // H)
        HL = TQ - (nb - 1) * H
        H2 = H // 2

        wc = {n: pltpu.make_async_copy(s, d, wsem.at[k]) for k, (n, s, d) in enumerate(
            [("v", wv_hbm, wa.at[0]), ("ao", wao_hbm, wb.at[0]), ("m0", wm_hbm.at[0:D], wb.at[1]),
             ("dn", wdn_hbm, wa.at[2]), ("m1", wm_hbm.at[D:2 * D], wb.at[2]),
             ("q", wq_hbm, wq), ("k", wk_hbm, wk), ("up", wup_hbm, wup), ("dw", dw_hbm, dwv)])}
        cuts = [0, 2 * H, 4 * H, 6 * H, TQ]
        xc = [pltpu.make_async_copy(x_hbm.at[0, :, pl.ds(a, e - a), :], x_v.at[0, :, pl.ds(a, e - a), :], xsem.at[n])
              for n, (a, e) in enumerate(zip(cuts[:-1], cuts[1:]))]
        xrest = pltpu.make_async_copy(x_hbm.at[pl.ds(1, B - 1)], x_v.at[pl.ds(1, B - 1), :, pl.ds(0, TQ), :],
                                      xsem.at[len(xc)])

        def set_proj(n, w):
            for k, v in enumerate(beta(quad(w))):
                wp_s[n, k] = pk(v)

        def proj(n, r0, first=lambda k, v: v):
            r2_ = r0 // 2 if isinstance(r0, int) else pl.multiple_of(r0 // 2, 8)
            return gamma([_dot(up(first(k, rows(x_s[2 * k, pl.ds(r2_, H2), :], x_s[2 * k + 1, pl.ds(r2_, H2), :]))),
                               up(wp_s[n, k])) for k in range(7)])

        for c in (wc["q"], wc["k"], xc[0], xc[1]):
            c.start()
        for b in range(B):
            for h in range(4):
                x_v[b, h, TQ:, :] = jnp.zeros((nb * H - TQ, D), x_v.dtype)
        for k in range(NX):
            x_s[k, nb * H2:, :] = jnp.zeros((NP // 2 - nb * H2, D // 2), i32)
        for c in range(NL):
            for h in range(4):
                g_s[nb, h, c, HALO + H:, :] = jnp.zeros((HALO, 128), f32)
            dw_s[c] = jnp.zeros((32, 128), f32)
        for c in (wc["q"], wc["k"]):
            c.wait()
        for c in (wc["up"], wc["dw"]):
            c.start()
        set_proj(0, _dot(wq[...], wk[...], NT) * (LOG2E * D ** -0.5))

        def normalize(b, r, n):
            rr = pl.ds(pl.multiple_of(r, 16), n)
            for h in range(4):
                xa_s[b, h, rr, :] = _ln(x_v[b, h, rr, :].astype(f32)).astype(bf)

        @pl.loop(0, nb)
        def _(i):
            for k in range(len(xc)):
                @pl.when(i * H == cuts[k])
                def _():
                    if k == 2:
                        for c in (wc["up"], wc["dw"]):
                            c.wait()
                        set_proj(1, wup[:, 0:D].astype(f32))
                        set_proj(2, wup[:, D:2 * D].astype(f32))
                        for c in range(NL):
                            dw_s[c, 0:K, :] = dwv[:, c * 128:(c + 1) * 128].astype(f32) * 0.5
                    xc[k].wait()
                    for c in ((xc[2],), (xc[3],), (), (wc["v"], wc["ao"], wc["m0"], wc["dn"], wc["m1"], xrest))[k]:
                        c.start()
            normalize(0, i * H, H)

        def prepare(b):
            @pl.loop(0, nb)
            def _(i):
                r = pl.multiple_of(i * H, 16)
                dst = pl.ds(pl.multiple_of(i * H2, 8), H2)
                never = i < 0
                zero8 = pl.multiple_of(jnp.minimum(i, 0), 8)
                x1, xq, left = [], [], None
                for a in range(7):
                    ra = pl.multiple_of(r + jnp.minimum(i + a, 0), 16) if STG else r
                    tile = lambda h, c: xa_s[b, h, pl.ds(ra, H), (c // 2) * 256:(c // 2 + 1) * 256].astype(f32)[
                        :, (c % 2) * 128:(c % 2 + 1) * 128]
                    l1 = [[alpha_one(a, lambda r1, c1: tile(2 * r1 + r2, 2 * c1 + c2)) for c2 in range(2)]
                          for r2 in range(2)]
                    x1.append([pk(cols(*l1[r2])) for r2 in range(2)])
                    for r2 in range(2):
                        x_s[2 * a + r2, dst, :] = x1[a][r2]
                    l2 = [v for k, v in enumerate(alpha(l1)) if k not in (2, 3)]
                    if left is not None:
                        l2 = [left] + l2
                    left = l2.pop() if len(l2) % 2 else None
                    if a == 6:
                        l2 += [left, left]
                    for k in range(len(l2) // 2):
                        x_s[14 + 5 * a // 2 + k, dst, :] = pk(cols(l2[2 * k], l2[2 * k + 1]))
                    xq.append([pltpu.bitcast(x_s[0, pl.ds(zero8, 8), :128], f32)])
                xq = [[]] * L0 + spread(xq, LE - L0) + [[]] * (14 - LE)
                xq = [sum(v, []) for v in xq]
                pr = lambda n, ts: gamma([_dot(up(tie(never, rows(*x1[k]), ts[k])), up(wp_s[n, k])) for k in range(7)])
                gpre = unlvl1(pr(2, xq))
                gq = []
                for p in range(0, H, GR):
                    for h in range(4):
                        gg = _ln(_gelu2(cols(*[t[p:p + GR] for t in gpre[h]])), 4e-5)
                        for c in range(NL):
                            t = gg[:, c * 128:(c + 1) * 128]
                            g_s[i + 1, h, c, HALO + p:HALO + p + GR, :] = t
                            if p < HALO:
                                g_s[i, h, c, HALO + H + p:HALO + H + min(p + GR, HALO), :] = t[:HALO - p]
                            if p + GR > H - HALO:
                                o = max(H - HALO - p, 0)
                                g_s[i + 2, h, c, p + o - (H - HALO):p + GR - (H - HALO), :] = t[o:]
                        if GH or h == 3:
                            gq.append(g_s[i + 1, 0, 0, pl.ds(zero8 + HALO, 8), :])
                gq = [[]] * G0 + spread(gq, GE - G0) + [[]] * (7 - GE)
                qn = beta(tr(pr(0, [gq[k] + xq[7 + k] for k in range(7)])))
                for k in range(7):
                    qc_s[i, k] = pk(qn[k])

            zero = jnp.zeros((HALO, 128), f32)
            for c in range(NL):
                for h in range(4):
                    g_s[nb, h, c, HALO + HL:2 * HALO + HL, :] = g_s[1, h + 1, c, HALO:2 * HALO, :] if h < 3 else zero
                    g_s[1, h, c, 0:HALO, :] = g_s[nb, h - 1, c, HL:HL + HALO, :] if h else zero

        def merge_weights():
            for n in ("v", "ao", "m0", "dn", "m1"):
                wc[n].wait()

            @pl.loop(0, 3)
            def _(n):
                w = _dot(wa[n], wb[n])
                for b in range(1, B):
                    normalize(b, n * (nb * H // 3), nb * H // 3)

                @pl.when(n == 0)
                def _():
                    wa[1] = w.astype(bf)

                @pl.when(n > 0)
                def _():
                    for k, v in enumerate(beta(quad(w))):
                        wf_s[k, pl.ds(pl.multiple_of((n - 1) * (D // 4), 8), D // 4), :] = pk(v)

        def ocopy(ob, b, r, n):
            return pltpu.make_async_copy(ob_s.at[ob, :, pl.ds(0, n), :], o_hbm.at[b, :, pl.ds(r, n), :], osem.at[ob])

        @jax.named_scope("step")
        def step(b, i):
            r = pl.multiple_of(i * H, 16)
            never = i < 0
            it = b * nb + i
            ob = it % 2
            short = (i == 1) & (b > 0)
            pl.when(short)(lambda: ocopy(ob, 0, 0, HL).wait())
            pl.when((it > 1) & jnp.logical_not(short))(lambda: ocopy(ob, 0, 0, H).wait())

            cv = [[None] * NL for _ in range(4)]
            convq = []
            for h in range(4):
                for c in range(NL):
                    w = dw_s[c]
                    ps = []
                    for rr in range(0, H, CR):
                        acc = None
                        for tt in sorted(range(K), key=lambda t: (t % 8, t)):
                            term = g_s[i + 1, h, c, pl.ds(rr + HALO - pad + tt, CR), :] * w[tt:tt + 1, :]
                            acc = term if acc is None else acc + term
                        ps.append(acc)
                        convq.append(toks(acc))
                    cv[h][c] = rows(*ps)

            qch = [(r2, j) for j in range(NP // C) for r2 in range(2)]
            qc = [qc_s[i, k] for k in range(7)]
            E = [[[None] * (NP // 128) for _ in range(4)] for _ in range(4)]
            m = [None] * 4
            l = [None] * 4
            statq = []
            for jj, (r2, j) in enumerate(qch):
                ks = slice(j * C // 2, (j + 1) * C // 2)
                st = [[]] * SK + spread(statq, 7 - SK)
                mm = []
                for k in range(7):
                    ts = st[k] + sum(take(convq, CQ.count(k)), [])
                    mm.append(_dot(up(tie(never, qc[k], ts)), up(x_s[2 * k + r2, ks, :]), NT))
                z = unlvl1(tr(gamma(mm)))
                for h in range(4):
                    new = []
                    for c1 in range(2):
                        v = cols(z[h][2 * c1], z[h][2 * c1 + 1])
                        for t_ in range(C // 128):
                            tl = v[:, t_ * 128:(t_ + 1) * 128]
                            c0 = j * C + t_ * 128
                            if c0 + 128 > TQ:
                                tl = jnp.where(c0 + lax.broadcasted_iota(i32, (H, 128), 1) < TQ, tl, -jnp.inf)
                            new.append((2 * c1 + r2, c0 // 128, tl))
                    mx = functools.reduce(jnp.maximum, [v for _, _, v in new])
                    if m[h] is None:
                        mn, ln_ = mx, None
                    else:
                        mn = jnp.maximum(m[h], mx)
                        ln_ = l[h] * jnp.exp2(m[h] - mn)
                    for n, t_, tl in new:
                        e = jnp.exp2(tl - mn)
                        E[h][n][t_] = (e, mn) if T2 else tl
                        ln_ = e if ln_ is None else ln_ + e
                    m[h], l[h] = mn, ln_
                tl_ = [toks(v) for v in l]
                statq = [tl_[2 * r1 + a][p] for a in range(2) for p in range(H // 8) for r1 in range(2)]
            sh = []
            for h in range(4):
                mr = jnp.max(m[h], axis=-1, keepdims=True)
                lr = jnp.sum(l[h] * jnp.exp2(m[h] - mr), axis=-1, keepdims=True)
                sh.append(mr + jnp.log2(lr))
            corr = {}

            def prob(h, n, t_):
                if not T2:
                    return jnp.exp2(E[h][n][t_] - sh[h])
                e, mn = E[h][n][t_]
                if (h, id(mn)) not in corr:
                    corr[h, id(mn)] = jnp.exp2(mn - sh[h])
                return e * corr[h, id(mn)]

            vt = np.cumsum((0,) + tuple(VCH))
            vch = [(r2, vt[j], vt[j + 1]) for j in range(len(VCH)) for r2 in range(2 if LV == 1 else 1)]
            NPR = 7 ** LV

            def pv_ops(jj):
                r2, ta, te = vch[jj]
                pe = lambda h, n: cols(*[prob(h, n, t_) for t_ in range(ta, te)])
                if LV == 1:
                    pc = alpha([[rows(pe(2 * r1, 2 * c1 + r2), pe(2 * r1 + 1, 2 * c1 + r2)) for c1 in range(2)]
                                for r1 in range(2)])
                    return pc, [pc[a][p:p + 8, t_ * 128:(t_ + 1) * 128]
                                for p in range(0, 2 * H, 8) for t_ in range(te - ta) for a in PA]
                g = [[pe(h, n) for n in range(4)] for h in range(4)]
                if not YM:
                    l1 = [[alpha([[g[2 * r1 + r_][2 * c1 + c2] for c1 in range(2)] for r1 in range(2)])
                           for c2 in range(2)] for r_ in range(2)]
                    pc = [v for a in range(7) for v in alpha([[l1[r_][c2][a] for c2 in range(2)] for r_ in range(2)])]
                    return pc, [l1[r_][c2][a][p:p + 8, t_ * 128:(t_ + 1) * 128] for p in range(0, H, 8)
                                for r_ in range(2) for c2 in range(2) for t_ in range(te - ta) for a in PA]
                return alpha2_direct(g), [g[h][n][p:p + 8, t_ * 128:(t_ + 1) * 128] for p in range(0, H, 8)
                                          for h in range(4) for n in range(4) for t_ in range(te - ta)]

            def pv_rhs(jj, k):
                r2, ta, te = vch[jj]
                ks = slice(ta * 64, te * 64)
                if LV == 1:
                    return x_s[2 * PERM[k] + r2, ks, :]
                a, k = PERM[k // 7], PERM[k % 7]
                n = 4 * a if k == 2 else 4 * a + 3 if k == 3 else 28 + 5 * a + (k if k < 2 else k - 2)
                return x_s[n // 2, ks, (n % 2) * 128:(n % 2 + 1) * 128]

            pc, pq = pv_ops(0)
            st = [[]] * U0 + spread(statq, UK) + [[]] * (7 - UK - U0)
            pp = [[]] * (7 - UG) + spread(pq, UG) if UG else [[]] * 7
            upre = unlvl1(proj(1, r, lambda k, v: tie(never, v, st[k] + pp[k])))
            u, uq = None, []

            acc = [None] * NPR
            nv = len(vch)
            f7 = NPR // 7
            win = lambda q, a, e: [[]] * (a * f7) + spread(q, (e - a) * f7) + [[]] * ((7 - e) * f7)
            assert US < UJ < nv
            for jj in range(nv):
                pcn, pq = pv_ops(jj + 1) if jj + 1 < nv else (None, [])
                pp = win(pq, *PW)
                ug = win(uq if jj == UJ else [], *UW)
                cg = win(take(convq, CJ[jj]), *CW)
                for k in range(NPR):
                    ts = pp[k] + ug[k] + sum(cg[k], [])
                    d = _dot(tie(never, pc[k], ts).astype(bf), up(pv_rhs(jj, k)))
                    if k == USK * f7:
                        d0 = d
                    acc[k] = d if acc[k] is None else acc[k] + d
                pc = pcn
                if jj == US:
                    u = [[_gelu2(jnp.where(never, d0[:H, :128], upre[h][c])) for c in range(4)] for h in range(4)]
                    uq = [t for row in u for v in row for t in toks(v)]
            o = gamma(acc) if LV == 1 else lvl1(gamma2([acc[7 * a:7 * a + 7] for a in range(7)]))
            uc = [[u[h][c] * cv[h][c] for c in range(4)] for h in range(4)]
            ao, au = alpha(o), alpha(lvl1(uc))

            fo = [None] * 7
            for k in FO:
                fo[k] = _dot(cols(ao[k], au[k]).astype(bf), up(wf_s[k]))
            out = unlvl1(gamma(fo))
            for h in range(4):
                ob_s[ob, h] = (x_v[b, h, pl.ds(r, H), :].astype(f32) + cols(*out[h])).astype(ob_s.dtype)
            pl.when(i < nb - 1)(lambda: ocopy(ob, b, r, H).start())
            pl.when(i == nb - 1)(lambda: ocopy(ob, b, r, HL).start())

        @pl.loop(0, B)
        def _(b):
            pl.when(b == 1)(lambda: xrest.wait())
            prepare(b)
            pl.when(b == 0)(merge_weights)
            pl.loop(0, nb)(functools.partial(step, b))

        ocopy((B * nb) % 2, 0, 0, H).wait()
        ocopy((B * nb + 1) % 2, 0, 0, HL).wait()

    @jax.jit
    def fn(x, w_q, w_k, w_v, w_ao, w_up, dw, w_dn, w_merge):
        B, T, D = x.shape
        K = dw.shape[0]
        TQ = T // 4
        TP = -(-TQ // H) * H
        NP = 128 * sum(VCH)
        assert NP >= TP + HALO and NP % C == 0
        ws = (w_q, w_k, w_v, w_ao, w_up, dw, w_dn, w_merge)
        anyspec = pl.BlockSpec(memory_space=pl.ANY)
        out = pl.pallas_call(
            functools.partial(kern, B=B, TQ=TQ, D=D, K=K, NP=NP),
            in_specs=[anyspec] * 9,
            out_specs=anyspec,
            out_shape=jax.ShapeDtypeStruct((B, 4, TQ, D), x.dtype),
            scratch_shapes=[pltpu.VMEM((B, 4, TP, D), x.dtype)] + [
                pltpu.VMEM(w.shape, w.dtype) for w in (w_q, w_k, w_up, dw)] + [
                pltpu.VMEM((3, D, D), bf),
                pltpu.VMEM((3, D, D), bf),
                pltpu.VMEM((3, 7, D // 4, D // 2), i32),
                pltpu.VMEM((7, D // 2, D // 2), i32),
                pltpu.VMEM((B, 4, TP, D), bf),
                pltpu.VMEM((NX, NP // 2, D // 2), i32),
                pltpu.VMEM((TP // H, 7, H, D // 2), i32),
                pltpu.VMEM((TP // H + 2, 4, D // 128, H + 2 * HALO, 128), f32),
                pltpu.VMEM((D // 128, 32, 128), f32),
                pltpu.VMEM((2, 4, H, D), x.dtype),
                pltpu.SemaphoreType.DMA((9,)),
                pltpu.SemaphoreType.DMA((5,)),
                pltpu.SemaphoreType.DMA((2,)),
            ],
            compiler_params=pltpu.CompilerParams(vmem_limit_bytes=112 * 1024 * 1024, flags=FLAGS),
        )(x.reshape(B, 4, TQ, D), *ws)
        return out.reshape(B, T, D)
    return fn


_impl = make()


def pallas_standalone__conformer_family_branchformer__speech_kernel(x, w_q, w_k, w_v, w_ao, w_up, dw, w_dn, w_merge):
    return _impl(x, w_q, w_k, w_v, w_ao, w_up, dw, w_dn, w_merge)
```

```python
import functools
import jax
import jax.numpy as jnp
import numpy as np
from jax import lax
import jax.experimental.pallas as pl
import jax.experimental.pallas.tpu as pltpu

LOG2E = 1.4426950408889634
NT = (((1,), (1,)), ((), ()))
NN = (((1,), (0,)), ((), ()))
bf = jnp.bfloat16
f32 = jnp.float32
i32 = jnp.int32
HALO = 16
PERM = (0, 2, 6, 5, 3, 4, 1)


def _ln(x, eps=1e-5):
    m = jnp.mean(x, axis=-1, keepdims=True)
    d = x - m
    v = jnp.mean(d * d, axis=-1, keepdims=True)
    return d * lax.rsqrt(v + eps)


def _gelu2(x):
    c = float(np.sqrt(2.0 / np.pi))
    return x * jnp.tanh((x * x * (0.044715 * c) + c) * x) + x


def _dot(a, b, dims=NN):
    return lax.dot_general(a, b, dims, preferred_element_type=f32)


def rows(*p):
    return jnp.concatenate(p, axis=0)


def cols(*p):
    return jnp.concatenate(p, axis=1)


def pk(v):
    return pltpu.bitcast(v.astype(bf), i32)


def up(v):
    return pltpu.bitcast(v, bf)


def alpha(z):
    (a, b), (c, d) = z
    return [a + d, c + d, a, d, a + b, c - a, b - d]


def alpha_one(k, z):
    return [lambda: z(0, 0) + z(1, 1), lambda: z(1, 0) + z(1, 1), lambda: z(0, 0), lambda: z(1, 1),
            lambda: z(0, 0) + z(0, 1), lambda: z(1, 0) - z(0, 0), lambda: z(0, 1) - z(1, 1)][k]()


def beta(z):
    t = alpha(z)
    return [t[k] for k in PERM]


def gamma(n):
    return [[n[0] + n[3] - n[4] + n[6], n[2] + n[4]], [n[1] + n[3], n[0] - n[1] + n[2] + n[5]]]


def tr(z):
    return [list(r) for r in zip(*z)]


def lvl1(g):
    return [[rows(*[cols(g[2 * r1 + r2][2 * c1], g[2 * r1 + r2][2 * c1 + 1]) for r2 in range(2)])
             for c1 in range(2)] for r1 in range(2)]


def unlvl1(z):
    out = [[None] * 4 for _ in range(4)]
    for r1 in range(2):
        for c1 in range(2):
            v = z[r1][c1]
            n, m = v.shape[0] // 2, v.shape[1] // 2
            for r2 in range(2):
                for c2 in range(2):
                    out[2 * r1 + r2][2 * c1 + c2] = v[r2 * n:(r2 + 1) * n, c2 * m:(c2 + 1) * m]
    return out


def two(f, g):
    l1 = [[f([[g[2 * r1 + r2][2 * c1 + c2] for c1 in range(2)] for r1 in range(2)])
           for c2 in range(2)] for r2 in range(2)]
    return [f([[l1[r2][c2][a] for c2 in range(2)] for r2 in range(2)]) for a in range(7)]


def alpha2_direct(g):
    terms = [[(0, 0, 1), (1, 1, 1)], [(1, 0, 1), (1, 1, 1)], [(0, 0, 1)], [(1, 1, 1)],
             [(0, 0, 1), (0, 1, 1)], [(1, 0, 1), (0, 0, -1)], [(0, 1, 1), (1, 1, -1)]]

    def pair(u, v):
        (x, sx), (y, sy) = u, v
        if sx > 0:
            return (x + y if sy > 0 else x - y), 1
        return (y - x, 1) if sy > 0 else (x + y, -1)

    out = []
    for a in range(7):
        for k in range(7):
            t = [[(g[2 * r1 + r2][2 * c1 + c2], s1 * s2) for r2, c2, s2 in terms[k]] for r1, c1, s1 in terms[a]]
            if len(t) == 2 and len(t[0]) == 2:
                v, sign = pair(pair(t[0][0], t[1][1]), pair(t[0][1], t[1][0]))
            else:
                f = [e for row in t for e in row]
                v, sign = pair(*f) if len(f) == 2 else f[0]
            assert sign > 0
            out.append(v)
    return out


def gamma2(n):
    inner = [gamma(n[a]) for a in range(7)]
    out = [[None] * 4 for _ in range(4)]
    for r2 in range(2):
        for c2 in range(2):
            z = gamma([inner[a][r2][c2] for a in range(7)])
            for r1 in range(2):
                for c1 in range(2):
                    out[2 * r1 + r2][2 * c1 + c2] = z[r1][c1]
    return out


def toks(a):
    return [a[k:k + 8, :128] for k in range(0, a.shape[0], 8)]


def take(q, n):
    out = q[:n]
    del q[:n]
    return out


def spread(q, n):
    q0 = list(q)
    del q[:]
    return [q0[k * len(q0) // n:(k + 1) * len(q0) // n] for k in range(n)]


def tie(never, a, ts):
    if not ts:
        return a
    nr, nc = a.shape[0] // 8, a.shape[1] // 128
    cells = {}
    for j, t in enumerate(ts):
        p = j * nr * nc // len(ts)
        cells[p] = jnp.maximum(cells[p], t) if p in cells else t
    out = []
    for p in range(nr):
        row = []
        for c in range(nc):
            v = a[8 * p:8 * p + 8, 128 * c:128 * c + 128]
            t = cells.get(p * nc + c)
            if t is not None:
                v = jnp.where(never, t if t.dtype == a.dtype else pltpu.bitcast(t, a.dtype), v)
            row.append(v)
        out.append(cols(*row))
    return rows(*out)


def quad(w):
    n, m = w.shape[0] // 2, w.shape[1] // 2
    return [[w[i * n:(i + 1) * n, j * m:(j + 1) * m] for j in range(2)] for i in range(2)]


DEFAULTS = {
    1: dict(VCH=(2, 2, 2, 2), CR=72, T2=True, SK=3, CQ=(1, 2), U0=1, UK=3, UG=2,
            PA=(5, 6), PW=(2, 7), CJ=(0, 0, 3, 3, 3, 3, 2, 2), CW=(0, 2), US=0, USK=4, UJ=1, UW=(0, 7), YM=False),
    2: dict(VCH=(2, 2, 4), CR=72, T2=False, SK=3, CQ=(1, 1, 2), U0=0, UK=2, UG=2,
            PA=(5, 6), PW=(5, 7), CJ=(0, 2, 6), CW=(2, 4), US=0, USK=2, UJ=1, UW=(1, 3), YM=True),
}


def make(H=144, C=256, LV=2, FLAGS=None, FO=(3, 1, 6, 2, 0, 4, 5), QB=False, LF=1, QO=(0, 5, 6, 1, 3, 2, 4), STG=False, L0=1, LE=12, GR=24, GH=False, G0=2, GE=7, **kw):
    cfg = dict(DEFAULTS[LV], **kw)
    VCH, CR, T2, SK, CQ, U0, UK, UG = (cfg[k] for k in "VCH CR T2 SK CQ U0 UK UG".split())
    PA, PW, CJ, CW, US, USK, UJ, UW, YM = (cfg[k] for k in "PA PW CJ CW US USK UJ UW YM".split())
    NX = 32
    def kern(x_hbm, wq_hbm, wk_hbm, wv_hbm, wao_hbm, wup_hbm, dw_hbm, wdn_hbm, wm_hbm,
             o_hbm,
             x_v, wq, wk, wup, dwv, wa, wb,
             wp_s, wf_s, xa_s, x_s, qc_s, g_s, dw_s, ob_s,
             wsem, xsem, osem, *, B, TQ, D, K, NP):
        NL = D // 128
        pad = K // 2
        nb = -(-TQ // H)
        HL = TQ - (nb - 1) * H
        H2 = H // 2

        wc = {n: pltpu.make_async_copy(s, d, wsem.at[k]) for k, (n, s, d) in enumerate(
            [("v", wv_hbm, wa.at[0]), ("ao", wao_hbm, wb.at[0]), ("m0", wm_hbm.at[0:D], wb.at[1]),
             ("dn", wdn_hbm, wa.at[2]), ("m1", wm_hbm.at[D:2 * D], wb.at[2]),
             ("q", wq_hbm, wq), ("k", wk_hbm, wk), ("up", wup_hbm, wup), ("dw", dw_hbm, dwv)])}
        cuts = [0, 2 * H, 4 * H, 6 * H, TQ]
        xc = [pltpu.make_async_copy(x_hbm.at[0, :, pl.ds(a, e - a), :], x_v.at[0, :, pl.ds(a, e - a), :], xsem.at[n])
              for n, (a, e) in enumerate(zip(cuts[:-1], cuts[1:]))]
        xrest = pltpu.make_async_copy(x_hbm.at[pl.ds(1, B - 1)], x_v.at[pl.ds(1, B - 1), :, pl.ds(0, TQ), :],
                                      xsem.at[len(xc)])

        def set_proj(n, w):
            for k, v in enumerate(beta(quad(w))):
                wp_s[n, k] = pk(v)

        def proj(n, r0, first=lambda k, v: v):
            r2_ = r0 // 2 if isinstance(r0, int) else pl.multiple_of(r0 // 2, 8)
            return gamma([_dot(up(first(k, rows(x_s[2 * k, pl.ds(r2_, H2), :], x_s[2 * k + 1, pl.ds(r2_, H2), :]))),
                               up(wp_s[n, k])) for k in range(7)])

        for c in (wc["q"], wc["k"], xc[0]):
            c.start()
        for b in range(B):
            for h in range(4):
                x_v[b, h, TQ:, :] = jnp.zeros((nb * H - TQ, D), x_v.dtype)
        for k in range(NX):
            x_s[k, nb * H2:, :] = jnp.zeros((NP // 2 - nb * H2, D // 2), i32)
        for c in range(NL):
            for h in range(4):
                g_s[nb, h, c, HALO + H:, :] = jnp.zeros((HALO, 128), f32)
            dw_s[c] = jnp.zeros((32, 128), f32)
        for c in (wc["q"], wc["k"]):
            c.wait()
        for c in (xc[1], wc["up"], wc["dw"]):
            c.start()
        set_proj(0, _dot(wq[...], wk[...], NT) * (LOG2E * D ** -0.5))
        xc[2].start()

        def normalize(b, r, n):
            rr = pl.ds(pl.multiple_of(r, 16), n)
            for h in range(4):
                xa_s[b, h, rr, :] = _ln(x_v[b, h, rr, :].astype(f32)).astype(bf)

        @pl.loop(0, nb)
        def _(i):
            for k in range(len(xc)):
                @pl.when(i * H == cuts[k])
                def _():
                    if k == 2:
                        for c in (wc["up"], wc["dw"]):
                            c.wait()
                        set_proj(1, wup[:, 0:D].astype(f32))
                        set_proj(2, wup[:, D:2 * D].astype(f32))
                        for c in range(NL):
                            dw_s[c, 0:K, :] = dwv[:, c * 128:(c + 1) * 128].astype(f32) * 0.5
                    xc[k].wait()
                    for c in ((), (xc[3],), (), (wc["v"], wc["ao"], wc["m0"], wc["dn"], wc["m1"], xrest))[k]:
                        c.start()
            normalize(0, i * H, H)

        def prepare(b):
            @pl.loop(0, nb)
            def _(i):
                r = pl.multiple_of(i * H, 16)
                dst = pl.ds(pl.multiple_of(i * H2, 8), H2)
                never = i < 0
                zero8 = pl.multiple_of(jnp.minimum(i, 0), 8)
                x1, xq, left = [], [], None
                for a in range(7):
                    ra = pl.multiple_of(r + jnp.minimum(i + a, 0), 16) if STG else r
                    tile = lambda h, c: xa_s[b, h, pl.ds(ra, H), (c // 2) * 256:(c // 2 + 1) * 256].astype(f32)[
                        :, (c % 2) * 128:(c % 2 + 1) * 128]
                    l1 = [[alpha_one(a, lambda r1, c1: tile(2 * r1 + r2, 2 * c1 + c2)) for c2 in range(2)]
                          for r2 in range(2)]
                    x1.append([pk(cols(*l1[r2])) for r2 in range(2)])
                    for r2 in range(2):
                        x_s[2 * a + r2, dst, :] = x1[a][r2]
                    l2 = [v for k, v in enumerate(alpha(l1)) if k not in (2, 3)]
                    if left is not None:
                        l2 = [left] + l2
                    left = l2.pop() if len(l2) % 2 else None
                    if a == 6:
                        l2 += [left, left]
                    for k in range(len(l2) // 2):
                        x_s[14 + 5 * a // 2 + k, dst, :] = pk(cols(l2[2 * k], l2[2 * k + 1]))
                    xq.append([pltpu.bitcast(x_s[0, pl.ds(zero8, 8), :128], f32)])
                xq = [[]] * L0 + spread(xq, LE - L0) + [[]] * (14 - LE)
                xq = [sum(v, []) for v in xq]
                def pr(n, ts, order=range(7)):
                    res = [None] * 7
                    for j, k in enumerate(order):
                        res[k] = _dot(up(tie(never, rows(*x1[k]), ts[j])), up(wp_s[n, k]))
                    return gamma(res)
                gpre = unlvl1(pr(2, xq))
                gq = []
                for p in range(0, H, GR):
                    for h in range(4):
                        gg = _ln(_gelu2(cols(*[t[p:p + GR] for t in gpre[h]])), 4e-5)
                        for c in range(NL):
                            t = gg[:, c * 128:(c + 1) * 128]
                            g_s[i + 1, h, c, HALO + p:HALO + p + GR, :] = t
                            if p < HALO:
                                g_s[i, h, c, HALO + H + p:HALO + H + min(p + GR, HALO), :] = t[:HALO - p]
                            if p + GR > H - HALO:
                                o = max(H - HALO - p, 0)
                                g_s[i + 2, h, c, p + o - (H - HALO):p + GR - (H - HALO), :] = t[o:]
                        if GH or h == 3:
                            gq.append(g_s[i + 1, 0, 0, pl.ds(zero8 + HALO, 8), :])
                gq = [[]] * G0 + spread(gq, GE - G0) + [[]] * (7 - GE)
                qn = beta(tr(pr(0, [gq[k] + xq[7 + k] for k in range(7)], QO)))
                for k in range(7):
                    qc_s[i, k] = qn[k].astype(bf) if QB else pk(qn[k])

            zero = jnp.zeros((HALO, 128), f32)
            for c in range(NL):
                for h in range(4):
                    g_s[nb, h, c, HALO + HL:2 * HALO + HL, :] = g_s[1, h + 1, c, HALO:2 * HALO, :] if h < 3 else zero
                    g_s[1, h, c, 0:HALO, :] = g_s[nb, h - 1, c, HL:HL + HALO, :] if h else zero

        def merge_weights():
            for n in ("v", "ao", "m0", "dn", "m1"):
                wc[n].wait()

            @pl.loop(0, 3)
            def _(n):
                w = _dot(wa[n], wb[n])
                for b in range(1, B):
                    normalize(b, n * (nb * H // 3), nb * H // 3)

                @pl.when(n == 0)
                def _():
                    wa[1] = w.astype(bf)

                @pl.when(n > 0)
                def _():
                    if LF == 1:
                        for k, v in enumerate(beta(quad(w))):
                            wf_s[k, pl.ds(pl.multiple_of((n - 1) * (D // 4), 8), D // 4), :] = pk(v)
                    else:
                        g = [[w[a * 128:(a + 1) * 128, c * 128:(c + 1) * 128] for c in range(4)] for a in range(4)]
                        t = [v for row in two(beta, g) for v in row]
                        for k in range(25):
                            wf_s[k, pl.ds(pl.multiple_of((n - 1) * (D // 8), 8), D // 8), :] = pk(
                                cols(t[2 * k], t[min(2 * k + 1, 48)]))

        def ocopy(ob, b, r, n):
            return pltpu.make_async_copy(ob_s.at[ob, :, pl.ds(0, n), :], o_hbm.at[b, :, pl.ds(r, n), :], osem.at[ob])

        @jax.named_scope("step")
        def step(b, i):
            r = pl.multiple_of(i * H, 16)
            never = i < 0
            it = b * nb + i
            ob = it % 2
            short = (i == 1) & (b > 0)
            pl.when(short)(lambda: ocopy(ob, 0, 0, HL).wait())
            pl.when((it > 1) & jnp.logical_not(short))(lambda: ocopy(ob, 0, 0, H).wait())

            cv = [[None] * NL for _ in range(4)]
            convq = []
            for h in range(4):
                for c in range(NL):
                    w = dw_s[c]
                    ps = []
                    for rr in range(0, H, CR):
                        acc = None
                        for tt in sorted(range(K), key=lambda t: (t % 8, t)):
                            term = g_s[i + 1, h, c, pl.ds(rr + HALO - pad + tt, CR), :] * w[tt:tt + 1, :]
                            acc = term if acc is None else acc + term
                        ps.append(acc)
                        convq.append(toks(acc))
                    cv[h][c] = rows(*ps)

            qch = [(r2, j) for j in range(NP // C) for r2 in range(2)]
            qc = [pltpu.bitcast(qc_s[i, k], i32) if QB else qc_s[i, k] for k in range(7)]
            E = [[[None] * (NP // 128) for _ in range(4)] for _ in range(4)]
            m = [None] * 4
            l = [None] * 4
            statq = []
            for jj, (r2, j) in enumerate(qch):
                ks = slice(j * C // 2, (j + 1) * C // 2)
                st = [[]] * SK + spread(statq, 7 - SK)
                mm = []
                for k in range(7):
                    ts = st[k] + sum(take(convq, CQ.count(k)), [])
                    mm.append(_dot(up(tie(never, qc[k], ts)), up(x_s[2 * k + r2, ks, :]), NT))
                z = unlvl1(tr(gamma(mm)))
                for h in range(4):
                    new = []
                    for c1 in range(2):
                        v = cols(z[h][2 * c1], z[h][2 * c1 + 1])
                        for t_ in range(C // 128):
                            tl = v[:, t_ * 128:(t_ + 1) * 128]
                            c0 = j * C + t_ * 128
                            if c0 + 128 > TQ:
                                tl = jnp.where(c0 + lax.broadcasted_iota(i32, (H, 128), 1) < TQ, tl, -jnp.inf)
                            new.append((2 * c1 + r2, c0 // 128, tl))
                    mx = functools.reduce(jnp.maximum, [v for _, _, v in new])
                    if m[h] is None:
                        mn, ln_ = mx, None
                    else:
                        mn = jnp.maximum(m[h], mx)
                        ln_ = l[h] * jnp.exp2(m[h] - mn)
                    for n, t_, tl in new:
                        e = jnp.exp2(tl - mn)
                        E[h][n][t_] = (e, mn) if T2 else tl
                        ln_ = e if ln_ is None else ln_ + e
                    m[h], l[h] = mn, ln_
                tl_ = [toks(v) for v in l]
                statq = [tl_[2 * r1 + a][p] for a in range(2) for p in range(H // 8) for r1 in range(2)]
            sh = []
            for h in range(4):
                mr = jnp.max(m[h], axis=-1, keepdims=True)
                lr = jnp.sum(l[h] * jnp.exp2(m[h] - mr), axis=-1, keepdims=True)
                sh.append(mr + jnp.log2(lr))
            corr = {}

            def prob(h, n, t_):
                if not T2:
                    return jnp.exp2(E[h][n][t_] - sh[h])
                e, mn = E[h][n][t_]
                if (h, id(mn)) not in corr:
                    corr[h, id(mn)] = jnp.exp2(mn - sh[h])
                return e * corr[h, id(mn)]

            vt = np.cumsum((0,) + tuple(VCH))
            vch = [(r2, vt[j], vt[j + 1]) for j in range(len(VCH)) for r2 in range(2 if LV == 1 else 1)]
            NPR = 7 ** LV

            def pv_ops(jj):
                r2, ta, te = vch[jj]
                pe = lambda h, n: cols(*[prob(h, n, t_) for t_ in range(ta, te)])
                if LV == 1:
                    pc = alpha([[rows(pe(2 * r1, 2 * c1 + r2), pe(2 * r1 + 1, 2 * c1 + r2)) for c1 in range(2)]
                                for r1 in range(2)])
                    return pc, [pc[a][p:p + 8, t_ * 128:(t_ + 1) * 128]
                                for p in range(0, 2 * H, 8) for t_ in range(te - ta) for a in PA]
                g = [[pe(h, n) for n in range(4)] for h in range(4)]
                if not YM:
                    l1 = [[alpha([[g[2 * r1 + r_][2 * c1 + c2] for c1 in range(2)] for r1 in range(2)])
                           for c2 in range(2)] for r_ in range(2)]
                    pc = [v for a in range(7) for v in alpha([[l1[r_][c2][a] for c2 in range(2)] for r_ in range(2)])]
                    return pc, [l1[r_][c2][a][p:p + 8, t_ * 128:(t_ + 1) * 128] for p in range(0, H, 8)
                                for r_ in range(2) for c2 in range(2) for t_ in range(te - ta) for a in PA]
                return alpha2_direct(g), [g[h][n][p:p + 8, t_ * 128:(t_ + 1) * 128] for p in range(0, H, 8)
                                          for h in range(4) for n in range(4) for t_ in range(te - ta)]

            def pv_rhs(jj, k):
                r2, ta, te = vch[jj]
                ks = slice(ta * 64, te * 64)
                if LV == 1:
                    return x_s[2 * PERM[k] + r2, ks, :]
                a, k = PERM[k // 7], PERM[k % 7]
                n = 4 * a if k == 2 else 4 * a + 3 if k == 3 else 28 + 5 * a + (k if k < 2 else k - 2)
                return x_s[n // 2, ks, (n % 2) * 128:(n % 2 + 1) * 128]

            pc, pq = pv_ops(0)
            st = [[]] * U0 + spread(statq, UK) + [[]] * (7 - UK - U0)
            pp = [[]] * (7 - UG) + spread(pq, UG) if UG else [[]] * 7
            upre = unlvl1(proj(1, r, lambda k, v: tie(never, v, st[k] + pp[k])))
            u, uq = None, []

            acc = [None] * NPR
            nv = len(vch)
            f7 = NPR // 7
            win = lambda q, a, e: [[]] * (a * f7) + spread(q, (e - a) * f7) + [[]] * ((7 - e) * f7)
            assert US < UJ < nv
            for jj in range(nv):
                pcn, pq = pv_ops(jj + 1) if jj + 1 < nv else (None, [])
                pp = win(pq, *PW)
                ug = win(uq if jj == UJ else [], *UW)
                cg = win(take(convq, CJ[jj]), *CW)
                for k in range(NPR):
                    ts = pp[k] + ug[k] + sum(cg[k], [])
                    d = _dot(tie(never, pc[k], ts).astype(bf), up(pv_rhs(jj, k)))
                    if k == USK * f7:
                        d0 = d
                    acc[k] = d if acc[k] is None else acc[k] + d
                pc = pcn
                if jj == US:
                    u = [[_gelu2(jnp.where(never, d0[:H, :128], upre[h][c])) for c in range(4)] for h in range(4)]
                    uq = [t for row in u for v in row for t in toks(v)]
            o4 = gamma2([acc[7 * a:7 * a + 7] for a in range(7)])
            o = lvl1(o4)
            uc = [[u[h][c] * cv[h][c] for c in range(4)] for h in range(4)]
            ao, au = alpha(o), alpha(lvl1(uc))

            if LF == 1:
                fo = [None] * 7
                for k in FO:
                    fo[k] = _dot(cols(ao[k], au[k]).astype(bf), up(wf_s[k]))
                out = unlvl1(gamma(fo))
            else:
                f2 = alpha2_direct if LF == 3 else (lambda g: [v for row in two(alpha, g) for v in row])
                ao, au = f2(o4), f2(uc)
                fo = [[None] * 7 for _ in range(7)]
                for a in FO:
                    for k in FO:
                        n = 7 * a + k
                        fo[a][k] = _dot(cols(ao[n], au[n]).astype(bf),
                                        up(wf_s[n // 2, :, (n % 2) * 128:(n % 2 + 1) * 128]))
                out = gamma2(fo)
            for h in range(4):
                ob_s[ob, h] = (x_v[b, h, pl.ds(r, H), :].astype(f32) + cols(*out[h])).astype(ob_s.dtype)
            pl.when(i < nb - 1)(lambda: ocopy(ob, b, r, H).start())
            pl.when(i == nb - 1)(lambda: ocopy(ob, b, r, HL).start())

        @pl.loop(0, B)
        def _(b):
            pl.when(b == 1)(lambda: xrest.wait())
            prepare(b)
            pl.when(b == 0)(merge_weights)
            pl.loop(0, nb)(functools.partial(step, b))

        ocopy((B * nb) % 2, 0, 0, H).wait()
        ocopy((B * nb + 1) % 2, 0, 0, HL).wait()

    @jax.jit
    def fn(x, w_q, w_k, w_v, w_ao, w_up, dw, w_dn, w_merge):
        B, T, D = x.shape
        K = dw.shape[0]
        TQ = T // 4
        TP = -(-TQ // H) * H
        NP = 128 * sum(VCH)
        assert NP >= TP + HALO and NP % C == 0
        ws = (w_q, w_k, w_v, w_ao, w_up, dw, w_dn, w_merge)
        anyspec = pl.BlockSpec(memory_space=pl.ANY)
        out = pl.pallas_call(
            functools.partial(kern, B=B, TQ=TQ, D=D, K=K, NP=NP),
            in_specs=[anyspec] * 9,
            out_specs=anyspec,
            out_shape=jax.ShapeDtypeStruct((B, 4, TQ, D), x.dtype),
            scratch_shapes=[pltpu.VMEM((B, 4, TP, D), x.dtype)] + [
                pltpu.VMEM(w.shape, w.dtype) for w in (w_q, w_k, w_up, dw)] + [
                pltpu.VMEM((3, D, D), bf),
                pltpu.VMEM((3, D, D), bf),
                pltpu.VMEM((3, 7, D // 4, D // 2), i32),
                pltpu.VMEM((7, D // 2, D // 2) if LF == 1 else (25, D // 4, D // 2), i32),
                pltpu.VMEM((B, 4, TP, D), bf),
                pltpu.VMEM((NX, NP // 2, D // 2), i32),
                pltpu.VMEM((TP // H, 7, 2 * H, D // 2), bf) if QB else pltpu.VMEM((TP // H, 7, H, D // 2), i32),
                pltpu.VMEM((TP // H + 2, 4, D // 128, H + 2 * HALO, 128), f32),
                pltpu.VMEM((D // 128, 32, 128), f32),
                pltpu.VMEM((2, 4, H, D), x.dtype),
                pltpu.SemaphoreType.DMA((9,)),
                pltpu.SemaphoreType.DMA((5,)),
                pltpu.SemaphoreType.DMA((2,)),
            ],
            compiler_params=pltpu.CompilerParams(vmem_limit_bytes=112 * 1024 * 1024, flags=FLAGS),
        )(x.reshape(B, 4, TQ, D), *ws)
        return out.reshape(B, T, D)
    return fn


_impl = make()


def pallas_standalone__conformer_family_branchformer__speech_kernel(x, w_q, w_k, w_v, w_ao, w_up, dw, w_dn, w_merge):
    return _impl(x, w_q, w_k, w_v, w_ao, w_up, dw, w_dn, w_merge)
```

```python
import functools
import jax
import jax.numpy as jnp
import numpy as np
from jax import lax
import jax.experimental.pallas as pl
import jax.experimental.pallas.tpu as pltpu

LOG2E = 1.4426950408889634
NT = (((1,), (1,)), ((), ()))
NN = (((1,), (0,)), ((), ()))
bf = jnp.bfloat16
f32 = jnp.float32
i32 = jnp.int32
HALO = 16
PERM = (0, 2, 6, 5, 3, 4, 1)


def _ln(x, eps=1e-5):
    m = jnp.mean(x, axis=-1, keepdims=True)
    d = x - m
    v = jnp.mean(d * d, axis=-1, keepdims=True)
    return d * jnp.exp2(jnp.log(v + eps) * (-0.5 * LOG2E))


def _gelu2(x):
    c = float(np.sqrt(2.0 / np.pi))
    return x * jnp.tanh((x * x * (0.044715 * c) + c) * x) + x


def _dot(a, b, dims=NN):
    return lax.dot_general(a, b, dims, preferred_element_type=f32)


def rows(*p):
    return jnp.concatenate(p, axis=0)


def cols(*p):
    return jnp.concatenate(p, axis=1)


def pk(v):
    return pltpu.bitcast(v.astype(bf), i32)


def up(v):
    return pltpu.bitcast(v, bf)


def alpha(z):
    (a, b), (c, d) = z
    return [a + d, c + d, a, d, a + b, c - a, b - d]


def alpha_one(k, z):
    return [lambda: z(0, 0) + z(1, 1), lambda: z(1, 0) + z(1, 1), lambda: z(0, 0), lambda: z(1, 1),
            lambda: z(0, 0) + z(0, 1), lambda: z(1, 0) - z(0, 0), lambda: z(0, 1) - z(1, 1)][k]()


def beta(z):
    t = alpha(z)
    return [t[k] for k in PERM]


def gamma(n):
    return [[n[0] + n[3] - n[4] + n[6], n[2] + n[4]], [n[1] + n[3], n[0] - n[1] + n[2] + n[5]]]


def tr(z):
    return [list(r) for r in zip(*z)]


def lvl1(g):
    return [[rows(*[cols(g[2 * r1 + r2][2 * c1], g[2 * r1 + r2][2 * c1 + 1]) for r2 in range(2)])
             for c1 in range(2)] for r1 in range(2)]


def unlvl1(z):
    out = [[None] * 4 for _ in range(4)]
    for r1 in range(2):
        for c1 in range(2):
            v = z[r1][c1]
            n, m = v.shape[0] // 2, v.shape[1] // 2
            for r2 in range(2):
                for c2 in range(2):
                    out[2 * r1 + r2][2 * c1 + c2] = v[r2 * n:(r2 + 1) * n, c2 * m:(c2 + 1) * m]
    return out


def two(f, g):
    l1 = [[f([[g[2 * r1 + r2][2 * c1 + c2] for c1 in range(2)] for r1 in range(2)])
           for c2 in range(2)] for r2 in range(2)]
    return [f([[l1[r2][c2][a] for c2 in range(2)] for r2 in range(2)]) for a in range(7)]


def alpha2_direct(g):
    terms = [[(0, 0, 1), (1, 1, 1)], [(1, 0, 1), (1, 1, 1)], [(0, 0, 1)], [(1, 1, 1)],
             [(0, 0, 1), (0, 1, 1)], [(1, 0, 1), (0, 0, -1)], [(0, 1, 1), (1, 1, -1)]]

    def pair(u, v):
        (x, sx), (y, sy) = u, v
        if sx > 0:
            return (x + y if sy > 0 else x - y), 1
        return (y - x, 1) if sy > 0 else (x + y, -1)

    out = []
    for a in range(7):
        for k in range(7):
            t = [[(g[2 * r1 + r2][2 * c1 + c2], s1 * s2) for r2, c2, s2 in terms[k]] for r1, c1, s1 in terms[a]]
            if len(t) == 2 and len(t[0]) == 2:
                v, sign = pair(pair(t[0][0], t[1][1]), pair(t[0][1], t[1][0]))
            else:
                f = [e for row in t for e in row]
                v, sign = pair(*f) if len(f) == 2 else f[0]
            assert sign > 0
            out.append(v)
    return out


def gamma2(n):
    inner = [gamma(n[a]) for a in range(7)]
    out = [[None] * 4 for _ in range(4)]
    for r2 in range(2):
        for c2 in range(2):
            z = gamma([inner[a][r2][c2] for a in range(7)])
            for r1 in range(2):
                for c1 in range(2):
                    out[2 * r1 + r2][2 * c1 + c2] = z[r1][c1]
    return out


def toks(a):
    return [a[k:k + 8, :128] for k in range(0, a.shape[0], 8)]


def take(q, n):
    out = q[:n]
    del q[:n]
    return out


def spread(q, n):
    q0 = list(q)
    del q[:]
    return [q0[k * len(q0) // n:(k + 1) * len(q0) // n] for k in range(n)]


def tie(never, a, ts):
    if not ts:
        return a
    nr, nc = a.shape[0] // 8, a.shape[1] // 128
    cells = {}
    for j, t in enumerate(ts):
        p = j * nr * nc // len(ts)
        cells[p] = jnp.maximum(cells[p], t) if p in cells else t
    out = []
    for p in range(nr):
        row = []
        for c in range(nc):
            v = a[8 * p:8 * p + 8, 128 * c:128 * c + 128]
            t = cells.get(p * nc + c)
            if t is not None:
                v = jnp.where(never, t if t.dtype == a.dtype else pltpu.bitcast(t, a.dtype), v)
            row.append(v)
        out.append(cols(*row))
    return rows(*out)


def quad(w):
    n, m = w.shape[0] // 2, w.shape[1] // 2
    return [[w[i * n:(i + 1) * n, j * m:(j + 1) * m] for j in range(2)] for i in range(2)]


DEFAULTS = {
    1: dict(VCH=(2, 2, 2, 2), CR=72, T2=True, SK=3, CQ=(1, 2), U0=1, UK=3, UG=2,
            PA=(5, 6), PW=(2, 7), CJ=(0, 0, 3, 3, 3, 3, 2, 2), CW=(0, 2), US=0, USK=4, UJ=1, UW=(0, 7), YM=False),
    2: dict(VCH=(2, 2, 4), CR=72, T2=False, SK=3, CQ=(1, 1, 2), U0=0, UK=1, UG=2,
            PA=(5, 6), PW=(3, 7), CJ=(0, 2, 6), CW=(2, 4), US=0, USK=2, UJ=1, UW=(1, 3), YM=True),
}


def make(H=144, C=256, LV=2, FLAGS=None, FO=(3, 1, 6, 2, 4, 0, 5), QB=False, LF=1, MR=48, M0=1, ME=12, KO=(0, 1, 2, 3, 4, 5, 6), UO=(1, 3, 2, 4, 0, 5, 6), CQ0=(1, 1, 2), CQL=(1, 1, 2), PW1=None, CW2=None, UC=(), QO=(0, 5, 6, 2, 4, 1, 3), STG=False, L0=1, LE=12, GR=24, GH=False, G0=2, GE=7, **kw):
    cfg = dict(DEFAULTS[LV], **kw)
    VCH, CR, T2, SK, CQ, U0, UK, UG = (cfg[k] for k in "VCH CR T2 SK CQ U0 UK UG".split())
    PA, PW, CJ, CW, US, USK, UJ, UW, YM = (cfg[k] for k in "PA PW CJ CW US USK UJ UW YM".split())
    NX = 32
    def kern(x_hbm, wq_hbm, wk_hbm, wv_hbm, wao_hbm, wup_hbm, dw_hbm, wdn_hbm, wm_hbm,
             o_hbm,
             x_v, wq, wk, wup, dwv, wa, wb,
             wp_s, wf_s, xa_s, x_s, qc_s, g_s, dw_s, ob_s,
             wsem, xsem, osem, *, B, TQ, D, K, NP):
        NL = D // 128
        pad = K // 2
        nb = -(-TQ // H)
        HL = TQ - (nb - 1) * H
        H2 = H // 2

        wc = {n: pltpu.make_async_copy(s, d, wsem.at[k]) for k, (n, s, d) in enumerate(
            [("v", wv_hbm, wa.at[0]), ("ao", wao_hbm, wb.at[0]), ("m0", wm_hbm.at[0:D], wb.at[1]),
             ("dn", wdn_hbm, wa.at[2]), ("m1", wm_hbm.at[D:2 * D], wb.at[2]),
             ("q", wq_hbm, wq), ("k", wk_hbm, wk), ("up", wup_hbm, wup), ("dw", dw_hbm, dwv)])}
        cuts = [0, 2 * H, 4 * H, 6 * H, TQ]
        xc = [pltpu.make_async_copy(x_hbm.at[0, :, pl.ds(a, e - a), :], x_v.at[0, :, pl.ds(a, e - a), :], xsem.at[n])
              for n, (a, e) in enumerate(zip(cuts[:-1], cuts[1:]))]
        xrest = pltpu.make_async_copy(x_hbm.at[pl.ds(1, B - 1)], x_v.at[pl.ds(1, B - 1), :, pl.ds(0, TQ), :],
                                      xsem.at[len(xc)])

        def set_proj(n, w):
            for k, v in enumerate(beta(quad(w))):
                wp_s[n, k] = pk(v)

        def proj(n, r0, first=lambda k, v: v):
            r2_ = r0 // 2 if isinstance(r0, int) else pl.multiple_of(r0 // 2, 8)
            res = [None] * 7
            for j, k in enumerate(UO):
                res[k] = _dot(up(first(j, rows(x_s[2 * k, pl.ds(r2_, H2), :], x_s[2 * k + 1, pl.ds(r2_, H2), :]))),
                              up(wp_s[n, k]))
            return gamma(res)

        for c in (wc["q"], wc["k"], xc[0]):
            c.start()
        for b in range(B):
            for h in range(4):
                x_v[b, h, TQ:, :] = jnp.zeros((nb * H - TQ, D), x_v.dtype)
        for k in range(NX):
            x_s[k, nb * H2:, :] = jnp.zeros((NP // 2 - nb * H2, D // 2), i32)
        for c in range(NL):
            for h in range(4):
                g_s[nb, h, c, HALO + H:, :] = jnp.zeros((HALO, 128), f32)
            dw_s[c] = jnp.zeros((32, 128), f32)
        for c in (wc["q"], wc["k"]):
            c.wait()
        for c in (xc[1], wc["up"], wc["dw"]):
            c.start()
        set_proj(0, _dot(wq[...], wk[...], NT) * (LOG2E * D ** -0.5))
        xc[2].start()

        def normalize(b, r, n):
            rr = pl.ds(r if isinstance(r, int) else pl.multiple_of(r, 16), n)
            for h in range(4):
                xa_s[b, h, rr, :] = _ln(x_v[b, h, rr, :].astype(f32)).astype(bf)

        @pl.loop(0, nb)
        def _(i):
            for k in range(len(xc)):
                @pl.when(i * H == cuts[k])
                def _():
                    if k == 2:
                        for c in (wc["up"], wc["dw"]):
                            c.wait()
                        set_proj(1, wup[:, 0:D].astype(f32))
                        set_proj(2, wup[:, D:2 * D].astype(f32))
                        for c in range(NL):
                            dw_s[c, 0:K, :] = dwv[:, c * 128:(c + 1) * 128].astype(f32) * 0.5
                    xc[k].wait()
                    for c in ((), (xc[3],), (), (wc["v"], wc["ao"], wc["m0"], wc["dn"], wc["m1"], xrest))[k]:
                        c.start()
            normalize(0, i * H, H)

        def prepare(b):
            @pl.loop(0, nb)
            def _(i):
                r = pl.multiple_of(i * H, 16)
                dst = pl.ds(pl.multiple_of(i * H2, 8), H2)
                never = i < 0
                zero8 = pl.multiple_of(jnp.minimum(i, 0), 8)
                x1, xq, left = [], [], None
                for a in range(7):
                    ra = pl.multiple_of(r + jnp.minimum(i + a, 0), 16) if STG else r
                    tile = lambda h, c: xa_s[b, h, pl.ds(ra, H), (c // 2) * 256:(c // 2 + 1) * 256].astype(f32)[
                        :, (c % 2) * 128:(c % 2 + 1) * 128]
                    l1 = [[alpha_one(a, lambda r1, c1: tile(2 * r1 + r2, 2 * c1 + c2)) for c2 in range(2)]
                          for r2 in range(2)]
                    x1.append([pk(cols(*l1[r2])) for r2 in range(2)])
                    for r2 in range(2):
                        x_s[2 * a + r2, dst, :] = x1[a][r2]
                    l2 = [v for k, v in enumerate(alpha(l1)) if k not in (2, 3)]
                    if left is not None:
                        l2 = [left] + l2
                    left = l2.pop() if len(l2) % 2 else None
                    if a == 6:
                        l2 += [left, left]
                    for k in range(len(l2) // 2):
                        x_s[14 + 5 * a // 2 + k, dst, :] = pk(cols(l2[2 * k], l2[2 * k + 1]))
                    xq.append([pltpu.bitcast(x_s[0, pl.ds(zero8, 8), :128], f32)])
                xq = [[]] * L0 + spread(xq, LE - L0) + [[]] * (14 - LE)
                xq = [sum(v, []) for v in xq]
                def pr(n, ts, order=range(7)):
                    res = [None] * 7
                    for j, k in enumerate(order):
                        res[k] = _dot(up(tie(never, rows(*x1[k]), ts[j])), up(wp_s[n, k]))
                    return gamma(res)
                gpre = unlvl1(pr(2, xq))
                gq = []
                for p in range(0, H, GR):
                    for h in range(4):
                        gg = _ln(_gelu2(cols(*[t[p:p + GR] for t in gpre[h]])), 4e-5)
                        for c in range(NL):
                            t = gg[:, c * 128:(c + 1) * 128]
                            g_s[i + 1, h, c, HALO + p:HALO + p + GR, :] = t
                            if p < HALO:
                                g_s[i, h, c, HALO + H + p:HALO + H + min(p + GR, HALO), :] = t[:HALO - p]
                            if p + GR > H - HALO:
                                o = max(H - HALO - p, 0)
                                g_s[i + 2, h, c, p + o - (H - HALO):p + GR - (H - HALO), :] = t[o:]
                        if GH or h == 3:
                            gq.append(g_s[i + 1, 0, 0, pl.ds(zero8 + HALO, 8), :])
                gq = [[]] * G0 + spread(gq, GE - G0) + [[]] * (7 - GE)
                qn = beta(tr(pr(0, [gq[k] + xq[7 + k] for k in range(7)], QO)))
                for k in range(7):
                    qc_s[i, k] = qn[k].astype(bf) if QB else pk(qn[k])

            zero = jnp.zeros((HALO, 128), f32)
            for c in range(NL):
                for h in range(4):
                    g_s[nb, h, c, HALO + HL:2 * HALO + HL, :] = g_s[1, h + 1, c, HALO:2 * HALO, :] if h < 3 else zero
                    g_s[1, h, c, 0:HALO, :] = g_s[nb, h - 1, c, HL:HL + HALO, :] if h else zero

        def merge_weights(b0):
            for n in ("v", "ao", "m0", "dn", "m1"):
                wc[n].wait()

            zero16 = pl.multiple_of(jnp.minimum(b0, 0), 16)
            tq = []
            for b in range(1, B):
                for p in range(0, nb * H, MR):
                    normalize(b, p, MR)
                    tq.append(pltpu.bitcast(xa_s[b, 0, pl.ds(zero16, 16), :128], i32))
            tq = [[]] * M0 + spread(tq, ME - M0) + [[]] * (12 - ME)

            def product(n, a, w_ref):
                return cols(*[_dot(up(tie(b0 < 0, a, tq[4 * n + c])), w_ref[:, c * 128:(c + 1) * 128]) for c in range(4)])

            t = product(0, pltpu.bitcast(wa[0], i32), wb.at[0])
            for k, v in enumerate(beta(quad(product(1, pltpu.bitcast(wa[2], i32), wb.at[2])))):
                wf_s[k, D // 4:, :] = pk(v)
            tq[11].append(wf_s[0, pl.ds(zero16, 8), :128])
            for k, v in enumerate(beta(quad(product(2, pk(t), wb.at[1])))):
                wf_s[k, :D // 4, :] = pk(v)

        def ocopy(ob, b, r, n):
            return pltpu.make_async_copy(ob_s.at[ob, :, pl.ds(0, n), :], o_hbm.at[b, :, pl.ds(r, n), :], osem.at[ob])

        @jax.named_scope("step")
        def step(b, i):
            r = pl.multiple_of(i * H, 16)
            never = i < 0
            it = b * nb + i
            ob = it % 2
            short = (i == 1) & (b > 0)
            pl.when(short)(lambda: ocopy(ob, 0, 0, HL).wait())
            pl.when((it > 1) & jnp.logical_not(short))(lambda: ocopy(ob, 0, 0, H).wait())

            cv = [[None] * NL for _ in range(4)]
            convq = []
            for h in range(4):
                for c in range(NL):
                    w = dw_s[c]
                    ps = []
                    for rr in range(0, H, CR):
                        acc = None
                        for tt in sorted(range(K), key=lambda t: (t % 8, t)):
                            term = g_s[i + 1, h, c, pl.ds(rr + HALO - pad + tt, CR), :] * w[tt:tt + 1, :]
                            acc = term if acc is None else acc + term
                        ps.append(acc)
                        convq.append(toks(acc))
                    cv[h][c] = rows(*ps)

            qch = [(r2, j) for j in range(NP // C) for r2 in range(2)]
            qc = [pltpu.bitcast(qc_s[i, k], i32) if QB else qc_s[i, k] for k in range(7)]
            E = [[[None] * (NP // 128) for _ in range(4)] for _ in range(4)]
            m = [None] * 4
            l = [None] * 4
            statq = []
            for jj, (r2, j) in enumerate(qch):
                ks = slice(j * C // 2, (j + 1) * C // 2)
                st = [[]] * SK + spread(statq, 7 - SK)
                mm = [None] * 7
                cq = CQ0 if jj == 0 else CQL if jj == len(qch) - 1 else CQ
                for n_, k in enumerate(KO):
                    ts = st[n_] + sum(take(convq, cq.count(n_)), [])
                    mm[k] = (_dot(up(tie(never, qc[k], ts)), up(x_s[2 * k + r2, ks, :]), NT))
                z = unlvl1(tr(gamma(mm)))
                for h in range(4):
                    new = []
                    for c1 in range(2):
                        v = cols(z[h][2 * c1], z[h][2 * c1 + 1])
                        for t_ in range(C // 128):
                            tl = v[:, t_ * 128:(t_ + 1) * 128]
                            c0 = j * C + t_ * 128
                            if c0 + 128 > TQ:
                                tl = jnp.where(c0 + lax.broadcasted_iota(i32, (H, 128), 1) < TQ, tl, -jnp.inf)
                            new.append((2 * c1 + r2, c0 // 128, tl))
                    mx = functools.reduce(jnp.maximum, [v for _, _, v in new])
                    if m[h] is None:
                        mn, ln_ = mx, None
                    else:
                        mn = jnp.maximum(m[h], mx)
                        ln_ = l[h] * jnp.exp2(m[h] - mn)
                    for n, t_, tl in new:
                        e = jnp.exp2(tl - mn)
                        E[h][n][t_] = (e, mn) if T2 else tl
                        ln_ = e if ln_ is None else ln_ + e
                    m[h], l[h] = mn, ln_
                tl_ = [toks(v) for v in l]
                statq = [tl_[2 * r1 + a][p] for a in range(2) for p in range(H // 8) for r1 in range(2)]
            sh = []
            for h in range(4):
                mr = jnp.max(m[h], axis=-1, keepdims=True)
                lr = jnp.sum(l[h] * jnp.exp2(m[h] - mr), axis=-1, keepdims=True)
                sh.append(mr + jnp.log2(lr))
            corr = {}

            def prob(h, n, t_):
                if not T2:
                    return jnp.exp2(E[h][n][t_] - sh[h])
                e, mn = E[h][n][t_]
                if (h, id(mn)) not in corr:
                    corr[h, id(mn)] = jnp.exp2(mn - sh[h])
                return e * corr[h, id(mn)]

            vt = np.cumsum((0,) + tuple(VCH))
            vch = [(r2, vt[j], vt[j + 1]) for j in range(len(VCH)) for r2 in range(2 if LV == 1 else 1)]
            NPR = 7 ** LV

            def pv_ops(jj):
                r2, ta, te = vch[jj]
                pe = lambda h, n: cols(*[prob(h, n, t_) for t_ in range(ta, te)])
                if LV == 1:
                    pc = alpha([[rows(pe(2 * r1, 2 * c1 + r2), pe(2 * r1 + 1, 2 * c1 + r2)) for c1 in range(2)]
                                for r1 in range(2)])
                    return pc, [pc[a][p:p + 8, t_ * 128:(t_ + 1) * 128]
                                for p in range(0, 2 * H, 8) for t_ in range(te - ta) for a in PA]
                g = [[pe(h, n) for n in range(4)] for h in range(4)]
                if not YM:
                    l1 = [[alpha([[g[2 * r1 + r_][2 * c1 + c2] for c1 in range(2)] for r1 in range(2)])
                           for c2 in range(2)] for r_ in range(2)]
                    pc = [v for a in range(7) for v in alpha([[l1[r_][c2][a] for c2 in range(2)] for r_ in range(2)])]
                    return pc, [l1[r_][c2][a][p:p + 8, t_ * 128:(t_ + 1) * 128] for p in range(0, H, 8)
                                for r_ in range(2) for c2 in range(2) for t_ in range(te - ta) for a in PA]
                return alpha2_direct(g), [g[h][n][p:p + 8, t_ * 128:(t_ + 1) * 128] for p in range(0, H, 8)
                                          for h in range(4) for n in range(4) for t_ in range(te - ta)]

            def pv_rhs(jj, k):
                r2, ta, te = vch[jj]
                ks = slice(ta * 64, te * 64)
                if LV == 1:
                    return x_s[2 * PERM[k] + r2, ks, :]
                a, k = PERM[k // 7], PERM[k % 7]
                n = 4 * a if k == 2 else 4 * a + 3 if k == 3 else 28 + 5 * a + (k if k < 2 else k - 2)
                return x_s[n // 2, ks, (n % 2) * 128:(n % 2 + 1) * 128]

            pc, pq = pv_ops(0)
            st = [[]] * U0 + spread(statq, UK) + [[]] * (7 - UK - U0)
            pp = [[]] * (7 - UG) + spread(pq, UG) if UG else [[]] * 7
            upre = unlvl1(proj(1, r, lambda k, v: tie(never, v, st[k] + pp[k] + sum(take(convq, UC.count(k)), []))))
            u, uq = None, []

            acc = [None] * NPR
            nv = len(vch)
            f7 = NPR // 7
            win = lambda q, a, e: [[]] * (a * f7) + spread(q, (e - a) * f7) + [[]] * ((7 - e) * f7)
            assert US < UJ < nv
            for jj in range(nv):
                pcn, pq = pv_ops(jj + 1) if jj + 1 < nv else (None, [])
                pp = win(pq, *(PW1 if jj == 1 and PW1 else PW))
                ug = win(uq if jj == UJ else [], *UW)
                cg = win(take(convq, CJ[jj]), *(CW2 if jj == nv - 1 and CW2 else CW))
                for k in range(NPR):
                    ts = pp[k] + ug[k] + sum(cg[k], [])
                    d = _dot(tie(never, pc[k], ts).astype(bf), up(pv_rhs(jj, k)))
                    if k == USK * f7:
                        d0 = d
                    acc[k] = d if acc[k] is None else acc[k] + d
                pc = pcn
                if jj == US:
                    u = [[_gelu2(jnp.where(never, d0[:H, :128], upre[h][c])) for c in range(4)] for h in range(4)]
                    uq = [t for row in u for v in row for t in toks(v)]
            o4 = gamma2([acc[7 * a:7 * a + 7] for a in range(7)])
            o = lvl1(o4)
            uc = [[u[h][c] * cv[h][c] for c in range(4)] for h in range(4)]
            ao, au = alpha(o), alpha(lvl1(uc))

            if LF == 1:
                fo = [None] * 7
                for k in FO:
                    fo[k] = _dot(cols(ao[k], au[k]).astype(bf), up(wf_s[k]))
                out = unlvl1(gamma(fo))
            else:
                f2 = alpha2_direct if LF == 3 else (lambda g: [v for row in two(alpha, g) for v in row])
                ao, au = f2(o4), f2(uc)
                fo = [[None] * 7 for _ in range(7)]
                for a in FO:
                    for k in FO:
                        n = 7 * a + k
                        fo[a][k] = _dot(cols(ao[n], au[n]).astype(bf),
                                        up(wf_s[n // 2, :, (n % 2) * 128:(n % 2 + 1) * 128]))
                out = gamma2(fo)
            for h in range(4):
                ob_s[ob, h] = (x_v[b, h, pl.ds(r, H), :].astype(f32) + cols(*out[h])).astype(ob_s.dtype)
            pl.when(i < nb - 1)(lambda: ocopy(ob, b, r, H).start())
            pl.when(i == nb - 1)(lambda: ocopy(ob, b, r, HL).start())

        @pl.loop(0, B)
        def _(b):
            pl.when(b == 1)(lambda: xrest.wait())
            prepare(b)
            pl.when(b == 0)(lambda: merge_weights(b))
            pl.loop(0, nb)(functools.partial(step, b))

        ocopy((B * nb) % 2, 0, 0, H).wait()
        ocopy((B * nb + 1) % 2, 0, 0, HL).wait()

    @jax.jit
    def fn(x, w_q, w_k, w_v, w_ao, w_up, dw, w_dn, w_merge):
        B, T, D = x.shape
        K = dw.shape[0]
        TQ = T // 4
        TP = -(-TQ // H) * H
        NP = 128 * sum(VCH)
        assert NP >= TP + HALO and NP % C == 0
        ws = (w_q, w_k, w_v, w_ao, w_up, dw, w_dn, w_merge)
        anyspec = pl.BlockSpec(memory_space=pl.ANY)
        out = pl.pallas_call(
            functools.partial(kern, B=B, TQ=TQ, D=D, K=K, NP=NP),
            in_specs=[anyspec] * 9,
            out_specs=anyspec,
            out_shape=jax.ShapeDtypeStruct((B, 4, TQ, D), x.dtype),
            scratch_shapes=[pltpu.VMEM((B, 4, TP, D), x.dtype)] + [
                pltpu.VMEM(w.shape, w.dtype) for w in (w_q, w_k, w_up, dw)] + [
                pltpu.VMEM((3, D, D), bf),
                pltpu.VMEM((3, D, D), bf),
                pltpu.VMEM((3, 7, D // 4, D // 2), i32),
                pltpu.VMEM((7, D // 2, D // 2) if LF == 1 else (25, D // 4, D // 2), i32),
                pltpu.VMEM((B, 4, TP, D), bf),
                pltpu.VMEM((NX, NP // 2, D // 2), i32),
                pltpu.VMEM((TP // H, 7, 2 * H, D // 2), bf) if QB else pltpu.VMEM((TP // H, 7, H, D // 2), i32),
                pltpu.VMEM((TP // H + 2, 4, D // 128, H + 2 * HALO, 128), f32),
                pltpu.VMEM((D // 128, 32, 128), f32),
                pltpu.VMEM((2, 4, H, D), x.dtype),
                pltpu.SemaphoreType.DMA((9,)),
                pltpu.SemaphoreType.DMA((5,)),
                pltpu.SemaphoreType.DMA((2,)),
            ],
            compiler_params=pltpu.CompilerParams(vmem_limit_bytes=112 * 1024 * 1024, flags=FLAGS),
        )(x.reshape(B, 4, TQ, D), *ws)
        return out.reshape(B, T, D)
    return fn


_impl = make()


def pallas_standalone__conformer_family_branchformer__speech_kernel(x, w_q, w_k, w_v, w_ao, w_up, dw, w_dn, w_merge):
    return _impl(x, w_q, w_k, w_v, w_ao, w_up, dw, w_dn, w_merge)
```

```python
import functools

import jax
import jax.numpy as jnp
import numpy as np
from jax import lax
import jax.experimental.pallas as pl
import jax.experimental.pallas.tpu as pltpu

bf16, f32, i32 = jnp.bfloat16, jnp.float32, jnp.int32
LOG2E = 1.4426950408889634
EPS = 1e-5
NN = (((1,), (0,)), ((), ()))
NT = (((1,), (1,)), ((), ()))

H = 144
HALO = 16
PERM = (0, 2, 6, 5, 3, 4, 1)
ALPHA_TERMS = (((0, 0, 1), (1, 1, 1)), ((1, 0, 1), (1, 1, 1)), ((0, 0, 1),), ((1, 1, 1),),
               ((0, 0, 1), (0, 1, 1)), ((1, 0, 1), (0, 0, -1)), ((0, 1, 1), (1, 1, -1)))

PLAN = dict(
    MR=48, MW=(1, 11),
    XW=(2, 14), GR=24, GW=(2, 5), QO=(0, 5, 6, 2, 4, 1, 3),
    SK=3, CR=48, CQ0=(0, 1, 1, 2, 2), CQ=(0, 1, 1, 2, 2), CQL=(0, 1, 1, 2),
    UO=(1, 3, 2, 4, 0, 5, 6), SW=(0, 1), FW=(5, 7),
    VCH=(2, 2, 4), PW=((4, 7), (4, 7)), CJ=(0, 5, 7), CW=((2, 4), (2, 4), (2, 4)), US=2, UJ=2, UW=(1, 3),
    FO=(3, 1, 6, 2, 0, 4, 5),
)


def _ln(x, eps):
    d = x - jnp.mean(x, axis=-1, keepdims=True)
    v = jnp.mean(d * d, axis=-1, keepdims=True)
    return d * jnp.exp2(jnp.log(v + eps) * (-0.5 * LOG2E))


def _gelu2(x):
    c = float(np.sqrt(2.0 / np.pi))
    return x * jnp.tanh((x * x * (0.044715 * c) + c) * x) + x


def _dot(a, b, dims=NN):
    return lax.dot_general(a, b, dims, preferred_element_type=f32)


def rows(*parts):
    return jnp.concatenate(parts, axis=0)


def cols(*parts):
    return jnp.concatenate(parts, axis=1)


def pack(v):
    return pltpu.bitcast(v.astype(bf16), i32)


def unpack(v):
    return pltpu.bitcast(v, bf16)


def alpha(z):
    (a, b), (c, d) = z
    return [a + d, c + d, a, d, a + b, c - a, b - d]


def alpha_entry(k, z):
    (r0, c0, _), *rest = ALPHA_TERMS[k]
    v = z(r0, c0)
    for r, c, sign in rest:
        v = v + z(r, c) if sign > 0 else v - z(r, c)
    return v


def beta(z):
    t = alpha(z)
    return [t[k] for k in PERM]


def gamma(n):
    return [[n[0] + n[3] - n[4] + n[6], n[2] + n[4]], [n[1] + n[3], n[0] - n[1] + n[2] + n[5]]]


def alpha2(g):
    def pair(u, v):
        (x, sx), (y, sy) = u, v
        if sx > 0:
            return (x + y if sy > 0 else x - y), 1
        return (y - x, 1) if sy > 0 else (x + y, -1)

    out = []
    for a in range(7):
        for k in range(7):
            t = [[(g[2 * r1 + r2][2 * c1 + c2], s1 * s2) for r2, c2, s2 in ALPHA_TERMS[k]]
                 for r1, c1, s1 in ALPHA_TERMS[a]]
            if len(t) == 2 and len(t[0]) == 2:
                v, sign = pair(pair(t[0][0], t[1][1]), pair(t[0][1], t[1][0]))
            else:
                flat = [e for row in t for e in row]
                v, sign = pair(*flat) if len(flat) == 2 else flat[0]
            assert sign > 0
            out.append(v)
    return out


def gamma2(n):
    inner = [gamma(n[7 * a:7 * a + 7]) for a in range(7)]
    out = [[None] * 4 for _ in range(4)]
    for r2 in range(2):
        for c2 in range(2):
            z = gamma([inner[a][r2][c2] for a in range(7)])
            for r1 in range(2):
                for c1 in range(2):
                    out[2 * r1 + r2][2 * c1 + c2] = z[r1][c1]
    return out


def transpose(z):
    return [list(r) for r in zip(*z)]


def quadrants(w):
    n, m = w.shape[0] // 2, w.shape[1] // 2
    return [[w[i * n:(i + 1) * n, j * m:(j + 1) * m] for j in range(2)] for i in range(2)]


def merge(g):
    return [[rows(*[cols(g[2 * r1 + r2][2 * c1], g[2 * r1 + r2][2 * c1 + 1]) for r2 in range(2)])
             for c1 in range(2)] for r1 in range(2)]


def split(z):
    q = [[quadrants(v) for v in row] for row in z]
    return [[q[r // 2][c // 2][r % 2][c % 2] for c in range(4)] for r in range(4)]


def tie(never, a, tokens):
    if not tokens:
        return a
    nr, nc = a.shape[0] // 8, a.shape[1] // 128
    cells = {}
    for j, t in enumerate(tokens):
        p = j * nr * nc // len(tokens)
        cells[p] = jnp.maximum(cells[p], t) if p in cells else t
    out = []
    for p in range(nr):
        row = []
        for c in range(nc):
            v = a[8 * p:8 * p + 8, 128 * c:128 * c + 128]
            t = cells.get(p * nc + c)
            if t is not None:
                v = jnp.where(never, t if t.dtype == a.dtype else pltpu.bitcast(t, a.dtype), v)
            row.append(v)
        out.append(cols(*row))
    return rows(*out)


def take(queue, n):
    out = queue[:n]
    del queue[:n]
    return out


def window(queue, lo, hi, n):
    m = hi - lo
    return [[]] * lo + [queue[k * len(queue) // m:(k + 1) * len(queue) // m] for k in range(m)] + [[]] * (n - hi)


def _kernel(x_hbm, wq_hbm, wk_hbm, wv_hbm, wao_hbm, wup_hbm, dw_hbm, wdn_hbm, wm_hbm, o_hbm,
            x_v, wq, wk, wup, dwv, wa, wb,
            wp_s,
            wf_s,
            xa_s,
            x_s,
            qc_s,
            g_s,
            dw_s, ob_s, wsem, xsem, osem, *, plan):
    B, _, TQ, D = x_hbm.shape
    K = dw_hbm.shape[0]
    NL = D // 128
    nb = -(-TQ // H)
    HL = TQ - (nb - 1) * H
    H2 = H // 2
    NT_ = sum(plan["VCH"])
    assert NL == 4 and K // 2 <= HALO <= HL and nb * H <= 128 * NT_

    wc = {n: pltpu.make_async_copy(s, d, wsem.at[k]) for k, (n, s, d) in enumerate([
        ("q", wq_hbm, wq), ("k", wk_hbm, wk), ("up", wup_hbm, wup), ("dw", dw_hbm, dwv),
        ("v", wv_hbm, wa.at[0]), ("dn", wdn_hbm, wa.at[1]),
        ("ao", wao_hbm, wb.at[0]), ("m0", wm_hbm.at[0:D], wb.at[1]), ("m1", wm_hbm.at[D:2 * D], wb.at[2])])}
    late = [wc[n] for n in ("v", "ao", "m0", "dn", "m1")]
    cuts = list(range(0, nb * H, 2 * H)) + [TQ]
    xc = [pltpu.make_async_copy(x_hbm.at[0, :, pl.ds(a, e - a), :], x_v.at[0, :, pl.ds(a, e - a), :], xsem.at[n])
          for n, (a, e) in enumerate(zip(cuts[:-1], cuts[1:]))]
    late.append(pltpu.make_async_copy(x_hbm.at[pl.ds(1, B - 1)], x_v.at[pl.ds(1, B - 1), :, pl.ds(0, TQ), :],
                                      xsem.at[len(xc)]))

    def set_projection(n, w):
        for k, v in enumerate(beta(quadrants(w))):
            wp_s[n, k] = pack(v)

    def project(n, lhs, order=range(7)):
        res = [None] * 7
        for j, k in enumerate(order):
            res[k] = _dot(unpack(lhs(j, k)), unpack(wp_s[n, k]))
        return gamma(res)

    def normalize(b, r, n):
        rr = pl.ds(r if isinstance(r, int) else pl.multiple_of(r, 16), n)
        for h in range(4):
            xa_s[b, h, rr, :] = _ln(x_v[b, h, rr, :].astype(f32), EPS).astype(bf16)

    for c in (wc["q"], wc["k"], xc[0]):
        c.start()
    for b in range(B):
        for h in range(4):
            x_v[b, h, TQ:, :] = jnp.zeros((nb * H - TQ, D), x_v.dtype)
    for k in range(x_s.shape[0]):
        x_s[k, nb * H2:, :] = jnp.zeros((x_s.shape[1] - nb * H2, D // 2), i32)
    for c in range(NL):
        for h in range(4):
            g_s[nb, h, c, HALO + H:, :] = jnp.zeros((HALO, 128), f32)
        dw_s[c] = jnp.zeros(dw_s.shape[1:], f32)
    for c in (wc["q"], wc["k"]):
        c.wait()
    for c in (xc[1], wc["up"], wc["dw"]):
        c.start()
    set_projection(0, _dot(wq[...], wk[...], NT) * (LOG2E * D ** -0.5))
    xc[2].start()

    @pl.loop(0, nb)
    def _(i):
        for k in range(len(xc)):
            @pl.when(i * H == cuts[k])
            def _():
                if k == 2:
                    for c in (wc["up"], wc["dw"]):
                        c.wait()
                    set_projection(1, wup[:, 0:D].astype(f32))
                    set_projection(2, wup[:, D:2 * D].astype(f32))
                    for c in range(NL):
                        dw_s[c, 0:K, :] = dwv[:, c * 128:(c + 1) * 128].astype(f32) * 0.5
                xc[k].wait()
                for c in ((), (xc[3],), (), late)[k]:
                    c.start()
        normalize(0, i * H, H)

    def prepare(b, i):
        dst = pl.ds(pl.multiple_of(i * H2, 8), H2)
        rr = pl.ds(pl.multiple_of(i * H, 16), H)
        never = i < 0
        zero = pl.multiple_of(jnp.minimum(i, 0), 8)

        def tile(h, c):
            v = xa_s[b, h, rr, (c // 2) * 256:(c // 2 + 1) * 256].astype(f32)
            return v[:, (c % 2) * 128:(c % 2 + 1) * 128]

        x1, xq, left = [], [], []
        for a in range(7):
            z = [[alpha_entry(a, lambda r1, c1: tile(2 * r1 + r2, 2 * c1 + c2)) for c2 in range(2)] for r2 in range(2)]
            x1.append([pack(cols(*z[r2])) for r2 in range(2)])
            for r2 in range(2):
                x_s[2 * a + r2, dst, :] = x1[a][r2]
            l2 = left + [v for k, v in enumerate(alpha(z)) if k not in (2, 3)]
            if a == 6:
                l2.append(l2[-1])
            left = [l2.pop()] if len(l2) % 2 else []
            for k in range(len(l2) // 2):
                x_s[14 + 5 * a // 2 + k, dst, :] = pack(cols(l2[2 * k], l2[2 * k + 1]))
            xq.append(x_s[0, pl.ds(zero, 8), :128])
        xq = window(xq, *plan["XW"], 14)
        gpre = split(project(2, lambda j, k: tie(never, rows(*x1[k]), xq[j])))
        gq, GR = [], plan["GR"]
        for p in range(0, H, GR):
            for h in range(4):
                gate = _ln(_gelu2(cols(*[t[p:p + GR] for t in gpre[h]])), 4 * EPS)
                for c in range(NL):
                    t = gate[:, c * 128:(c + 1) * 128]
                    g_s[i + 1, h, c, HALO + p:HALO + p + GR, :] = t
                    if p < HALO:
                        g_s[i, h, c, HALO + H + p:HALO + H + min(p + GR, HALO), :] = t[:HALO - p]
                    if p + GR > H - HALO:
                        o = max(H - HALO - p, 0)
                        g_s[i + 2, h, c, p + o - (H - HALO):p + GR - (H - HALO), :] = t[o:]
            gq.append(pltpu.bitcast(g_s[i + 1, 0, 0, pl.ds(zero + HALO, 8), :], i32))
        gq = window(gq, *plan["GW"], 7)
        q = project(0, lambda j, k: tie(never, rows(*x1[k]), gq[j] + xq[7 + k]), plan["QO"])
        for k, v in enumerate(beta(transpose(q))):
            qc_s[i, k] = pack(v)

    def connect_quarters():
        zero = jnp.zeros((HALO, 128), f32)
        for c in range(NL):
            for h in range(4):
                g_s[nb, h, c, HALO + HL:2 * HALO + HL, :] = g_s[1, h + 1, c, HALO:2 * HALO, :] if h < 3 else zero
                g_s[1, h, c, 0:HALO, :] = g_s[nb, h - 1, c, HL:HL + HALO, :] if h else zero

    def merge_weights(b0):
        for c in late:
            c.wait()
        zero = pl.multiple_of(jnp.minimum(b0, 0), 16)
        tq = []
        for b in range(1, B):
            for p in range(0, nb * H, plan["MR"]):
                normalize(b, p, plan["MR"])
                tq.append(pltpu.bitcast(xa_s[b, 0, pl.ds(zero, 16), :128], i32))
        tq = [list(t) for t in window(tq, *plan["MW"], 12)]

        def product(n, a, w):
            return cols(*[_dot(unpack(tie(b0 < 0, a, tq[4 * n + c])), wb[w, :, c * 128:(c + 1) * 128])
                          for c in range(4)])

        t = product(0, pltpu.bitcast(wa[0], i32), 0)
        for k, v in enumerate(beta(quadrants(product(1, pltpu.bitcast(wa[1], i32), 2)))):
            wf_s[k, D // 4:, :] = pack(v)
        tq[11].append(wf_s[0, pl.ds(zero + D // 4, 8), :128])
        for k, v in enumerate(beta(quadrants(product(2, pack(t), 1)))):
            wf_s[k, :D // 4, :] = pack(v)

    def out_copy(slot, b, r, n):
        return pltpu.make_async_copy(ob_s.at[slot, :, pl.ds(0, n), :], o_hbm.at[b, :, pl.ds(r, n), :], osem.at[slot])

    def step(b, i):
        r = pl.multiple_of(i * H, 16)
        never = i < 0
        it = b * nb + i
        slot = it % 2
        short = (i == 1) & (b > 0)
        pl.when(short)(lambda: out_copy(slot, 0, 0, HL).wait())
        pl.when((it > 1) & jnp.logical_not(short))(lambda: out_copy(slot, 0, 0, H).wait())

        conv = [[None] * NL for _ in range(4)]
        convq, CR = [], plan["CR"]
        for h in range(4):
            for c in range(NL):
                w = dw_s[c]
                pieces = []
                for p in range(0, H, CR):
                    acc = None
                    for t in sorted(range(K), key=lambda t: (t % 8, t)):
                        term = g_s[i + 1, h, c, pl.ds(p + HALO - K // 2 + t, CR), :] * w[t:t + 1, :]
                        acc = term if acc is None else acc + term
                    pieces.append(acc)
                    convq.append([acc[k:k + 8] for k in range(0, CR, 8)])
                conv[h][c] = rows(*pieces)

        chunks = [(j, r2) for j in range(NT_ // 2) for r2 in range(2)]
        qc = [qc_s[i, k] for k in range(7)]
        s = [[[None] * NT_ for _ in range(4)] for _ in range(4)]
        m, l, statq = [None] * 4, [None] * 4, []
        for n, (j, r2) in enumerate(chunks):
            st = window(statq, plan["SK"], 7, 7)
            cq = plan["CQ0"] if n == 0 else plan["CQL"] if n == len(chunks) - 1 else plan["CQ"]
            z = split(transpose(gamma([
                _dot(unpack(tie(never, qc[k], st[k] + sum(take(convq, cq.count(k)), []))),
                     unpack(x_s[2 * k + r2, j * 128:(j + 1) * 128, :]), NT) for k in range(7)])))
            for h in range(4):
                new = []
                for c in range(4):
                    v, t = z[h][c], 2 * j + c % 2
                    if (t + 1) * 128 > TQ:
                        v = jnp.where(t * 128 + lax.broadcasted_iota(i32, v.shape, 1) < TQ, v, -jnp.inf)
                    s[h][2 * (c // 2) + r2][t] = v
                    new.append(v)
                mx = functools.reduce(jnp.maximum, new)
                tot = None
                if m[h] is not None:
                    mx = jnp.maximum(m[h], mx)
                    tot = l[h] * jnp.exp2(m[h] - mx)
                for v in new:
                    e = jnp.exp2(v - mx)
                    tot = e if tot is None else tot + e
                m[h], l[h] = mx, tot
            statq = [l[2 * r1 + a][p:p + 8] for a in range(2) for p in range(0, H, 8) for r1 in range(2)]
        shift = []
        for h in range(4):
            mr = jnp.max(m[h], axis=-1, keepdims=True)
            shift.append(mr + jnp.log2(jnp.sum(l[h] * jnp.exp2(m[h] - mr), axis=-1, keepdims=True)))

        edges = np.cumsum((0,) + tuple(plan["VCH"]))

        def probabilities(n):
            tiles = range(edges[n], edges[n + 1])
            g = [[cols(*[jnp.exp2(s[h][c][t] - shift[h]) for t in tiles]) for c in range(4)] for h in range(4)]
            return alpha2(g), [g[h][c][p:p + 8, t * 128:(t + 1) * 128] for p in range(0, H, 8)
                               for h in range(4) for c in range(4) for t in range(len(tiles))]

        operands, pq = probabilities(0)
        st, pq = window(statq, *plan["SW"], 7), window(pq, *plan["FW"], 7)
        r2 = pl.ds(pl.multiple_of(i * H2, 8), H2)
        upre = split(project(1, lambda j, k: tie(never, rows(x_s[2 * k, r2, :], x_s[2 * k + 1, r2, :]),
                                                 st[j] + pq[j]), plan["UO"]))

        acc, uq, nv = [None] * 49, [], len(plan["VCH"])
        win = lambda queue, w: window(queue, 7 * w[0], 7 * w[1], 49)
        for n in range(nv):
            following, pq = probabilities(n + 1) if n + 1 < nv else (None, [])
            pq = win(pq, plan["PW"][n]) if n + 1 < nv else [[]] * 49
            ug = win(uq if n == plan["UJ"] else [], plan["UW"])
            cg = win(take(convq, plan["CJ"][n]), plan["CW"][n])
            for k in range(49):
                a, c = PERM[k // 7], PERM[k % 7]
                t = 4 * a if c == 2 else 4 * a + 3 if c == 3 else 28 + 5 * a + (c if c < 2 else c - 2)
                d = _dot(tie(never, operands[k], pq[k] + ug[k] + sum(cg[k], [])).astype(bf16),
                         unpack(x_s[t // 2, edges[n] * 64:edges[n + 1] * 64, (t % 2) * 128:(t % 2 + 1) * 128]))
                acc[k] = d if acc[k] is None else acc[k] + d
                if n == 0 and k == 7 * plan["US"]:
                    started = d
            operands = following
            if n == 0:
                u = [[_gelu2(jnp.where(never, started, v)) for v in row] for row in upre]
                uq = [v[p:p + 8] for row in u for v in row for p in range(0, H, 8)]

        uc = [[u[h][c] * conv[h][c] for c in range(4)] for h in range(4)]
        ao, ac = alpha(merge(gamma2(acc))), alpha(merge(uc))
        res = [None] * 7
        for k in plan["FO"]:
            res[k] = _dot(cols(ao[k], ac[k]).astype(bf16), unpack(wf_s[k]))
        out = split(gamma(res))
        for h in range(4):
            ob_s[slot, h] = (x_v[b, h, pl.ds(r, H), :].astype(f32) + cols(*out[h])).astype(ob_s.dtype)
        pl.when(i < nb - 1)(lambda: out_copy(slot, b, r, H).start())
        pl.when(i == nb - 1)(lambda: out_copy(slot, b, r, HL).start())

    @pl.loop(0, B)
    def _(b):
        pl.loop(0, nb)(functools.partial(prepare, b))
        connect_quarters()
        pl.when(b == 0)(lambda: merge_weights(b))
        pl.loop(0, nb)(functools.partial(step, b))

    out_copy((B * nb) % 2, 0, 0, H).wait()
    out_copy((B * nb + 1) % 2, 0, 0, HL).wait()


def _call(x, w_q, w_k, w_v, w_ao, w_up, dw, w_dn, w_merge, plan):
    B, T, D = x.shape
    TQ = T // 4
    nb = -(-TQ // H)
    hbm = pl.BlockSpec(memory_space=pl.ANY)
    out = pl.pallas_call(
        functools.partial(_kernel, plan=plan),
        in_specs=[hbm] * 9,
        out_specs=hbm,
        out_shape=jax.ShapeDtypeStruct((B, 4, TQ, D), x.dtype),
        scratch_shapes=[
            pltpu.VMEM((B, 4, nb * H, D), x.dtype),
            pltpu.VMEM(w_q.shape, w_q.dtype),
            pltpu.VMEM(w_k.shape, w_k.dtype),
            pltpu.VMEM(w_up.shape, w_up.dtype),
            pltpu.VMEM(dw.shape, dw.dtype),
            pltpu.VMEM((2, D, D), bf16),
            pltpu.VMEM((3, D, D), bf16),
            pltpu.VMEM((3, 7, D // 4, D // 2), i32),
            pltpu.VMEM((7, D // 2, D // 2), i32),
            pltpu.VMEM((B, 4, nb * H, D), bf16),
            pltpu.VMEM((32, 64 * sum(plan["VCH"]), D // 2), i32),
            pltpu.VMEM((nb, 7, H, D // 2), i32),
            pltpu.VMEM((nb + 2, 4, D // 128, H + 2 * HALO, 128), f32),
            pltpu.VMEM((D // 128, 2 * HALO, 128), f32),
            pltpu.VMEM((2, 4, H, D), x.dtype),
            pltpu.SemaphoreType.DMA((9,)),
            pltpu.SemaphoreType.DMA((-(-nb // 2) + 1,)),
            pltpu.SemaphoreType.DMA((2,)),
        ],
        compiler_params=pltpu.CompilerParams(vmem_limit_bytes=112 * 1024 * 1024),
    )(x.reshape(B, 4, TQ, D), w_q, w_k, w_v, w_ao, w_up, dw, w_dn, w_merge)
    return out.reshape(B, T, D)


@jax.jit
def pallas_standalone__conformer_family_branchformer__speech_kernel(
    x: jax.Array,
    w_q: jax.Array,
    w_k: jax.Array,
    w_v: jax.Array,
    w_ao: jax.Array,
    w_up: jax.Array,
    dw: jax.Array,
    w_dn: jax.Array,
    w_merge: jax.Array,
):
    return _call(x, w_q, w_k, w_v, w_ao, w_up, dw, w_dn, w_merge, PLAN)
```

```python
import functools

import jax
import jax.numpy as jnp
import numpy as np
from jax import lax
import jax.experimental.pallas as pl
import jax.experimental.pallas.tpu as pltpu

bf16, f32, i32 = jnp.bfloat16, jnp.float32, jnp.int32
LOG2E = 1.4426950408889634
EPS = 1e-5
NN = (((1,), (0,)), ((), ()))
NT = (((1,), (1,)), ((), ()))

H = 144
HALO = 16
PERM = (0, 2, 6, 5, 3, 4, 1)
ALPHA_TERMS = (((0, 0, 1), (1, 1, 1)), ((1, 0, 1), (1, 1, 1)), ((0, 0, 1),), ((1, 1, 1),),
               ((0, 0, 1), (0, 1, 1)), ((1, 0, 1), (0, 0, -1)), ((0, 1, 1), (1, 1, -1)))

PLAN = dict(
    MR=48, MW=(1, 11),
    XW=(2, 14), GR=24, GW=(2, 5), QO=(0, 5, 6, 2, 4, 1, 3),
    SK=3, CR=48, CQ0=(0, 1, 1, 2, 2), CQ=(0, 1, 1, 2, 2), CQL=(0, 1, 1, 2),
    UO=(1, 3, 2, 4, 0, 5, 6), SW=(0, 1), FW=(5, 7),
    VCH=(2, 2, 4), PW=((4, 7), (5, 7)), CJ=(0, 5, 7), CW=((2, 4), (2, 4), (2, 4)), US=2, UJ=2, UW=(0, 2),
    FO=(3, 1, 6, 2, 0, 4, 5),
)


def _ln(x, eps):
    d = x - jnp.mean(x, axis=-1, keepdims=True)
    v = jnp.mean(d * d, axis=-1, keepdims=True)
    return d * jnp.exp2(jnp.log(v + eps) * (-0.5 * LOG2E))


def _gelu2(x):
    c = float(np.sqrt(2.0 / np.pi))
    return x * jnp.tanh((x * x * (0.044715 * c) + c) * x) + x


def _dot(a, b, dims=NN):
    return lax.dot_general(a, b, dims, preferred_element_type=f32)


def rows(*parts):
    return jnp.concatenate(parts, axis=0)


def cols(*parts):
    return jnp.concatenate(parts, axis=1)


def pack(v):
    return pltpu.bitcast(v.astype(bf16), i32)


def unpack(v):
    return pltpu.bitcast(v, bf16)


def alpha(z):
    (a, b), (c, d) = z
    return [a + d, c + d, a, d, a + b, c - a, b - d]


def alpha_entry(k, z):
    (r0, c0, _), *rest = ALPHA_TERMS[k]
    v = z(r0, c0)
    for r, c, sign in rest:
        v = v + z(r, c) if sign > 0 else v - z(r, c)
    return v


def beta(z):
    t = alpha(z)
    return [t[k] for k in PERM]


def gamma(n):
    return [[n[0] + n[3] - n[4] + n[6], n[2] + n[4]], [n[1] + n[3], n[0] - n[1] + n[2] + n[5]]]


def alpha2(g):
    def pair(u, v):
        (x, sx), (y, sy) = u, v
        if sx > 0:
            return (x + y if sy > 0 else x - y), 1
        return (y - x, 1) if sy > 0 else (x + y, -1)

    out = []
    for a in range(7):
        for k in range(7):
            t = [[(g[2 * r1 + r2][2 * c1 + c2], s1 * s2) for r2, c2, s2 in ALPHA_TERMS[k]]
                 for r1, c1, s1 in ALPHA_TERMS[a]]
            if len(t) == 2 and len(t[0]) == 2:
                v, sign = pair(pair(t[0][0], t[1][1]), pair(t[0][1], t[1][0]))
            else:
                flat = [e for row in t for e in row]
                v, sign = pair(*flat) if len(flat) == 2 else flat[0]
            assert sign > 0
            out.append(v)
    return out


def gamma2(n):
    inner = [gamma(n[7 * a:7 * a + 7]) for a in range(7)]
    out = [[None] * 4 for _ in range(4)]
    for r2 in range(2):
        for c2 in range(2):
            z = gamma([inner[a][r2][c2] for a in range(7)])
            for r1 in range(2):
                for c1 in range(2):
                    out[2 * r1 + r2][2 * c1 + c2] = z[r1][c1]
    return out


def transpose(z):
    return [list(r) for r in zip(*z)]


def quadrants(w):
    n, m = w.shape[0] // 2, w.shape[1] // 2
    return [[w[i * n:(i + 1) * n, j * m:(j + 1) * m] for j in range(2)] for i in range(2)]


def merge(g):
    return [[rows(*[cols(g[2 * r1 + r2][2 * c1], g[2 * r1 + r2][2 * c1 + 1]) for r2 in range(2)])
             for c1 in range(2)] for r1 in range(2)]


def split(z):
    q = [[quadrants(v) for v in row] for row in z]
    return [[q[r // 2][c // 2][r % 2][c % 2] for c in range(4)] for r in range(4)]


def tie(never, a, tokens):
    if not tokens:
        return a
    nr, nc = a.shape[0] // 8, a.shape[1] // 128
    cells = {}
    for j, t in enumerate(tokens):
        p = j * nr * nc // len(tokens)
        cells[p] = jnp.maximum(cells[p], t) if p in cells else t
    out = []
    for p in range(nr):
        row = []
        for c in range(nc):
            v = a[8 * p:8 * p + 8, 128 * c:128 * c + 128]
            t = cells.get(p * nc + c)
            if t is not None:
                v = jnp.where(never, t if t.dtype == a.dtype else pltpu.bitcast(t, a.dtype), v)
            row.append(v)
        out.append(cols(*row))
    return rows(*out)


def take(queue, n):
    out = queue[:n]
    del queue[:n]
    return out


def window(queue, lo, hi, n):
    m = hi - lo
    return [[]] * lo + [queue[k * len(queue) // m:(k + 1) * len(queue) // m] for k in range(m)] + [[]] * (n - hi)


def _kernel(x_hbm, wq_hbm, wk_hbm, wv_hbm, wao_hbm, wup_hbm, dw_hbm, wdn_hbm, wm_hbm, o_hbm,
            x_v, wq, wk, wup, dwv, wa, wb,
            wp_s,
            wf_s,
            xa_s,
            x_s,
            qc_s,
            g_s,
            dw_s, ob_s, wsem, xsem, osem, *, plan):
    B, _, TQ, D = x_hbm.shape
    K = dw_hbm.shape[0]
    NL = D // 128
    nb = -(-TQ // H)
    HL = TQ - (nb - 1) * H
    H2 = H // 2
    NT_ = sum(plan["VCH"])
    assert NL == 4 and K // 2 <= HALO <= HL and nb * H <= 128 * NT_

    wc = {n: pltpu.make_async_copy(s, d, wsem.at[k]) for k, (n, s, d) in enumerate([
        ("q", wq_hbm, wq), ("k", wk_hbm, wk), ("dw", dw_hbm, dwv),
        ("u", wup_hbm.at[:, 0:D], wup.at[0]), ("g", wup_hbm.at[:, D:2 * D], wup.at[1]),
        ("v", wv_hbm, wa.at[0]), ("dn", wdn_hbm, wa.at[1]),
        ("ao", wao_hbm, wb.at[0]), ("m0", wm_hbm.at[0:D], wb.at[1]), ("m1", wm_hbm.at[D:2 * D], wb.at[2])])}
    late = [wc[n] for n in ("v", "ao", "m0", "dn", "m1", "u", "dw")]
    cuts = list(range(0, nb * H, 2 * H)) + [TQ]
    xc = [pltpu.make_async_copy(x_hbm.at[0, :, pl.ds(a, e - a), :], x_v.at[0, :, pl.ds(a, e - a), :], xsem.at[n])
          for n, (a, e) in enumerate(zip(cuts[:-1], cuts[1:]))]
    late.append(pltpu.make_async_copy(x_hbm.at[pl.ds(1, B - 1)], x_v.at[pl.ds(1, B - 1), :, pl.ds(0, TQ), :],
                                      xsem.at[len(xc)]))

    def set_projection(n, w):
        for k, v in enumerate(beta(quadrants(w))):
            wp_s[n, k] = pack(v)

    def project(n, lhs, order=range(7)):
        res = [None] * 7
        for j, k in enumerate(order):
            res[k] = _dot(unpack(lhs(j, k)), unpack(wp_s[n, k]))
        return gamma(res)

    def normalize(b, r, n):
        rr = pl.ds(r if isinstance(r, int) else pl.multiple_of(r, 16), n)
        for h in range(4):
            xa_s[b, h, rr, :] = _ln(x_v[b, h, rr, :].astype(f32), EPS).astype(bf16)

    for c in (wc["q"], wc["k"], xc[0]):
        c.start()
    for b in range(B):
        for h in range(4):
            x_v[b, h, TQ:, :] = jnp.zeros((nb * H - TQ, D), x_v.dtype)
    for k in range(x_s.shape[0]):
        x_s[k, nb * H2:, :] = jnp.zeros((x_s.shape[1] - nb * H2, D // 2), i32)
    for c in range(NL):
        for h in range(4):
            g_s[nb, h, c, HALO + H:, :] = jnp.zeros((HALO, 128), f32)
        dw_s[c] = jnp.zeros(dw_s.shape[1:], f32)
    for c in (wc["q"], wc["k"]):
        c.wait()
    for c in (xc[1], wc["g"]):
        c.start()
    set_projection(0, _dot(wq[...], wk[...], NT) * (LOG2E * D ** -0.5))
    xc[2].start()

    @pl.loop(0, nb)
    def _(i):
        for k in range(len(xc)):
            @pl.when(i * H == cuts[k])
            def _():
                if k == 2:
                    wc["g"].wait()
                    set_projection(2, wup[1].astype(f32))
                xc[k].wait()
                for c in ((), (xc[3],), (), late)[k]:
                    c.start()
        normalize(0, i * H, H)

    def prepare(b, i):
        dst = pl.ds(pl.multiple_of(i * H2, 8), H2)
        rr = pl.ds(pl.multiple_of(i * H, 16), H)
        never = i < 0
        zero = pl.multiple_of(jnp.minimum(i, 0), 8)

        def tile(h, c):
            v = xa_s[b, h, rr, (c // 2) * 256:(c // 2 + 1) * 256].astype(f32)
            return v[:, (c % 2) * 128:(c % 2 + 1) * 128]

        x1, xq, left = [], [], []
        for a in range(7):
            z = [[alpha_entry(a, lambda r1, c1: tile(2 * r1 + r2, 2 * c1 + c2)) for c2 in range(2)] for r2 in range(2)]
            x1.append([pack(cols(*z[r2])) for r2 in range(2)])
            for r2 in range(2):
                x_s[2 * a + r2, dst, :] = x1[a][r2]
            l2 = left + [v for k, v in enumerate(alpha(z)) if k not in (2, 3)]
            if a == 6:
                l2.append(l2[-1])
            left = [l2.pop()] if len(l2) % 2 else []
            for k in range(len(l2) // 2):
                x_s[14 + 5 * a // 2 + k, dst, :] = pack(cols(l2[2 * k], l2[2 * k + 1]))
            xq.append(x_s[0, pl.ds(zero, 8), :128])
        xq = window(xq, *plan["XW"], 14)
        gpre = split(project(2, lambda j, k: tie(never, rows(*x1[k]), xq[j])))
        gq, GR = [], plan["GR"]
        for p in range(0, H, GR):
            for h in range(4):
                gate = _ln(_gelu2(cols(*[t[p:p + GR] for t in gpre[h]])), 4 * EPS)
                for c in range(NL):
                    t = gate[:, c * 128:(c + 1) * 128]
                    g_s[i + 1, h, c, HALO + p:HALO + p + GR, :] = t
                    if p < HALO:
                        g_s[i, h, c, HALO + H + p:HALO + H + min(p + GR, HALO), :] = t[:HALO - p]
                    if p + GR > H - HALO:
                        o = max(H - HALO - p, 0)
                        g_s[i + 2, h, c, p + o - (H - HALO):p + GR - (H - HALO), :] = t[o:]
            gq.append(pltpu.bitcast(g_s[i + 1, 0, 0, pl.ds(zero + HALO, 8), :], i32))
        gq = window(gq, *plan["GW"], 7)
        q = project(0, lambda j, k: tie(never, rows(*x1[k]), gq[j] + xq[7 + k]), plan["QO"])
        for k, v in enumerate(beta(transpose(q))):
            qc_s[i, k] = pack(v)

    def connect_quarters():
        zero = jnp.zeros((HALO, 128), f32)
        for c in range(NL):
            for h in range(4):
                g_s[nb, h, c, HALO + HL:2 * HALO + HL, :] = g_s[1, h + 1, c, HALO:2 * HALO, :] if h < 3 else zero
                g_s[1, h, c, 0:HALO, :] = g_s[nb, h - 1, c, HL:HL + HALO, :] if h else zero

    def merge_weights(b0):
        for c in late:
            c.wait()
        zero = pl.multiple_of(jnp.minimum(b0, 0), 16)
        tq = []
        for b in range(1, B):
            for p in range(0, nb * H, plan["MR"]):
                normalize(b, p, plan["MR"])
                tq.append(pltpu.bitcast(xa_s[b, 0, pl.ds(zero, 16), :128], i32))
        tq = [list(t) for t in window(tq, *plan["MW"], 12)]
        set_projection(1, wup[0].astype(f32))
        for c in range(NL):
            dw_s[c, 0:K, :] = dwv[:, c * 128:(c + 1) * 128].astype(f32) * 0.5
        tq[10].append(wp_s[1, 0, pl.ds(zero, 8), :128])

        def product(n, a, w):
            return cols(*[_dot(unpack(tie(b0 < 0, a, tq[4 * n + c])), wb[w, :, c * 128:(c + 1) * 128])
                          for c in range(4)])

        t = product(0, pltpu.bitcast(wa[0], i32), 0)
        for k, v in enumerate(beta(quadrants(product(1, pltpu.bitcast(wa[1], i32), 2)))):
            wf_s[k, D // 4:, :] = pack(v)
        tq[11].append(wf_s[0, pl.ds(zero + D // 4, 8), :128])
        for k, v in enumerate(beta(quadrants(product(2, pack(t), 1)))):
            wf_s[k, :D // 4, :] = pack(v)

    def out_copy(slot, b, r, n):
        return pltpu.make_async_copy(ob_s.at[slot, :, pl.ds(0, n), :], o_hbm.at[b, :, pl.ds(r, n), :], osem.at[slot])

    def step(b, i):
        r = pl.multiple_of(i * H, 16)
        never = i < 0
        it = b * nb + i
        slot = it % 2
        short = (i == 1) & (b > 0)
        pl.when(short)(lambda: out_copy(slot, 0, 0, HL).wait())
        pl.when((it > 1) & jnp.logical_not(short))(lambda: out_copy(slot, 0, 0, H).wait())

        conv = [[None] * NL for _ in range(4)]
        convq, CR = [], plan["CR"]
        for h in range(4):
            for c in range(NL):
                w = dw_s[c]
                pieces = []
                for p in range(0, H, CR):
                    acc = None
                    for t in sorted(range(K), key=lambda t: (t % 8, t)):
                        term = g_s[i + 1, h, c, pl.ds(p + HALO - K // 2 + t, CR), :] * w[t:t + 1, :]
                        acc = term if acc is None else acc + term
                    pieces.append(acc)
                    convq.append([acc[k:k + 8] for k in range(0, CR, 8)])
                conv[h][c] = rows(*pieces)

        chunks = [(j, r2) for j in range(NT_ // 2) for r2 in range(2)]
        qc = [qc_s[i, k] for k in range(7)]
        s = [[[None] * NT_ for _ in range(4)] for _ in range(4)]
        m, l, statq = [None] * 4, [None] * 4, []
        for n, (j, r2) in enumerate(chunks):
            st = window(statq, plan["SK"], 7, 7)
            cq = plan["CQ0"] if n == 0 else plan["CQL"] if n == len(chunks) - 1 else plan["CQ"]
            z = split(transpose(gamma([
                _dot(unpack(tie(never, qc[k], st[k] + sum(take(convq, cq.count(k)), []))),
                     unpack(x_s[2 * k + r2, j * 128:(j + 1) * 128, :]), NT) for k in range(7)])))
            for h in range(4):
                new = []
                for c in range(4):
                    v, t = z[h][c], 2 * j + c % 2
                    if (t + 1) * 128 > TQ:
                        v = jnp.where(t * 128 + lax.broadcasted_iota(i32, v.shape, 1) < TQ, v, -jnp.inf)
                    s[h][2 * (c // 2) + r2][t] = v
                    new.append(v)
                mx = functools.reduce(jnp.maximum, new)
                tot = None
                if m[h] is not None:
                    mx = jnp.maximum(m[h], mx)
                    tot = l[h] * jnp.exp2(m[h] - mx)
                for v in new:
                    e = jnp.exp2(v - mx)
                    tot = e if tot is None else tot + e
                m[h], l[h] = mx, tot
            statq = [l[2 * r1 + a][p:p + 8] for a in range(2) for p in range(0, H, 8) for r1 in range(2)]
        shift = []
        for h in range(4):
            mr = jnp.max(m[h], axis=-1, keepdims=True)
            shift.append(mr + jnp.log2(jnp.sum(l[h] * jnp.exp2(m[h] - mr), axis=-1, keepdims=True)))

        edges = np.cumsum((0,) + tuple(plan["VCH"]))

        def probabilities(n):
            tiles = range(edges[n], edges[n + 1])
            g = [[cols(*[jnp.exp2(s[h][c][t] - shift[h]) for t in tiles]) for c in range(4)] for h in range(4)]
            return alpha2(g), [g[h][c][p:p + 8, t * 128:(t + 1) * 128] for p in range(0, H, 8)
                               for h in range(4) for c in range(4) for t in range(len(tiles))]

        operands, pq = probabilities(0)
        st, pq = window(statq, *plan["SW"], 7), window(pq, *plan["FW"], 7)
        r2 = pl.ds(pl.multiple_of(i * H2, 8), H2)
        upre = split(project(1, lambda j, k: tie(never, rows(x_s[2 * k, r2, :], x_s[2 * k + 1, r2, :]),
                                                 st[j] + pq[j]), plan["UO"]))

        acc, uq, nv = [None] * 49, [], len(plan["VCH"])
        win = lambda queue, w: window(queue, 7 * w[0], 7 * w[1], 49)
        for n in range(nv):
            following, pq = probabilities(n + 1) if n + 1 < nv else (None, [])
            pq = win(pq, plan["PW"][n]) if n + 1 < nv else [[]] * 49
            ug = win(uq if n == plan["UJ"] else [], plan["UW"])
            cg = win(take(convq, plan["CJ"][n]), plan["CW"][n])
            for k in range(49):
                a, c = PERM[k // 7], PERM[k % 7]
                t = 4 * a if c == 2 else 4 * a + 3 if c == 3 else 28 + 5 * a + (c if c < 2 else c - 2)
                d = _dot(tie(never, operands[k], pq[k] + ug[k] + sum(cg[k], [])).astype(bf16),
                         unpack(x_s[t // 2, edges[n] * 64:edges[n + 1] * 64, (t % 2) * 128:(t % 2 + 1) * 128]))
                acc[k] = d if acc[k] is None else acc[k] + d
                if n == 0 and k == 7 * plan["US"]:
                    started = d
            operands = following
            if n == 0:
                u = [[_gelu2(jnp.where(never, started, v)) for v in row] for row in upre]
                uq = [v[p:p + 8] for row in u for v in row for p in range(0, H, 8)]

        uc = [[u[h][c] * conv[h][c] for c in range(4)] for h in range(4)]
        ao, ac = alpha(merge(gamma2(acc))), alpha(merge(uc))
        res = [None] * 7
        for k in plan["FO"]:
            res[k] = _dot(cols(ao[k], ac[k]).astype(bf16), unpack(wf_s[k]))
        out = split(gamma(res))
        for h in range(4):
            ob_s[slot, h] = (x_v[b, h, pl.ds(r, H), :].astype(f32) + cols(*out[h])).astype(ob_s.dtype)
        pl.when(i < nb - 1)(lambda: out_copy(slot, b, r, H).start())
        pl.when(i == nb - 1)(lambda: out_copy(slot, b, r, HL).start())

    @pl.loop(0, B)
    def _(b):
        pl.loop(0, nb)(functools.partial(prepare, b))
        connect_quarters()
        pl.when(b == 0)(lambda: merge_weights(b))
        pl.loop(0, nb)(functools.partial(step, b))

    out_copy((B * nb) % 2, 0, 0, H).wait()
    out_copy((B * nb + 1) % 2, 0, 0, HL).wait()


def _call(x, w_q, w_k, w_v, w_ao, w_up, dw, w_dn, w_merge, plan):
    B, T, D = x.shape
    TQ = T // 4
    nb = -(-TQ // H)
    hbm = pl.BlockSpec(memory_space=pl.ANY)
    out = pl.pallas_call(
        functools.partial(_kernel, plan=plan),
        in_specs=[hbm] * 9,
        out_specs=hbm,
        out_shape=jax.ShapeDtypeStruct((B, 4, TQ, D), x.dtype),
        scratch_shapes=[
            pltpu.VMEM((B, 4, nb * H, D), x.dtype),
            pltpu.VMEM(w_q.shape, w_q.dtype),
            pltpu.VMEM(w_k.shape, w_k.dtype),
            pltpu.VMEM((2, D, D), w_up.dtype),
            pltpu.VMEM(dw.shape, dw.dtype),
            pltpu.VMEM((2, D, D), bf16),
            pltpu.VMEM((3, D, D), bf16),
            pltpu.VMEM((3, 7, D // 4, D // 2), i32),
            pltpu.VMEM((7, D // 2, D // 2), i32),
            pltpu.VMEM((B, 4, nb * H, D), bf16),
            pltpu.VMEM((32, 64 * sum(plan["VCH"]), D // 2), i32),
            pltpu.VMEM((nb, 7, H, D // 2), i32),
            pltpu.VMEM((nb + 2, 4, D // 128, H + 2 * HALO, 128), f32),
            pltpu.VMEM((D // 128, 2 * HALO, 128), f32),
            pltpu.VMEM((2, 4, H, D), x.dtype),
            pltpu.SemaphoreType.DMA((10,)),
            pltpu.SemaphoreType.DMA((-(-nb // 2) + 1,)),
            pltpu.SemaphoreType.DMA((2,)),
        ],
        compiler_params=pltpu.CompilerParams(vmem_limit_bytes=112 * 1024 * 1024),
    )(x.reshape(B, 4, TQ, D), w_q, w_k, w_v, w_ao, w_up, dw, w_dn, w_merge)
    return out.reshape(B, T, D)


@jax.jit
def pallas_standalone__conformer_family_branchformer__speech_kernel(
    x: jax.Array,
    w_q: jax.Array,
    w_k: jax.Array,
    w_v: jax.Array,
    w_ao: jax.Array,
    w_up: jax.Array,
    dw: jax.Array,
    w_dn: jax.Array,
    w_merge: jax.Array,
):
    return _call(x, w_q, w_k, w_v, w_ao, w_up, dw, w_dn, w_merge, PLAN)
```

```python
import functools

import jax
import jax.numpy as jnp
import numpy as np
from jax import lax
import jax.experimental.pallas as pl
import jax.experimental.pallas.tpu as pltpu

bf16, f32, i32 = jnp.bfloat16, jnp.float32, jnp.int32
LOG2E = 1.4426950408889634
EPS = 1e-5
NN = (((1,), (0,)), ((), ()))
NT = (((1,), (1,)), ((), ()))

H = 144
HALO = 16
PERM = (0, 2, 6, 5, 3, 4, 1)
ALPHA_TERMS = (((0, 0, 1), (1, 1, 1)), ((1, 0, 1), (1, 1, 1)), ((0, 0, 1),), ((1, 1, 1),),
               ((0, 0, 1), (0, 1, 1)), ((1, 0, 1), (0, 0, -1)), ((0, 1, 1), (1, 1, -1)))

PLAN = dict(
    MR=48, MW=(1, 11),
    XW=(2, 14), GR=24, GW=(2, 5), QO=(0, 1, 5, 2, 4, 3, 6),
    AO=(0, 1, 2, 5, 4, 3, 6), IO=(0, 1, 3, 2, 5, 4, 6), QW=(1, 7), CR=48, QC=6, QCW=(0, 3),
    UO=(1, 3, 2, 4, 0, 5, 6), SW=(1, 2), FW=(5, 7),
    VCH=(2, 2, 4), PA=(0, 1, 2, 3, 4, 5, 6), PL=(4, 5, 2, 3, 0, 1, 6), PI=(2, 3, 0, 1, 4, 5, 6),
    PW=((4, 7), (4, 7)), CJ=(4, 8, 12), CW=((2, 4), (2, 4), (2, 4)), US=6, UJ=2, UW=(0, 2),
    FO=(3, 1, 6, 2, 0, 4, 5), FS=(0, 7),
)


def _ln(x, eps):
    d = x - jnp.mean(x, axis=-1, keepdims=True)
    v = jnp.mean(d * d, axis=-1, keepdims=True)
    return d * jnp.exp2(jnp.log(v + eps) * (-0.5 * LOG2E))


def _gelu2(x):
    c = float(np.sqrt(2.0 / np.pi))
    return x * jnp.tanh((x * x * (0.044715 * c) + c) * x) + x


def _dot(a, b, dims=NN):
    return lax.dot_general(a, b, dims, preferred_element_type=f32)


def rows(*parts):
    return jnp.concatenate(parts, axis=0)


def cols(*parts):
    return jnp.concatenate(parts, axis=1)


def pack(v):
    return pltpu.bitcast(v.astype(bf16), i32)


def unpack(v):
    return pltpu.bitcast(v, bf16)


def alpha(z):
    (a, b), (c, d) = z
    return [a + d, c + d, a, d, a + b, c - a, b - d]


def alpha_entry(k, z):
    (r0, c0, _), *rest = ALPHA_TERMS[k]
    v = z(r0, c0)
    for r, c, sign in rest:
        v = v + z(r, c) if sign > 0 else v - z(r, c)
    return v


def beta(z):
    t = alpha(z)
    return [t[k] for k in PERM]


def gamma(n):
    return [[n[0] + n[3] - n[4] + n[6], n[2] + n[4]], [n[1] + n[3], n[0] - n[1] + n[2] + n[5]]]


def alpha2(g):
    def pair(u, v):
        (x, sx), (y, sy) = u, v
        if sx > 0:
            return (x + y if sy > 0 else x - y), 1
        return (y - x, 1) if sy > 0 else (x + y, -1)

    out = []
    for a in range(7):
        for k in range(7):
            t = [[(g[2 * r1 + r2][2 * c1 + c2], s1 * s2) for r2, c2, s2 in ALPHA_TERMS[k]]
                 for r1, c1, s1 in ALPHA_TERMS[a]]
            if len(t) == 2 and len(t[0]) == 2:
                v, sign = pair(pair(t[0][0], t[1][1]), pair(t[0][1], t[1][0]))
            else:
                flat = [e for row in t for e in row]
                v, sign = pair(*flat) if len(flat) == 2 else flat[0]
            assert sign > 0
            out.append(v)
    return out


def beta2(g):
    t = [[beta([[g[2 * r1 + r2][2 * c1 + c2] for c1 in range(2)] for r1 in range(2)])
          for c2 in range(2)] for r2 in range(2)]
    return [v for a in range(7) for v in beta([[t[r2][c2][a] for c2 in range(2)] for r2 in range(2)])]


def gamma2(n):
    inner = [gamma(n[7 * a:7 * a + 7]) for a in range(7)]
    out = [[None] * 4 for _ in range(4)]
    for r2 in range(2):
        for c2 in range(2):
            z = gamma([inner[a][r2][c2] for a in range(7)])
            for r1 in range(2):
                for c1 in range(2):
                    out[2 * r1 + r2][2 * c1 + c2] = z[r1][c1]
    return out


def transpose(z):
    return [list(r) for r in zip(*z)]


def quadrants(w):
    n, m = w.shape[0] // 2, w.shape[1] // 2
    return [[w[i * n:(i + 1) * n, j * m:(j + 1) * m] for j in range(2)] for i in range(2)]


def merge(g):
    return [[rows(*[cols(g[2 * r1 + r2][2 * c1], g[2 * r1 + r2][2 * c1 + 1]) for r2 in range(2)])
             for c1 in range(2)] for r1 in range(2)]


def split(z):
    q = [[quadrants(v) for v in row] for row in z]
    return [[q[r // 2][c // 2][r % 2][c % 2] for c in range(4)] for r in range(4)]


def tie(never, a, tokens):
    if not tokens:
        return a
    nr, nc = a.shape[0] // 8, a.shape[1] // 128
    cells = {}
    for j, t in enumerate(tokens):
        p = j * nr * nc // len(tokens)
        cells[p] = jnp.maximum(cells[p], t) if p in cells else t
    out = []
    for p in range(nr):
        row = []
        for c in range(nc):
            v = a[8 * p:8 * p + 8, 128 * c:128 * c + 128]
            t = cells.get(p * nc + c)
            if t is not None:
                v = jnp.where(never, t if t.dtype == a.dtype else pltpu.bitcast(t, a.dtype), v)
            row.append(v)
        out.append(cols(*row))
    return rows(*out)


def take(queue, n):
    out = queue[:n]
    del queue[:n]
    return out


def window(queue, lo, hi, n):
    m = hi - lo
    return [[]] * lo + [queue[k * len(queue) // m:(k + 1) * len(queue) // m] for k in range(m)] + [[]] * (n - hi)


def _kernel(x_hbm, wq_hbm, wk_hbm, wv_hbm, wao_hbm, wup_hbm, dw_hbm, wdn_hbm, wm_hbm, o_hbm,
            x_v, wq, wk, wup, dwv, wa, wb,
            wp_s,
            wf_s,
            xa_s,
            x_s,
            qc_s,
            g_s,
            dw_s, ob_s, wsem, xsem, osem, *, plan):
    B, _, TQ, D = x_hbm.shape
    K = dw_hbm.shape[0]
    NL = D // 128
    nb = -(-TQ // H)
    HL = TQ - (nb - 1) * H
    H2 = H // 2
    NT_ = sum(plan["VCH"])
    assert NL == 4 and K // 2 <= HALO <= HL and nb * H <= 128 * NT_

    wc = {n: pltpu.make_async_copy(s, d, wsem.at[k]) for k, (n, s, d) in enumerate([
        ("q", wq_hbm, wq), ("k", wk_hbm, wk), ("dw", dw_hbm, dwv),
        ("u", wup_hbm.at[:, 0:D], wup.at[0]), ("g", wup_hbm.at[:, D:2 * D], wup.at[1]),
        ("v", wv_hbm, wa.at[0]), ("dn", wdn_hbm, wa.at[1]),
        ("ao", wao_hbm, wb.at[0]), ("m0", wm_hbm.at[0:D], wb.at[1]), ("m1", wm_hbm.at[D:2 * D], wb.at[2])])}
    late = [wc[n] for n in ("v", "ao", "m0", "dn", "m1", "u", "dw")]
    cuts = list(range(0, nb * H, 2 * H)) + [TQ]
    xc = [pltpu.make_async_copy(x_hbm.at[0, :, pl.ds(a, e - a), :], x_v.at[0, :, pl.ds(a, e - a), :], xsem.at[n])
          for n, (a, e) in enumerate(zip(cuts[:-1], cuts[1:]))]
    late.append(pltpu.make_async_copy(x_hbm.at[pl.ds(1, B - 1)], x_v.at[pl.ds(1, B - 1), :, pl.ds(0, TQ), :],
                                      xsem.at[len(xc)]))

    def set_projection(n, w):
        for k, v in enumerate(beta(quadrants(w))):
            wp_s[n, k] = pack(v)

    def project(n, lhs, order=range(7)):
        res = [None] * 7
        for j, k in enumerate(order):
            res[k] = _dot(unpack(lhs(j, k)), unpack(wp_s[n, k]))
        return gamma(res)

    def normalize(b, r, n):
        rr = pl.ds(r if isinstance(r, int) else pl.multiple_of(r, 16), n)
        for h in range(4):
            xa_s[b, h, rr, :] = _ln(x_v[b, h, rr, :].astype(f32), EPS).astype(bf16)

    for c in (wc["q"], wc["k"], xc[0]):
        c.start()
    for b in range(B):
        for h in range(4):
            x_v[b, h, TQ:, :] = jnp.zeros((nb * H - TQ, D), x_v.dtype)
    for k in range(x_s.shape[0]):
        x_s[k, nb * H2:, :] = jnp.zeros((x_s.shape[1] - nb * H2, D // 2), i32)
    for c in range(NL):
        for h in range(4):
            g_s[nb, h, c, HALO + H:, :] = jnp.zeros((HALO, 128), f32)
        dw_s[c] = jnp.zeros(dw_s.shape[1:], f32)
    for c in (wc["q"], wc["k"]):
        c.wait()
    for c in (xc[1], wc["g"]):
        c.start()
    set_projection(0, _dot(wq[...], wk[...], NT) * (LOG2E * D ** -0.5))
    xc[2].start()

    @pl.loop(0, nb)
    def _(i):
        for k in range(len(xc)):
            @pl.when(i * H == cuts[k])
            def _():
                if k == 2:
                    wc["g"].wait()
                    set_projection(2, wup[1].astype(f32))
                xc[k].wait()
                for c in ((), (xc[3],), (), late)[k]:
                    c.start()
        normalize(0, i * H, H)

    def prepare(b, i):
        dst = pl.ds(pl.multiple_of(i * H2, 8), H2)
        rr = pl.ds(pl.multiple_of(i * H, 16), H)
        never = i < 0
        zero = pl.multiple_of(jnp.minimum(i, 0), 8)

        def tile(h, c):
            v = xa_s[b, h, rr, (c // 2) * 256:(c // 2 + 1) * 256].astype(f32)
            return v[:, (c % 2) * 128:(c % 2 + 1) * 128]

        x1, xq, left = [], [], []
        for a in range(7):
            z = [[alpha_entry(a, lambda r1, c1: tile(2 * r1 + r2, 2 * c1 + c2)) for c2 in range(2)] for r2 in range(2)]
            x1.append([pack(cols(*z[r2])) for r2 in range(2)])
            for r2 in range(2):
                x_s[2 * a + r2, dst, :] = x1[a][r2]
            l2 = left + [v for k, v in enumerate(alpha(z)) if k not in (2, 3)]
            if a == 6:
                l2.append(l2[-1])
            left = [l2.pop()] if len(l2) % 2 else []
            for k in range(len(l2) // 2):
                x_s[14 + 5 * a // 2 + k, dst, :] = pack(cols(l2[2 * k], l2[2 * k + 1]))
            xq.append(x_s[0, pl.ds(zero, 8), :128])
        xq = window(xq, *plan["XW"], 14)
        gpre = split(project(2, lambda j, k: tie(never, rows(*x1[k]), xq[j])))
        gq, GR = [], plan["GR"]
        for p in range(0, H, GR):
            for h in range(4):
                gate = _ln(_gelu2(cols(*[t[p:p + GR] for t in gpre[h]])), 4 * EPS)
                for c in range(NL):
                    t = gate[:, c * 128:(c + 1) * 128]
                    g_s[i + 1, h, c, HALO + p:HALO + p + GR, :] = t
                    if p < HALO:
                        g_s[i, h, c, HALO + H + p:HALO + H + min(p + GR, HALO), :] = t[:HALO - p]
                    if p + GR > H - HALO:
                        o = max(H - HALO - p, 0)
                        g_s[i + 2, h, c, p + o - (H - HALO):p + GR - (H - HALO), :] = t[o:]
            gq.append(pltpu.bitcast(g_s[i + 1, 0, 0, pl.ds(zero + HALO, 8), :], i32))
        gq = window(gq, *plan["GW"], 7)
        q = project(0, lambda j, k: tie(never, rows(*x1[k]), gq[j] + xq[7 + k]), plan["QO"])
        qn = beta2(transpose(split(q)))
        for k in range(25):
            qc_s[i, k] = cols(qn[2 * k], qn[min(2 * k + 1, 48)]).astype(bf16)

    def connect_quarters():
        zero = jnp.zeros((HALO, 128), f32)
        for c in range(NL):
            for h in range(4):
                g_s[nb, h, c, HALO + HL:2 * HALO + HL, :] = g_s[1, h + 1, c, HALO:2 * HALO, :] if h < 3 else zero
                g_s[1, h, c, 0:HALO, :] = g_s[nb, h - 1, c, HL:HL + HALO, :] if h else zero

    def merge_weights(b0):
        for c in late:
            c.wait()
        zero = pl.multiple_of(jnp.minimum(b0, 0), 16)
        tq = []
        for b in range(1, B):
            for p in range(0, nb * H, plan["MR"]):
                normalize(b, p, plan["MR"])
                tq.append(pltpu.bitcast(xa_s[b, 0, pl.ds(zero, 16), :128], i32))
        tq = [list(t) for t in window(tq, *plan["MW"], 12)]
        set_projection(1, wup[0].astype(f32))
        for c in range(NL):
            dw_s[c, 0:K, :] = dwv[:, c * 128:(c + 1) * 128].astype(f32) * 0.5
        tq[10].append(wp_s[1, 0, pl.ds(zero, 8), :128])

        def product(n, a, w):
            return cols(*[_dot(unpack(tie(b0 < 0, a, tq[4 * n + c])), wb[w, :, c * 128:(c + 1) * 128])
                          for c in range(4)])

        t = product(0, pltpu.bitcast(wa[0], i32), 0)
        for k, v in enumerate(beta(quadrants(product(1, pltpu.bitcast(wa[1], i32), 2)))):
            wf_s[k, D // 4:, :] = pack(v)
        tq[11].append(wf_s[0, pl.ds(zero + D // 4, 8), :128])
        for k, v in enumerate(beta(quadrants(product(2, pack(t), 1)))):
            wf_s[k, :D // 4, :] = pack(v)

    def out_copy(slot, b, r, n):
        return pltpu.make_async_copy(ob_s.at[slot, :, pl.ds(0, n), :], o_hbm.at[b, :, pl.ds(r, n), :], osem.at[slot])

    def step(b, i):
        r = pl.multiple_of(i * H, 16)
        never = i < 0
        it = b * nb + i
        slot = it % 2
        short = (i == 1) & (b > 0)
        pl.when(short)(lambda: out_copy(slot, 0, 0, HL).wait())
        pl.when((it > 1) & jnp.logical_not(short))(lambda: out_copy(slot, 0, 0, H).wait())

        CR = plan["CR"]
        todo = [(h, c, p) for h in range(4) for c in range(NL) for p in range(0, H, CR)]
        conv = {}

        def conv_pieces(n):
            out = []
            for h, c, p in take(todo, n):
                w = dw_s[c]
                acc = None
                for t in sorted(range(K), key=lambda t: (t % 8, t)):
                    term = g_s[i + 1, h, c, pl.ds(p + HALO - K // 2 + t, CR), :] * w[t:t + 1, :]
                    acc = term if acc is None else acc + term
                conv[h, c, p] = acc
                out.append([acc[k:k + 8] for k in range(0, CR, 8)])
            return out

        def keys(a, c, lo, hi):
            t = 4 * a if c == 2 else 4 * a + 3 if c == 3 else 28 + 5 * a + (c if c < 2 else c - 2)
            return unpack(x_s[t // 2, lo * 64:hi * 64, (t % 2) * 128:(t % 2 + 1) * 128])

        def win(queue, w):
            return window(queue, 7 * w[0], 7 * w[1], 49)

        qc = [pltpu.bitcast(qc_s[i, k // 2], i32)[:, (k % 2) * 128:(k % 2 + 1) * 128] for k in range(49)]
        s = [[[None] * NT_ for _ in range(4)] for _ in range(4)]
        m, l, statq = [None] * 4, [None] * 4, []
        for t in range(NT_):
            st = win(statq, plan["QW"])
            cq = win(conv_pieces(plan["QC"] if t == 0 else 0), plan["QCW"])
            res = [None] * 49
            for p, k in enumerate([7 * a + c for a in plan["AO"] for c in plan["IO"]]):
                res[k] = _dot(unpack(tie(never, qc[k], st[p] + sum(cq[p], []))), keys(k // 7, k % 7, t, t + 1), NT)
            z = transpose(gamma2(res))
            for h in range(4):
                new = []
                for c in range(4):
                    v = z[h][c]
                    if (t + 1) * 128 > TQ:
                        v = jnp.where(t * 128 + lax.broadcasted_iota(i32, v.shape, 1) < TQ, v, -jnp.inf)
                    s[h][c][t] = v
                    new.append(v)
                mx = functools.reduce(jnp.maximum, new)
                tot = None
                if m[h] is not None:
                    mx = jnp.maximum(m[h], mx)
                    tot = l[h] * jnp.exp2(m[h] - mx)
                for v in new:
                    e = jnp.exp2(v - mx)
                    tot = e if tot is None else tot + e
                m[h], l[h] = mx, tot
            statq = [l[h][p:p + 8] for p in range(0, H, 8) for h in range(4)]
        shift = []
        for h in range(4):
            mr = jnp.max(m[h], axis=-1, keepdims=True)
            shift.append(mr + jnp.log2(jnp.sum(l[h] * jnp.exp2(m[h] - mr), axis=-1, keepdims=True)))

        edges = [sum(plan["VCH"][:n]) for n in range(len(plan["VCH"]) + 1)]

        def probabilities(n):
            tiles = range(edges[n], edges[n + 1])
            g = [[cols(*[jnp.exp2(s[h][c][t] - shift[h]) for t in tiles]) for c in range(4)] for h in range(4)]
            return alpha2(g), [g[h][c][p:p + 8, t * 128:(t + 1) * 128] for p in range(0, H, 8)
                               for h in range(4) for c in range(4) for t in range(len(tiles))]

        operands, pq = probabilities(0)
        st, pq = window(statq, *plan["SW"], 7), window(pq, *plan["FW"], 7)
        r2 = pl.ds(pl.multiple_of(i * H2, 8), H2)
        upre = split(project(1, lambda j, k: tie(never, rows(x_s[2 * k, r2, :], x_s[2 * k + 1, r2, :]),
                                                 st[j] + pq[j]), plan["UO"]))

        acc, uq, nv = [None] * 49, [], len(plan["VCH"])
        for n in range(nv):
            following, pq = probabilities(n + 1) if n + 1 < nv else (None, [])
            pq = win(pq, plan["PW"][n]) if n + 1 < nv else [[]] * 49
            ug = win(uq if n == plan["UJ"] else [], plan["UW"])
            cg = win(conv_pieces(plan["CJ"][n]), plan["CW"][n])
            outer = plan["PL"] if n == nv - 1 else plan["PA"]
            for p, k in enumerate([7 * a + c for a in outer for c in plan["PI"]]):
                d = _dot(tie(never, operands[k], pq[p] + ug[p] + sum(cg[p], [])).astype(bf16),
                         keys(PERM[k // 7], PERM[k % 7], edges[n], edges[n + 1]))
                acc[k] = d if acc[k] is None else acc[k] + d
                if n == 0 and p == 7 * plan["US"]:
                    started = d
            operands = following
            if n == 0:
                u = [[_gelu2(jnp.where(never, started, v)) for v in row] for row in upre]
                uq = [v[p:p + 8] for row in u for v in row for p in range(0, H, 8)]

        cf = window(conv_pieces(len(todo)), *plan["FS"], 7)
        uc = [[u[h][c] * rows(*[conv[h, c, p] for p in range(0, H, CR)]) for c in range(4)] for h in range(4)]
        ao, ac = alpha(merge(gamma2(acc))), alpha(merge(uc))
        res = [None] * 7
        for n, k in enumerate(plan["FO"]):
            res[k] = _dot(tie(never, ao[k], sum(cf[n], [])).astype(bf16), unpack(wf_s[k, :D // 4, :]))
        for k in plan["FO"]:
            res[k] = res[k] + _dot(ac[k].astype(bf16), unpack(wf_s[k, D // 4:, :]))
        out = split(gamma(res))
        for h in range(4):
            ob_s[slot, h] = (x_v[b, h, pl.ds(r, H), :].astype(f32) + cols(*out[h])).astype(ob_s.dtype)
        pl.when(i < nb - 1)(lambda: out_copy(slot, b, r, H).start())
        pl.when(i == nb - 1)(lambda: out_copy(slot, b, r, HL).start())

    @pl.loop(0, B)
    def _(b):
        pl.loop(0, nb)(functools.partial(prepare, b))
        connect_quarters()
        pl.when(b == 0)(lambda: merge_weights(b))
        pl.loop(0, nb)(functools.partial(step, b))

    out_copy((B * nb) % 2, 0, 0, H).wait()
    out_copy((B * nb + 1) % 2, 0, 0, HL).wait()


def _call(x, w_q, w_k, w_v, w_ao, w_up, dw, w_dn, w_merge, plan):
    B, T, D = x.shape
    TQ = T // 4
    nb = -(-TQ // H)
    hbm = pl.BlockSpec(memory_space=pl.ANY)
    out = pl.pallas_call(
        functools.partial(_kernel, plan=plan),
        in_specs=[hbm] * 9,
        out_specs=hbm,
        out_shape=jax.ShapeDtypeStruct((B, 4, TQ, D), x.dtype),
        scratch_shapes=[
            pltpu.VMEM((B, 4, nb * H, D), x.dtype),
            pltpu.VMEM(w_q.shape, w_q.dtype),
            pltpu.VMEM(w_k.shape, w_k.dtype),
            pltpu.VMEM((2, D, D), w_up.dtype),
            pltpu.VMEM(dw.shape, dw.dtype),
            pltpu.VMEM((2, D, D), bf16),
            pltpu.VMEM((3, D, D), bf16),
            pltpu.VMEM((3, 7, D // 4, D // 2), i32),
            pltpu.VMEM((7, D // 2, D // 2), i32),
            pltpu.VMEM((B, 4, nb * H, D), bf16),
            pltpu.VMEM((32, 64 * sum(plan["VCH"]), D // 2), i32),
            pltpu.VMEM((nb, 32, H, D // 2), bf16),
            pltpu.VMEM((nb + 2, 4, D // 128, H + 2 * HALO, 128), f32),
            pltpu.VMEM((D // 128, 2 * HALO, 128), f32),
            pltpu.VMEM((2, 4, H, D), x.dtype),
            pltpu.SemaphoreType.DMA((10,)),
            pltpu.SemaphoreType.DMA((-(-nb // 2) + 1,)),
            pltpu.SemaphoreType.DMA((2,)),
        ],
        compiler_params=pltpu.CompilerParams(vmem_limit_bytes=112 * 1024 * 1024),
    )(x.reshape(B, 4, TQ, D), w_q, w_k, w_v, w_ao, w_up, dw, w_dn, w_merge)
    return out.reshape(B, T, D)


@jax.jit
def pallas_standalone__conformer_family_branchformer__speech_kernel(
    x: jax.Array,
    w_q: jax.Array,
    w_k: jax.Array,
    w_v: jax.Array,
    w_ao: jax.Array,
    w_up: jax.Array,
    dw: jax.Array,
    w_dn: jax.Array,
    w_merge: jax.Array,
):
    return _call(x, w_q, w_k, w_v, w_ao, w_up, dw, w_dn, w_merge, PLAN)
```

```python
import functools

import jax
import jax.numpy as jnp
import numpy as np
from jax import lax
import jax.experimental.pallas as pl
import jax.experimental.pallas.tpu as pltpu

bf16, f32, i32 = jnp.bfloat16, jnp.float32, jnp.int32
LOG2E = 1.4426950408889634
EPS = 1e-5
NN = (((1,), (0,)), ((), ()))
NT = (((1,), (1,)), ((), ()))

H = 144
HALO = 16
PERM = (0, 2, 6, 5, 3, 4, 1)
ALPHA_TERMS = (((0, 0, 1), (1, 1, 1)), ((1, 0, 1), (1, 1, 1)), ((0, 0, 1),), ((1, 1, 1),),
               ((0, 0, 1), (0, 1, 1)), ((1, 0, 1), (0, 0, -1)), ((0, 1, 1), (1, 1, -1)))

PLAN = dict(
    MR=48, MW=(1, 11),
    XW=(2, 14), GR=24, GW=(2, 5), QO=(0, 1, 2, 5, 4, 3, 6),
    AO=(0, 2, 1, 5, 4, 3, 6), IO=(0, 1, 3, 2, 5, 4, 6), QW=(1, 7), CR=48, QC=6, QCW=(0, 3),
    UO=(1, 3, 2, 4, 0, 5, 6), SW=(0, 2), FW=(5, 7),
    VCH=(2, 2, 4), PA=(0, 1, 2, 3, 4, 5, 6), PL=(4, 5, 2, 3, 0, 1, 6), PI=(2, 3, 0, 1, 4, 5, 6),
    PW=((4, 7), (4, 7)), CJ=(4, 8, 14), CW=((2, 4), (2, 4), (2, 4)), US=4, UJ=2, UW=(0, 2),
    FO=(3, 1, 6, 2, 0, 4, 5), FS=(0, 7),
)


def _ln(x, eps):
    d = x - jnp.mean(x, axis=-1, keepdims=True)
    v = jnp.mean(d * d, axis=-1, keepdims=True)
    return d * jnp.exp2(jnp.log(v + eps) * (-0.5 * LOG2E))


def _gelu2(x):
    c = float(np.sqrt(2.0 / np.pi))
    return x * jnp.tanh((x * x * (0.044715 * c) + c) * x) + x


def _dot(a, b, dims=NN):
    return lax.dot_general(a, b, dims, preferred_element_type=f32)


def rows(*parts):
    return jnp.concatenate(parts, axis=0)


def cols(*parts):
    return jnp.concatenate(parts, axis=1)


def pack(v):
    return pltpu.bitcast(v.astype(bf16), i32)


def unpack(v):
    return pltpu.bitcast(v, bf16)


def alpha(z):
    (a, b), (c, d) = z
    return [a + d, c + d, a, d, a + b, c - a, b - d]


def alpha_entry(k, z):
    (r0, c0, _), *rest = ALPHA_TERMS[k]
    v = z(r0, c0)
    for r, c, sign in rest:
        v = v + z(r, c) if sign > 0 else v - z(r, c)
    return v


def beta(z):
    t = alpha(z)
    return [t[k] for k in PERM]


def gamma(n):
    return [[n[0] + n[3] - n[4] + n[6], n[2] + n[4]], [n[1] + n[3], n[0] - n[1] + n[2] + n[5]]]


def alpha2(g):
    def pair(u, v):
        (x, sx), (y, sy) = u, v
        if sx > 0:
            return (x + y if sy > 0 else x - y), 1
        return (y - x, 1) if sy > 0 else (x + y, -1)

    out = []
    for a in range(7):
        for k in range(7):
            t = [[(g[2 * r1 + r2][2 * c1 + c2], s1 * s2) for r2, c2, s2 in ALPHA_TERMS[k]]
                 for r1, c1, s1 in ALPHA_TERMS[a]]
            if len(t) == 2 and len(t[0]) == 2:
                v, sign = pair(pair(t[0][0], t[1][1]), pair(t[0][1], t[1][0]))
            else:
                flat = [e for row in t for e in row]
                v, sign = pair(*flat) if len(flat) == 2 else flat[0]
            assert sign > 0
            out.append(v)
    return out


def beta2(g):
    t = [[beta([[g[2 * r1 + r2][2 * c1 + c2] for c1 in range(2)] for r1 in range(2)])
          for c2 in range(2)] for r2 in range(2)]
    return [v for a in range(7) for v in beta([[t[r2][c2][a] for c2 in range(2)] for r2 in range(2)])]


def gamma2(n):
    inner = [gamma(n[7 * a:7 * a + 7]) for a in range(7)]
    out = [[None] * 4 for _ in range(4)]
    for r2 in range(2):
        for c2 in range(2):
            z = gamma([inner[a][r2][c2] for a in range(7)])
            for r1 in range(2):
                for c1 in range(2):
                    out[2 * r1 + r2][2 * c1 + c2] = z[r1][c1]
    return out


def transpose(z):
    return [list(r) for r in zip(*z)]


def quadrants(w):
    n, m = w.shape[0] // 2, w.shape[1] // 2
    return [[w[i * n:(i + 1) * n, j * m:(j + 1) * m] for j in range(2)] for i in range(2)]


def merge(g):
    return [[rows(*[cols(g[2 * r1 + r2][2 * c1], g[2 * r1 + r2][2 * c1 + 1]) for r2 in range(2)])
             for c1 in range(2)] for r1 in range(2)]


def split(z):
    q = [[quadrants(v) for v in row] for row in z]
    return [[q[r // 2][c // 2][r % 2][c % 2] for c in range(4)] for r in range(4)]


def tie(never, a, tokens):
    if not tokens:
        return a
    nr, nc = a.shape[0] // 8, a.shape[1] // 128
    cells = {}
    for j, t in enumerate(tokens):
        p = j * nr * nc // len(tokens)
        cells[p] = jnp.maximum(cells[p], t) if p in cells else t
    out = []
    for p in range(nr):
        row = []
        for c in range(nc):
            v = a[8 * p:8 * p + 8, 128 * c:128 * c + 128]
            t = cells.get(p * nc + c)
            if t is not None:
                v = jnp.where(never, t if t.dtype == a.dtype else pltpu.bitcast(t, a.dtype), v)
            row.append(v)
        out.append(cols(*row))
    return rows(*out)


def take(queue, n):
    out = queue[:n]
    del queue[:n]
    return out


def window(queue, lo, hi, n):
    m = hi - lo
    return [[]] * lo + [queue[k * len(queue) // m:(k + 1) * len(queue) // m] for k in range(m)] + [[]] * (n - hi)


def _kernel(x_hbm, wq_hbm, wk_hbm, wv_hbm, wao_hbm, wup_hbm, dw_hbm, wdn_hbm, wm_hbm, o_hbm,
            x_v, wq, wk, wup, dwv, wa, wb,
            wp_s,
            wf_s,
            xa_s,
            x_s,
            qc_s,
            g_s,
            dw_s, ob_s, wsem, xsem, osem, *, plan):
    B, _, TQ, D = x_hbm.shape
    K = dw_hbm.shape[0]
    NL = D // 128
    nb = -(-TQ // H)
    HL = TQ - (nb - 1) * H
    H2 = H // 2
    NT_ = sum(plan["VCH"])
    assert NL == 4 and K // 2 <= HALO <= HL and nb * H <= 128 * NT_

    wc = {n: pltpu.make_async_copy(s, d, wsem.at[k]) for k, (n, s, d) in enumerate([
        ("q", wq_hbm, wq), ("k", wk_hbm, wk), ("dw", dw_hbm, dwv),
        ("u", wup_hbm.at[:, 0:D], wup.at[0]), ("g", wup_hbm.at[:, D:2 * D], wup.at[1]),
        ("v", wv_hbm, wa.at[0]), ("dn", wdn_hbm, wa.at[1]),
        ("ao", wao_hbm, wb.at[0]), ("m0", wm_hbm.at[0:D], wb.at[1]), ("m1", wm_hbm.at[D:2 * D], wb.at[2])])}
    late = [wc[n] for n in ("v", "ao", "m0", "dn", "m1", "u", "dw")]
    cuts = list(range(0, nb * H, 2 * H)) + [TQ]
    xc = [pltpu.make_async_copy(x_hbm.at[0, :, pl.ds(a, e - a), :], x_v.at[0, :, pl.ds(a, e - a), :], xsem.at[n])
          for n, (a, e) in enumerate(zip(cuts[:-1], cuts[1:]))]
    late.append(pltpu.make_async_copy(x_hbm.at[pl.ds(1, B - 1)], x_v.at[pl.ds(1, B - 1), :, pl.ds(0, TQ), :],
                                      xsem.at[len(xc)]))

    def set_projection(n, w):
        for k, v in enumerate(beta(quadrants(w))):
            wp_s[n, k] = pack(v)

    def project(n, lhs, order=range(7)):
        res = [None] * 7
        for j, k in enumerate(order):
            res[k] = _dot(unpack(lhs(j, k)), unpack(wp_s[n, k]))
        return gamma(res)

    def normalize(b, r, n):
        rr = pl.ds(r if isinstance(r, int) else pl.multiple_of(r, 16), n)
        for h in range(4):
            xa_s[b, h, rr, :] = _ln(x_v[b, h, rr, :].astype(f32), EPS).astype(bf16)

    for c in (wc["q"], wc["k"], xc[0]):
        c.start()
    for b in range(B):
        for h in range(4):
            x_v[b, h, TQ:, :] = jnp.zeros((nb * H - TQ, D), x_v.dtype)
    for k in range(x_s.shape[0]):
        x_s[k, nb * H2:, :] = jnp.zeros((x_s.shape[1] - nb * H2, D // 2), i32)
    for c in range(NL):
        for h in range(4):
            g_s[nb, h, c, HALO + H:, :] = jnp.zeros((HALO, 128), f32)
        dw_s[c] = jnp.zeros(dw_s.shape[1:], f32)
    for c in (wc["q"], wc["k"]):
        c.wait()
    for c in (xc[1], wc["g"]):
        c.start()
    set_projection(0, _dot(wq[...], wk[...], NT) * (LOG2E * D ** -0.5))
    xc[2].start()

    @pl.loop(0, nb)
    def _(i):
        for k in range(len(xc)):
            @pl.when(i * H == cuts[k])
            def _():
                if k == 2:
                    wc["g"].wait()
                    set_projection(2, wup[1].astype(f32))
                xc[k].wait()
                for c in ((), (xc[3],), (), late)[k]:
                    c.start()
        normalize(0, i * H, H)

    def prepare(b, i):
        dst = pl.ds(pl.multiple_of(i * H2, 8), H2)
        rr = pl.ds(pl.multiple_of(i * H, 16), H)
        never = i < 0
        zero = pl.multiple_of(jnp.minimum(i, 0), 8)

        def tile(h, c):
            v = xa_s[b, h, rr, (c // 2) * 256:(c // 2 + 1) * 256].astype(f32)
            return v[:, (c % 2) * 128:(c % 2 + 1) * 128]

        x1, xq, left = [], [], []
        for a in range(7):
            z = [[alpha_entry(a, lambda r1, c1: tile(2 * r1 + r2, 2 * c1 + c2)) for c2 in range(2)] for r2 in range(2)]
            x1.append([pack(cols(*z[r2])) for r2 in range(2)])
            for r2 in range(2):
                x_s[2 * a + r2, dst, :] = x1[a][r2]
            l2 = left + [v for k, v in enumerate(alpha(z)) if k not in (2, 3)]
            if a == 6:
                l2.append(l2[-1])
            left = [l2.pop()] if len(l2) % 2 else []
            for k in range(len(l2) // 2):
                x_s[14 + 5 * a // 2 + k, dst, :] = pack(cols(l2[2 * k], l2[2 * k + 1]))
            xq.append(x_s[0, pl.ds(zero, 8), :128])
        xq = window(xq, *plan["XW"], 14)
        gpre = split(project(2, lambda j, k: tie(never, rows(*x1[k]), xq[j])))
        gq, GR = [], plan["GR"]
        for p in range(0, H, GR):
            for h in range(4):
                gate = _ln(_gelu2(cols(*[t[p:p + GR] for t in gpre[h]])), 4 * EPS)
                for c in range(NL):
                    t = gate[:, c * 128:(c + 1) * 128]
                    g_s[i + 1, h, c, HALO + p:HALO + p + GR, :] = t
                    if p < HALO:
                        g_s[i, h, c, HALO + H + p:HALO + H + min(p + GR, HALO), :] = t[:HALO - p]
                    if p + GR > H - HALO:
                        o = max(H - HALO - p, 0)
                        g_s[i + 2, h, c, p + o - (H - HALO):p + GR - (H - HALO), :] = t[o:]
            gq.append(pltpu.bitcast(g_s[i + 1, 0, 0, pl.ds(zero + HALO, 8), :], i32))
        gq = window(gq, *plan["GW"], 7)
        q = project(0, lambda j, k: tie(never, rows(*x1[k]), gq[j] + xq[7 + k]), plan["QO"])
        qn = beta2(transpose(split(q)))
        for k in range(25):
            qc_s[i, k] = cols(qn[2 * k], qn[min(2 * k + 1, 48)]).astype(bf16)

    def connect_quarters():
        zero = jnp.zeros((HALO, 128), f32)
        for c in range(NL):
            for h in range(4):
                g_s[nb, h, c, HALO + HL:2 * HALO + HL, :] = g_s[1, h + 1, c, HALO:2 * HALO, :] if h < 3 else zero
                g_s[1, h, c, 0:HALO, :] = g_s[nb, h - 1, c, HL:HL + HALO, :] if h else zero

    def merge_weights(b0):
        for c in late:
            c.wait()
        zero = pl.multiple_of(jnp.minimum(b0, 0), 16)
        tq = []
        for b in range(1, B):
            for p in range(0, nb * H, plan["MR"]):
                normalize(b, p, plan["MR"])
                tq.append(pltpu.bitcast(xa_s[b, 0, pl.ds(zero, 16), :128], i32))
        tq = [list(t) for t in window(tq, *plan["MW"], 12)]
        set_projection(1, wup[0].astype(f32))
        for c in range(NL):
            dw_s[c, 0:K, :] = dwv[:, c * 128:(c + 1) * 128].astype(f32) * 0.5
        tq[10].append(wp_s[1, 0, pl.ds(zero, 8), :128])

        def product(n, a, w):
            return cols(*[_dot(unpack(tie(b0 < 0, a, tq[4 * n + c])), wb[w, :, c * 128:(c + 1) * 128])
                          for c in range(4)])

        t = product(0, pltpu.bitcast(wa[0], i32), 0)
        for k, v in enumerate(beta(quadrants(product(1, pltpu.bitcast(wa[1], i32), 2)))):
            wf_s[k, D // 4:, :] = pack(v)
        tq[11].append(wf_s[0, pl.ds(zero + D // 4, 8), :128])
        for k, v in enumerate(beta(quadrants(product(2, pack(t), 1)))):
            wf_s[k, :D // 4, :] = pack(v)

    def out_copy(slot, b, r, n):
        return pltpu.make_async_copy(ob_s.at[slot, :, pl.ds(0, n), :], o_hbm.at[b, :, pl.ds(r, n), :], osem.at[slot])

    def step(b, i):
        r = pl.multiple_of(i * H, 16)
        never = i < 0
        it = b * nb + i
        slot = it % 2
        short = (i == 1) & (b > 0)
        pl.when(short)(lambda: out_copy(slot, 0, 0, HL).wait())
        pl.when((it > 1) & jnp.logical_not(short))(lambda: out_copy(slot, 0, 0, H).wait())

        CR = plan["CR"]
        todo = [(h, c, p) for h in range(4) for c in range(NL) for p in range(0, H, CR)]
        conv = {}

        def conv_pieces(n):
            out = []
            for h, c, p in take(todo, n):
                w = dw_s[c]
                acc = None
                for t in sorted(range(K), key=lambda t: (t % 8, t)):
                    term = g_s[i + 1, h, c, pl.ds(p + HALO - K // 2 + t, CR), :] * w[t:t + 1, :]
                    acc = term if acc is None else acc + term
                conv[h, c, p] = acc
                out.append([acc[k:k + 8] for k in range(0, CR, 8)])
            return out

        def keys(a, c, lo, hi):
            t = 4 * a if c == 2 else 4 * a + 3 if c == 3 else 28 + 5 * a + (c if c < 2 else c - 2)
            return unpack(x_s[t // 2, lo * 64:hi * 64, (t % 2) * 128:(t % 2 + 1) * 128])

        def win(queue, w):
            return window(queue, 7 * w[0], 7 * w[1], 49)

        qc = [pltpu.bitcast(qc_s[i, k // 2], i32)[:, (k % 2) * 128:(k % 2 + 1) * 128] for k in range(49)]
        s = [[[None] * NT_ for _ in range(4)] for _ in range(4)]
        m, l, statq = [None] * 4, [None] * 4, []
        for t in range(NT_):
            st = win(statq, plan["QW"])
            cq = win(conv_pieces(plan["QC"] if t == 0 else 0), plan["QCW"])
            res = [None] * 49
            for p, k in enumerate([7 * a + c for a in plan["AO"] for c in plan["IO"]]):
                res[k] = _dot(unpack(tie(never, qc[k], st[p] + sum(cq[p], []))), keys(k // 7, k % 7, t, t + 1), NT)
            z = transpose(gamma2(res))
            for h in range(4):
                new = []
                for c in range(4):
                    v = z[h][c]
                    if (t + 1) * 128 > TQ:
                        v = jnp.where(t * 128 + lax.broadcasted_iota(i32, v.shape, 1) < TQ, v, -jnp.inf)
                    s[h][c][t] = v
                    new.append(v)
                mx = functools.reduce(jnp.maximum, new)
                tot = None
                if m[h] is not None:
                    mx = jnp.maximum(m[h], mx)
                    tot = l[h] * jnp.exp2(m[h] - mx)
                for v in new:
                    e = jnp.exp2(v - mx)
                    tot = e if tot is None else tot + e
                m[h], l[h] = mx, tot
            statq = [l[h][p:p + 8] for p in range(0, H, 8) for h in range(4)]
        shift = []
        for h in range(4):
            mr = jnp.max(m[h], axis=-1, keepdims=True)
            shift.append(mr + jnp.log2(jnp.sum(l[h] * jnp.exp2(m[h] - mr), axis=-1, keepdims=True)))

        edges = [sum(plan["VCH"][:n]) for n in range(len(plan["VCH"]) + 1)]

        def probabilities(n):
            tiles = range(edges[n], edges[n + 1])
            g = [[cols(*[jnp.exp2(s[h][c][t] - shift[h]) for t in tiles]) for c in range(4)] for h in range(4)]
            return alpha2(g), [g[h][c][p:p + 8, t * 128:(t + 1) * 128] for p in range(0, H, 8)
                               for h in range(4) for c in range(4) for t in range(len(tiles))]

        operands, pq = probabilities(0)
        st, pq = window(statq, *plan["SW"], 7), window(pq, *plan["FW"], 7)
        r2 = pl.ds(pl.multiple_of(i * H2, 8), H2)
        upre = split(project(1, lambda j, k: tie(never, rows(x_s[2 * k, r2, :], x_s[2 * k + 1, r2, :]),
                                                 st[j] + pq[j]), plan["UO"]))

        acc, uq, nv = [None] * 49, [], len(plan["VCH"])
        for n in range(nv):
            following, pq = probabilities(n + 1) if n + 1 < nv else (None, [])
            pq = win(pq, plan["PW"][n]) if n + 1 < nv else [[]] * 49
            ug = win(uq if n == plan["UJ"] else [], plan["UW"])
            cg = win(conv_pieces(plan["CJ"][n]), plan["CW"][n])
            outer = plan["PL"] if n == nv - 1 else plan["PA"]
            for p, k in enumerate([7 * a + c for a in outer for c in plan["PI"]]):
                d = _dot(tie(never, operands[k], pq[p] + ug[p] + sum(cg[p], [])).astype(bf16),
                         keys(PERM[k // 7], PERM[k % 7], edges[n], edges[n + 1]))
                acc[k] = d if acc[k] is None else acc[k] + d
                if n == 0 and p == 7 * plan["US"]:
                    started = d
            operands = following
            if n == 0:
                u = [[_gelu2(jnp.where(never, started, v)) for v in row] for row in upre]
                uq = [v[p:p + 8] for row in u for v in row for p in range(0, H, 8)]

        cf = window(conv_pieces(len(todo)), *plan["FS"], 7)
        uc = [[u[h][c] * rows(*[conv[h, c, p] for p in range(0, H, CR)]) for c in range(4)] for h in range(4)]
        ao, ac = alpha(merge(gamma2(acc))), alpha(merge(uc))
        res = [None] * 7
        for n, k in enumerate(plan["FO"]):
            res[k] = _dot(tie(never, ao[k], sum(cf[n], [])).astype(bf16), unpack(wf_s[k, :D // 4, :]))
        for k in plan["FO"]:
            res[k] = res[k] + _dot(ac[k].astype(bf16), unpack(wf_s[k, D // 4:, :]))
        out = split(gamma(res))
        for h in range(4):
            ob_s[slot, h] = (x_v[b, h, pl.ds(r, H), :].astype(f32) + cols(*out[h])).astype(ob_s.dtype)
        pl.when(i < nb - 1)(lambda: out_copy(slot, b, r, H).start())
        pl.when(i == nb - 1)(lambda: out_copy(slot, b, r, HL).start())

    @pl.loop(0, B)
    def _(b):
        pl.loop(0, nb)(functools.partial(prepare, b))
        connect_quarters()
        pl.when(b == 0)(lambda: merge_weights(b))
        pl.loop(0, nb)(functools.partial(step, b))

    out_copy((B * nb) % 2, 0, 0, H).wait()
    out_copy((B * nb + 1) % 2, 0, 0, HL).wait()


def _call(x, w_q, w_k, w_v, w_ao, w_up, dw, w_dn, w_merge, plan):
    B, T, D = x.shape
    TQ = T // 4
    nb = -(-TQ // H)
    hbm = pl.BlockSpec(memory_space=pl.ANY)
    out = pl.pallas_call(
        functools.partial(_kernel, plan=plan),
        in_specs=[hbm] * 9,
        out_specs=hbm,
        out_shape=jax.ShapeDtypeStruct((B, 4, TQ, D), x.dtype),
        scratch_shapes=[
            pltpu.VMEM((B, 4, nb * H, D), x.dtype),
            pltpu.VMEM(w_q.shape, w_q.dtype),
            pltpu.VMEM(w_k.shape, w_k.dtype),
            pltpu.VMEM((2, D, D), w_up.dtype),
            pltpu.VMEM(dw.shape, dw.dtype),
            pltpu.VMEM((2, D, D), bf16),
            pltpu.VMEM((3, D, D), bf16),
            pltpu.VMEM((3, 7, D // 4, D // 2), i32),
            pltpu.VMEM((7, D // 2, D // 2), i32),
            pltpu.VMEM((B, 4, nb * H, D), bf16),
            pltpu.VMEM((32, 64 * sum(plan["VCH"]), D // 2), i32),
            pltpu.VMEM((nb, 32, H, D // 2), bf16),
            pltpu.VMEM((nb + 2, 4, D // 128, H + 2 * HALO, 128), f32),
            pltpu.VMEM((D // 128, 2 * HALO, 128), f32),
            pltpu.VMEM((2, 4, H, D), x.dtype),
            pltpu.SemaphoreType.DMA((10,)),
            pltpu.SemaphoreType.DMA((-(-nb // 2) + 1,)),
            pltpu.SemaphoreType.DMA((2,)),
        ],
        compiler_params=pltpu.CompilerParams(vmem_limit_bytes=112 * 1024 * 1024),
    )(x.reshape(B, 4, TQ, D), w_q, w_k, w_v, w_ao, w_up, dw, w_dn, w_merge)
    return out.reshape(B, T, D)


@jax.jit
def pallas_standalone__conformer_family_branchformer__speech_kernel(
    x: jax.Array,
    w_q: jax.Array,
    w_k: jax.Array,
    w_v: jax.Array,
    w_ao: jax.Array,
    w_up: jax.Array,
    dw: jax.Array,
    w_dn: jax.Array,
    w_merge: jax.Array,
):
    return _call(x, w_q, w_k, w_v, w_ao, w_up, dw, w_dn, w_merge, PLAN)
```

```python
import functools

import jax
import jax.numpy as jnp
import numpy as np
from jax import lax
import jax.experimental.pallas as pl
import jax.experimental.pallas.tpu as pltpu

bf16, f32, i32 = jnp.bfloat16, jnp.float32, jnp.int32
LOG2E = 1.4426950408889634
EPS = 1e-5
NN = (((1,), (0,)), ((), ()))
NT = (((1,), (1,)), ((), ()))

H = 144
HALO = 16
PERM = (0, 2, 6, 5, 3, 4, 1)
ALPHA_TERMS = (((0, 0, 1), (1, 1, 1)), ((1, 0, 1), (1, 1, 1)), ((0, 0, 1),), ((1, 1, 1),),
               ((0, 0, 1), (0, 1, 1)), ((1, 0, 1), (0, 0, -1)), ((0, 1, 1), (1, 1, -1)))

PLAN = dict(
    MR=48, MW=(1, 11),
    XW=(2, 14), GR=24, GW=(2, 5), QO=(0, 1, 2, 5, 4, 3, 6),
    AO=(0, 2, 1, 5, 4, 3, 6), IO=(0, 1, 3, 2, 5, 4, 6), QW=(1, 7), CR=48, QC=6, QCW=(0, 3),
    UO=(1, 3, 2, 4, 0, 5, 6), SW=(0, 2), FW=(5, 7),
    VCH=(2, 2, 4), PA=(0, 1, 2, 3, 4, 5, 6), PL=(4, 5, 2, 3, 0, 1, 6), PI=(2, 3, 0, 1, 4, 5, 6),
    PW=((4, 7), (4, 7)), CJ=(4, 8, 14), CW=((2, 4), (2, 4), (2, 4)), US=4, UJ=2, UW=(0, 2),
    FO=(3, 1, 6, 2, 0, 4, 5), FS=(0, 7),
)


def _ln(x, eps):
    d = x - jnp.mean(x, axis=-1, keepdims=True)
    v = jnp.mean(d * d, axis=-1, keepdims=True)
    return d * jnp.exp2(jnp.log(v + eps) * (-0.5 * LOG2E))


def _gelu2(x):
    c = float(np.sqrt(2.0 / np.pi))
    return x * jnp.tanh((x * x * (0.044715 * c) + c) * x) + x


def _dot(a, b, dims=NN):
    return lax.dot_general(a, b, dims, preferred_element_type=f32)


def rows(*parts):
    return jnp.concatenate(parts, axis=0)


def cols(*parts):
    return jnp.concatenate(parts, axis=1)


def pack(v):
    return pltpu.bitcast(v.astype(bf16), i32)


def unpack(v):
    return pltpu.bitcast(v, bf16)


def alpha(z):
    (a, b), (c, d) = z
    return [a + d, c + d, a, d, a + b, c - a, b - d]


def alpha_entry(k, z):
    (r0, c0, _), *rest = ALPHA_TERMS[k]
    v = z(r0, c0)
    for r, c, sign in rest:
        v = v + z(r, c) if sign > 0 else v - z(r, c)
    return v


def beta(z):
    t = alpha(z)
    return [t[k] for k in PERM]


def gamma(n):
    return [[n[0] + n[3] - n[4] + n[6], n[2] + n[4]], [n[1] + n[3], n[0] - n[1] + n[2] + n[5]]]


def alpha2(g):
    def pair(u, v):
        (x, sx), (y, sy) = u, v
        if sx > 0:
            return (x + y if sy > 0 else x - y), 1
        return (y - x, 1) if sy > 0 else (x + y, -1)

    out = []
    for a in range(7):
        for k in range(7):
            t = [[(g[2 * r1 + r2][2 * c1 + c2], s1 * s2) for r2, c2, s2 in ALPHA_TERMS[k]]
                 for r1, c1, s1 in ALPHA_TERMS[a]]
            if len(t) == 2 and len(t[0]) == 2:
                v, sign = pair(pair(t[0][0], t[1][1]), pair(t[0][1], t[1][0]))
            else:
                flat = [e for row in t for e in row]
                v, sign = pair(*flat) if len(flat) == 2 else flat[0]
            assert sign > 0
            out.append(v)
    return out


def beta2(g):
    t = [[beta([[g[2 * r1 + r2][2 * c1 + c2] for c1 in range(2)] for r1 in range(2)])
          for c2 in range(2)] for r2 in range(2)]
    return [v for a in range(7) for v in beta([[t[r2][c2][a] for c2 in range(2)] for r2 in range(2)])]


def gamma2(n):
    inner = [gamma(n[7 * a:7 * a + 7]) for a in range(7)]
    out = [[None] * 4 for _ in range(4)]
    for r2 in range(2):
        for c2 in range(2):
            z = gamma([inner[a][r2][c2] for a in range(7)])
            for r1 in range(2):
                for c1 in range(2):
                    out[2 * r1 + r2][2 * c1 + c2] = z[r1][c1]
    return out


def transpose(z):
    return [list(r) for r in zip(*z)]


def quadrants(w):
    n, m = w.shape[0] // 2, w.shape[1] // 2
    return [[w[i * n:(i + 1) * n, j * m:(j + 1) * m] for j in range(2)] for i in range(2)]


def merge(g):
    return [[rows(*[cols(g[2 * r1 + r2][2 * c1], g[2 * r1 + r2][2 * c1 + 1]) for r2 in range(2)])
             for c1 in range(2)] for r1 in range(2)]


def split(z):
    q = [[quadrants(v) for v in row] for row in z]
    return [[q[r // 2][c // 2][r % 2][c % 2] for c in range(4)] for r in range(4)]


def tie(never, a, tokens):
    if not tokens:
        return a
    nr, nc = a.shape[0] // 8, a.shape[1] // 128
    cells = {}
    for j, t in enumerate(tokens):
        p = j * nr * nc // len(tokens)
        cells[p] = jnp.maximum(cells[p], t) if p in cells else t
    out = []
    for p in range(nr):
        row = []
        for c in range(nc):
            v = a[8 * p:8 * p + 8, 128 * c:128 * c + 128]
            t = cells.get(p * nc + c)
            if t is not None:
                v = jnp.where(never, t if t.dtype == a.dtype else pltpu.bitcast(t, a.dtype), v)
            row.append(v)
        out.append(cols(*row))
    return rows(*out)


def take(queue, n):
    out = queue[:n]
    del queue[:n]
    return out


def window(queue, lo, hi, n):
    m = hi - lo
    return [[]] * lo + [queue[k * len(queue) // m:(k + 1) * len(queue) // m] for k in range(m)] + [[]] * (n - hi)


def _kernel(x_hbm, wq_hbm, wk_hbm, wv_hbm, wao_hbm, wup_hbm, dw_hbm, wdn_hbm, wm_hbm, o_hbm,
            x_v, wq, wk, wup, dwv, wa, wb,
            wp_s,
            wf_s,
            xa_s,
            x_s,
            qc_s,
            g_s,
            dw_s, ob_s, wsem, xsem, osem, *, plan):
    B, _, TQ, D = x_hbm.shape
    K = dw_hbm.shape[0]
    NL = D // 128
    nb = -(-TQ // H)
    HL = TQ - (nb - 1) * H
    H2 = H // 2
    NT_ = sum(plan["VCH"])
    assert NL == 4 and K // 2 <= HALO <= HL and nb * H <= 128 * NT_

    wc = {n: pltpu.make_async_copy(s, d, wsem.at[k]) for k, (n, s, d) in enumerate([
        ("q", wq_hbm, wq), ("k", wk_hbm, wk), ("dw", dw_hbm, dwv),
        ("u", wup_hbm.at[:, 0:D], wup.at[0]), ("g", wup_hbm.at[:, D:2 * D], wup.at[1]),
        ("v", wv_hbm, wa.at[0]), ("dn", wdn_hbm, wa.at[1]),
        ("ao", wao_hbm, wb.at[0]), ("m0", wm_hbm.at[0:D], wb.at[1]), ("m1", wm_hbm.at[D:2 * D], wb.at[2])])}
    late = [wc[n] for n in ("v", "ao", "m0", "dn", "m1", "u", "dw")]
    cuts = [0] + list(range(H, nb * H, 2 * H)) + [TQ]
    xc = [pltpu.make_async_copy(x_hbm.at[0, :, pl.ds(a, e - a), :], x_v.at[0, :, pl.ds(a, e - a), :], xsem.at[n])
          for n, (a, e) in enumerate(zip(cuts[:-1], cuts[1:]))]
    late.append(pltpu.make_async_copy(x_hbm.at[pl.ds(1, B - 1)], x_v.at[pl.ds(1, B - 1), :, pl.ds(0, TQ), :],
                                      xsem.at[len(xc)]))

    def set_projection(n, w):
        for k, v in enumerate(beta(quadrants(w))):
            wp_s[n, k] = pack(v)

    def project(n, lhs, order=range(7)):
        res = [None] * 7
        for j, k in enumerate(order):
            res[k] = _dot(unpack(lhs(j, k)), unpack(wp_s[n, k]))
        return gamma(res)

    def normalize(b, r, n):
        rr = pl.ds(r if isinstance(r, int) else pl.multiple_of(r, 16), n)
        for h in range(4):
            xa_s[b, h, rr, :] = _ln(x_v[b, h, rr, :].astype(f32), EPS).astype(bf16)

    for c in (wc["q"], wc["k"], xc[0]):
        c.start()
    for b in range(B):
        for h in range(4):
            x_v[b, h, TQ:, :] = jnp.zeros((nb * H - TQ, D), x_v.dtype)
    for k in range(x_s.shape[0]):
        x_s[k, nb * H2:, :] = jnp.zeros((x_s.shape[1] - nb * H2, D // 2), i32)
    for c in range(NL):
        for h in range(4):
            g_s[nb, h, c, HALO + H:, :] = jnp.zeros((HALO, 128), f32)
        dw_s[c] = jnp.zeros(dw_s.shape[1:], f32)
    for c in (wc["q"], wc["k"]):
        c.wait()
    xc[1].start()
    set_projection(0, _dot(wq[...], wk[...], NT) * (LOG2E * D ** -0.5))
    xc[2].start()

    @pl.loop(0, nb)
    def _(i):
        for k in range(len(xc)):
            @pl.when(i * H == cuts[k])
            def _():
                xc[k].wait()
                for c in ((), (xc[3],), (wc["g"],), ())[k]:
                    c.start()
        normalize(0, i * H, H)

    wc["g"].wait()
    for c in late:
        c.start()
    set_projection(2, wup[1].astype(f32))

    def prepare(b, i):
        dst = pl.ds(pl.multiple_of(i * H2, 8), H2)
        rr = pl.ds(pl.multiple_of(i * H, 16), H)
        never = i < 0
        zero = pl.multiple_of(jnp.minimum(i, 0), 8)

        def tile(h, c):
            v = xa_s[b, h, rr, (c // 2) * 256:(c // 2 + 1) * 256].astype(f32)
            return v[:, (c % 2) * 128:(c % 2 + 1) * 128]

        x1, xq, left = [], [], []
        for a in range(7):
            z = [[alpha_entry(a, lambda r1, c1: tile(2 * r1 + r2, 2 * c1 + c2)) for c2 in range(2)] for r2 in range(2)]
            x1.append([pack(cols(*z[r2])) for r2 in range(2)])
            for r2 in range(2):
                x_s[2 * a + r2, dst, :] = x1[a][r2]
            l2 = left + [v for k, v in enumerate(alpha(z)) if k not in (2, 3)]
            if a == 6:
                l2.append(l2[-1])
            left = [l2.pop()] if len(l2) % 2 else []
            for k in range(len(l2) // 2):
                x_s[14 + 5 * a // 2 + k, dst, :] = pack(cols(l2[2 * k], l2[2 * k + 1]))
            xq.append(x_s[0, pl.ds(zero, 8), :128])
        xq = window(xq, *plan["XW"], 14)
        gpre = split(project(2, lambda j, k: tie(never, rows(*x1[k]), xq[j])))
        gq, GR = [], plan["GR"]
        for p in range(0, H, GR):
            for h in range(4):
                gate = _ln(_gelu2(cols(*[t[p:p + GR] for t in gpre[h]])), 4 * EPS)
                for c in range(NL):
                    t = gate[:, c * 128:(c + 1) * 128]
                    g_s[i + 1, h, c, HALO + p:HALO + p + GR, :] = t
                    if p < HALO:
                        g_s[i, h, c, HALO + H + p:HALO + H + min(p + GR, HALO), :] = t[:HALO - p]
                    if p + GR > H - HALO:
                        o = max(H - HALO - p, 0)
                        g_s[i + 2, h, c, p + o - (H - HALO):p + GR - (H - HALO), :] = t[o:]
            gq.append(pltpu.bitcast(g_s[i + 1, 0, 0, pl.ds(zero + HALO, 8), :], i32))
        gq = window(gq, *plan["GW"], 7)
        q = project(0, lambda j, k: tie(never, rows(*x1[k]), gq[j] + xq[7 + k]), plan["QO"])
        qn = beta2(transpose(split(q)))
        for k in range(25):
            qc_s[i, k] = cols(qn[2 * k], qn[min(2 * k + 1, 48)]).astype(bf16)

    def connect_quarters():
        zero = jnp.zeros((HALO, 128), f32)
        for c in range(NL):
            for h in range(4):
                g_s[nb, h, c, HALO + HL:2 * HALO + HL, :] = g_s[1, h + 1, c, HALO:2 * HALO, :] if h < 3 else zero
                g_s[1, h, c, 0:HALO, :] = g_s[nb, h - 1, c, HL:HL + HALO, :] if h else zero

    def merge_weights(b0):
        for c in late:
            c.wait()
        zero = pl.multiple_of(jnp.minimum(b0, 0), 16)
        tq = []
        for b in range(1, B):
            for p in range(0, nb * H, plan["MR"]):
                normalize(b, p, plan["MR"])
                tq.append(pltpu.bitcast(xa_s[b, 0, pl.ds(zero, 16), :128], i32))
        tq = [list(t) for t in window(tq, *plan["MW"], 12)]
        set_projection(1, wup[0].astype(f32))
        for c in range(NL):
            dw_s[c, 0:K, :] = dwv[:, c * 128:(c + 1) * 128].astype(f32) * 0.5
        tq[10].append(wp_s[1, 0, pl.ds(zero, 8), :128])

        def product(n, a, w):
            return cols(*[_dot(unpack(tie(b0 < 0, a, tq[4 * n + c])), wb[w, :, c * 128:(c + 1) * 128])
                          for c in range(4)])

        t = product(0, pltpu.bitcast(wa[0], i32), 0)
        for k, v in enumerate(beta(quadrants(product(1, pltpu.bitcast(wa[1], i32), 2)))):
            wf_s[k, D // 4:, :] = pack(v)
        tq[11].append(wf_s[0, pl.ds(zero + D // 4, 8), :128])
        for k, v in enumerate(beta(quadrants(product(2, pack(t), 1)))):
            wf_s[k, :D // 4, :] = pack(v)

    def out_copy(slot, b, r, n):
        return pltpu.make_async_copy(ob_s.at[slot, :, pl.ds(0, n), :], o_hbm.at[b, :, pl.ds(r, n), :], osem.at[slot])

    def step(b, i):
        r = pl.multiple_of(i * H, 16)
        never = i < 0
        it = b * nb + i
        slot = it % 2
        short = (i == 1) & (b > 0)
        pl.when(short)(lambda: out_copy(slot, 0, 0, HL).wait())
        pl.when((it > 1) & jnp.logical_not(short))(lambda: out_copy(slot, 0, 0, H).wait())

        CR = plan["CR"]
        todo = [(h, c, p) for h in range(4) for c in range(NL) for p in range(0, H, CR)]
        conv = {}

        def conv_pieces(n):
            out = []
            for h, c, p in take(todo, n):
                w = dw_s[c]
                acc = None
                for t in sorted(range(K), key=lambda t: (t % 8, t)):
                    term = g_s[i + 1, h, c, pl.ds(p + HALO - K // 2 + t, CR), :] * w[t:t + 1, :]
                    acc = term if acc is None else acc + term
                conv[h, c, p] = acc
                out.append([acc[k:k + 8] for k in range(0, CR, 8)])
            return out

        def keys(a, c, lo, hi):
            t = 4 * a if c == 2 else 4 * a + 3 if c == 3 else 28 + 5 * a + (c if c < 2 else c - 2)
            return unpack(x_s[t // 2, lo * 64:hi * 64, (t % 2) * 128:(t % 2 + 1) * 128])

        def win(queue, w):
            return window(queue, 7 * w[0], 7 * w[1], 49)

        qc = [pltpu.bitcast(qc_s[i, k // 2], i32)[:, (k % 2) * 128:(k % 2 + 1) * 128] for k in range(49)]
        s = [[[None] * NT_ for _ in range(4)] for _ in range(4)]
        m, l, statq = [None] * 4, [None] * 4, []
        for t in range(NT_):
            st = win(statq, plan["QW"])
            cq = win(conv_pieces(plan["QC"] if t == 0 else 0), plan["QCW"])
            res = [None] * 49
            for p, k in enumerate([7 * a + c for a in plan["AO"] for c in plan["IO"]]):
                res[k] = _dot(unpack(tie(never, qc[k], st[p] + sum(cq[p], []))), keys(k // 7, k % 7, t, t + 1), NT)
            z = transpose(gamma2(res))
            for h in range(4):
                new = []
                for c in range(4):
                    v = z[h][c]
                    if (t + 1) * 128 > TQ:
                        v = jnp.where(t * 128 + lax.broadcasted_iota(i32, v.shape, 1) < TQ, v, -jnp.inf)
                    s[h][c][t] = v
                    new.append(v)
                mx = functools.reduce(jnp.maximum, new)
                tot = None
                if m[h] is not None:
                    mx = jnp.maximum(m[h], mx)
                    tot = l[h] * jnp.exp2(m[h] - mx)
                for v in new:
                    e = jnp.exp2(v - mx)
                    tot = e if tot is None else tot + e
                m[h], l[h] = mx, tot
            statq = [l[h][p:p + 8] for p in range(0, H, 8) for h in range(4)]
        shift = []
        for h in range(4):
            mr = jnp.max(m[h], axis=-1, keepdims=True)
            shift.append(mr + jnp.log2(jnp.sum(l[h] * jnp.exp2(m[h] - mr), axis=-1, keepdims=True)))

        edges = [sum(plan["VCH"][:n]) for n in range(len(plan["VCH"]) + 1)]

        def probabilities(n):
            tiles = range(edges[n], edges[n + 1])
            g = [[cols(*[jnp.exp2(s[h][c][t] - shift[h]) for t in tiles]) for c in range(4)] for h in range(4)]
            return alpha2(g), [g[h][c][p:p + 8, t * 128:(t + 1) * 128] for p in range(0, H, 8)
                               for h in range(4) for c in range(4) for t in range(len(tiles))]

        operands, pq = probabilities(0)
        st, pq = window(statq, *plan["SW"], 7), window(pq, *plan["FW"], 7)
        r2 = pl.ds(pl.multiple_of(i * H2, 8), H2)
        upre = split(project(1, lambda j, k: tie(never, rows(x_s[2 * k, r2, :], x_s[2 * k + 1, r2, :]),
                                                 st[j] + pq[j]), plan["UO"]))

        acc, uq, nv = [None] * 49, [], len(plan["VCH"])
        for n in range(nv):
            following, pq = probabilities(n + 1) if n + 1 < nv else (None, [])
            pq = win(pq, plan["PW"][n]) if n + 1 < nv else [[]] * 49
            ug = win(uq if n == plan["UJ"] else [], plan["UW"])
            cg = win(conv_pieces(plan["CJ"][n]), plan["CW"][n])
            outer = plan["PL"] if n == nv - 1 else plan["PA"]
            for p, k in enumerate([7 * a + c for a in outer for c in plan["PI"]]):
                d = _dot(tie(never, operands[k], pq[p] + ug[p] + sum(cg[p], [])).astype(bf16),
                         keys(PERM[k // 7], PERM[k % 7], edges[n], edges[n + 1]))
                acc[k] = d if acc[k] is None else acc[k] + d
                if n == 0 and p == 7 * plan["US"]:
                    started = d
            operands = following
            if n == 0:
                u = [[_gelu2(jnp.where(never, started, v)) for v in row] for row in upre]
                uq = [v[p:p + 8] for row in u for v in row for p in range(0, H, 8)]

        cf = window(conv_pieces(len(todo)), *plan["FS"], 7)
        uc = [[u[h][c] * rows(*[conv[h, c, p] for p in range(0, H, CR)]) for c in range(4)] for h in range(4)]
        ao, ac = alpha(merge(gamma2(acc))), alpha(merge(uc))
        res = [None] * 7
        for n, k in enumerate(plan["FO"]):
            res[k] = _dot(tie(never, ao[k], sum(cf[n], [])).astype(bf16), unpack(wf_s[k, :D // 4, :]))
        for k in plan["FO"]:
            res[k] = res[k] + _dot(ac[k].astype(bf16), unpack(wf_s[k, D // 4:, :]))
        out = split(gamma(res))
        for h in range(4):
            ob_s[slot, h] = (x_v[b, h, pl.ds(r, H), :].astype(f32) + cols(*out[h])).astype(ob_s.dtype)
        pl.when(i < nb - 1)(lambda: out_copy(slot, b, r, H).start())
        pl.when(i == nb - 1)(lambda: out_copy(slot, b, r, HL).start())

    @pl.loop(0, B)
    def _(b):
        pl.loop(0, nb)(functools.partial(prepare, b))
        connect_quarters()
        pl.when(b == 0)(lambda: merge_weights(b))
        pl.loop(0, nb)(functools.partial(step, b))

    out_copy((B * nb) % 2, 0, 0, H).wait()
    out_copy((B * nb + 1) % 2, 0, 0, HL).wait()


def _call(x, w_q, w_k, w_v, w_ao, w_up, dw, w_dn, w_merge, plan):
    B, T, D = x.shape
    TQ = T // 4
    nb = -(-TQ // H)
    hbm = pl.BlockSpec(memory_space=pl.ANY)
    out = pl.pallas_call(
        functools.partial(_kernel, plan=plan),
        in_specs=[hbm] * 9,
        out_specs=hbm,
        out_shape=jax.ShapeDtypeStruct((B, 4, TQ, D), x.dtype),
        scratch_shapes=[
            pltpu.VMEM((B, 4, nb * H, D), x.dtype),
            pltpu.VMEM(w_q.shape, w_q.dtype),
            pltpu.VMEM(w_k.shape, w_k.dtype),
            pltpu.VMEM((2, D, D), w_up.dtype),
            pltpu.VMEM(dw.shape, dw.dtype),
            pltpu.VMEM((2, D, D), bf16),
            pltpu.VMEM((3, D, D), bf16),
            pltpu.VMEM((3, 7, D // 4, D // 2), i32),
            pltpu.VMEM((7, D // 2, D // 2), i32),
            pltpu.VMEM((B, 4, nb * H, D), bf16),
            pltpu.VMEM((32, 64 * sum(plan["VCH"]), D // 2), i32),
            pltpu.VMEM((nb, 32, H, D // 2), bf16),
            pltpu.VMEM((nb + 2, 4, D // 128, H + 2 * HALO, 128), f32),
            pltpu.VMEM((D // 128, 2 * HALO, 128), f32),
            pltpu.VMEM((2, 4, H, D), x.dtype),
            pltpu.SemaphoreType.DMA((10,)),
            pltpu.SemaphoreType.DMA((-(-nb // 2) + 1,)),
            pltpu.SemaphoreType.DMA((2,)),
        ],
        compiler_params=pltpu.CompilerParams(vmem_limit_bytes=112 * 1024 * 1024),
    )(x.reshape(B, 4, TQ, D), w_q, w_k, w_v, w_ao, w_up, dw, w_dn, w_merge)
    return out.reshape(B, T, D)


@jax.jit
def pallas_standalone__conformer_family_branchformer__speech_kernel(
    x: jax.Array,
    w_q: jax.Array,
    w_k: jax.Array,
    w_v: jax.Array,
    w_ao: jax.Array,
    w_up: jax.Array,
    dw: jax.Array,
    w_dn: jax.Array,
    w_merge: jax.Array,
):
    return _call(x, w_q, w_k, w_v, w_ao, w_up, dw, w_dn, w_merge, PLAN)
```

```python
import functools

import jax
import jax.numpy as jnp
import numpy as np
from jax import lax
import jax.experimental.pallas as pl
import jax.experimental.pallas.tpu as pltpu

bf16, f32, i32 = jnp.bfloat16, jnp.float32, jnp.int32
LOG2E = 1.4426950408889634
EPS = 1e-5
NN = (((1,), (0,)), ((), ()))
NT = (((1,), (1,)), ((), ()))

H = 144
HALO = 16
PERM = (0, 2, 6, 5, 3, 4, 1)
ALPHA_TERMS = (((0, 0, 1), (1, 1, 1)), ((1, 0, 1), (1, 1, 1)), ((0, 0, 1),), ((1, 1, 1),),
               ((0, 0, 1), (0, 1, 1)), ((1, 0, 1), (0, 0, -1)), ((0, 1, 1), (1, 1, -1)))

PLAN = dict(
    MR=48, MW=(1, 11),
    XW=(2, 14), GR=24, GW=(2, 5), QO=(0, 1, 2, 5, 4, 3, 6),
    AO=(0, 2, 1, 5, 4, 3, 6), IO=(0, 1, 3, 2, 5, 4, 6), QW=(1, 7), CR=48, QC=6, QCW=(0, 3),
    UO=(1, 3, 2, 4, 0, 5, 6), SW=(0, 2), FW=(5, 7),
    VCH=(2, 2, 4), PA=(0, 1, 2, 3, 4, 5, 6), PL=(4, 5, 2, 3, 0, 1, 6), PI=(2, 3, 0, 1, 4, 5, 6),
    PW=((4, 7), (4, 7)), CJ=(4, 8, 14), CW=((2, 4), (2, 4), (2, 4)), US=4, UJ=2, UW=(0, 2),
    FO=(3, 1, 6, 2, 0, 4, 5), FS=(0, 7),
)


def _ln(x, eps):
    d = x - jnp.mean(x, axis=-1, keepdims=True)
    v = jnp.mean(d * d, axis=-1, keepdims=True)
    return d * jnp.exp2(jnp.log(v + eps) * (-0.5 * LOG2E))


def _gelu2(x):
    c = float(np.sqrt(2.0 / np.pi))
    return x * jnp.tanh((x * x * (0.044715 * c) + c) * x) + x


def _dot(a, b, dims=NN):
    return lax.dot_general(a, b, dims, preferred_element_type=f32)


def rows(*parts):
    return lax.concatenate(parts, 0)


def cols(*parts):
    return lax.concatenate(parts, 1)


def pack(v):
    return pltpu.bitcast(v.astype(bf16), i32)


def unpack(v):
    return pltpu.bitcast(v, bf16)


def alpha(z):
    (a, b), (c, d) = z
    return [a + d, c + d, a, d, a + b, c - a, b - d]


def alpha_entry(k, z):
    (r0, c0, _), *rest = ALPHA_TERMS[k]
    v = z(r0, c0)
    for r, c, sign in rest:
        v = v + z(r, c) if sign > 0 else v - z(r, c)
    return v


def beta(z):
    t = alpha(z)
    return [t[k] for k in PERM]


def gamma(n):
    return [[n[0] + n[3] - n[4] + n[6], n[2] + n[4]], [n[1] + n[3], n[0] - n[1] + n[2] + n[5]]]


def alpha2(g):
    def pair(u, v):
        (x, sx), (y, sy) = u, v
        if sx > 0:
            return (x + y if sy > 0 else x - y), 1
        return (y - x, 1) if sy > 0 else (x + y, -1)

    out = []
    for a in range(7):
        for k in range(7):
            t = [[(g[2 * r1 + r2][2 * c1 + c2], s1 * s2) for r2, c2, s2 in ALPHA_TERMS[k]]
                 for r1, c1, s1 in ALPHA_TERMS[a]]
            if len(t) == 2 and len(t[0]) == 2:
                v, sign = pair(pair(t[0][0], t[1][1]), pair(t[0][1], t[1][0]))
            else:
                flat = [e for row in t for e in row]
                v, sign = pair(*flat) if len(flat) == 2 else flat[0]
            assert sign > 0
            out.append(v)
    return out


def beta2(g):
    t = [[beta([[g[2 * r1 + r2][2 * c1 + c2] for c1 in range(2)] for r1 in range(2)])
          for c2 in range(2)] for r2 in range(2)]
    return [v for a in range(7) for v in beta([[t[r2][c2][a] for c2 in range(2)] for r2 in range(2)])]


def gamma2(n):
    inner = [gamma(n[7 * a:7 * a + 7]) for a in range(7)]
    out = [[None] * 4 for _ in range(4)]
    for r2 in range(2):
        for c2 in range(2):
            z = gamma([inner[a][r2][c2] for a in range(7)])
            for r1 in range(2):
                for c1 in range(2):
                    out[2 * r1 + r2][2 * c1 + c2] = z[r1][c1]
    return out


def transpose(z):
    return [list(r) for r in zip(*z)]


def quadrants(w):
    n, m = w.shape[0] // 2, w.shape[1] // 2
    return [[w[i * n:(i + 1) * n, j * m:(j + 1) * m] for j in range(2)] for i in range(2)]


def merge(g):
    return [[rows(*[cols(g[2 * r1 + r2][2 * c1], g[2 * r1 + r2][2 * c1 + 1]) for r2 in range(2)])
             for c1 in range(2)] for r1 in range(2)]


def split(z):
    q = [[quadrants(v) for v in row] for row in z]
    return [[q[r // 2][c // 2][r % 2][c % 2] for c in range(4)] for r in range(4)]


def tie(never, a, tokens):
    if not tokens:
        return a
    nr, nc = a.shape[0] // 8, a.shape[1] // 128
    cells = {}
    for j, t in enumerate(tokens):
        p = j * nr * nc // len(tokens)
        cells[p] = jnp.maximum(cells[p], t) if p in cells else t
    out, done = [], 0
    for p in sorted({cell // nc for cell in cells}):
        if done < p:
            out.append(a[8 * done:8 * p])
        row = []
        for c in range(nc):
            v = a[8 * p:8 * p + 8, 128 * c:128 * c + 128]
            t = cells.get(p * nc + c)
            if t is not None:
                v = lax.select(never, t if t.dtype == a.dtype else pltpu.bitcast(t, a.dtype), v)
            row.append(v)
        out.append(cols(*row))
        done = p + 1
    if done < nr:
        out.append(a[8 * done:])
    return rows(*out)


def take(queue, n):
    out = queue[:n]
    del queue[:n]
    return out


def window(queue, lo, hi, n):
    m = hi - lo
    return [[]] * lo + [queue[k * len(queue) // m:(k + 1) * len(queue) // m] for k in range(m)] + [[]] * (n - hi)


def _kernel(x_hbm, wq_hbm, wk_hbm, wv_hbm, wao_hbm, wup_hbm, dw_hbm, wdn_hbm, wm_hbm, o_hbm,
            x_v, wq, wk, wup, dwv, wa, wb,
            wp_s,
            wf_s,
            xa_s,
            x_s,
            qc_s,
            g_s,
            dw_s, ob_s, wsem, xsem, osem, *, plan):
    B, _, TQ, D = x_hbm.shape
    K = dw_hbm.shape[0]
    NL = D // 128
    nb = -(-TQ // H)
    HL = TQ - (nb - 1) * H
    H2 = H // 2
    NT_ = sum(plan["VCH"])
    assert NL == 4 and K // 2 <= HALO <= HL and nb * H <= 128 * NT_

    wc = {n: pltpu.make_async_copy(s, d, wsem.at[k]) for k, (n, s, d) in enumerate([
        ("q", wq_hbm, wq), ("k", wk_hbm, wk), ("dw", dw_hbm, dwv),
        ("u", wup_hbm.at[:, 0:D], wup.at[0]), ("g", wup_hbm.at[:, D:2 * D], wup.at[1]),
        ("v", wv_hbm, wa.at[0]), ("dn", wdn_hbm, wa.at[1]),
        ("ao", wao_hbm, wb.at[0]), ("m0", wm_hbm.at[0:D], wb.at[1]), ("m1", wm_hbm.at[D:2 * D], wb.at[2])])}
    late = [wc[n] for n in ("v", "ao", "m0", "dn", "m1", "u", "dw")]
    cuts = [0] + list(range(H, nb * H, 2 * H)) + [TQ]
    xc = [pltpu.make_async_copy(x_hbm.at[0, :, pl.ds(a, e - a), :], x_v.at[0, :, pl.ds(a, e - a), :], xsem.at[n])
          for n, (a, e) in enumerate(zip(cuts[:-1], cuts[1:]))]
    late.append(pltpu.make_async_copy(x_hbm.at[pl.ds(1, B - 1)], x_v.at[pl.ds(1, B - 1), :, pl.ds(0, TQ), :],
                                      xsem.at[len(xc)]))

    def set_projection(n, w):
        for k, v in enumerate(beta(quadrants(w))):
            wp_s[n, k] = pack(v)

    def project(n, lhs, order=range(7)):
        res = [None] * 7
        for j, k in enumerate(order):
            res[k] = _dot(lhs(j, k), unpack(wp_s[n, k]))
        return gamma(res)

    def normalize(b, r, n):
        rr = pl.ds(r if isinstance(r, int) else pl.multiple_of(r, 16), n)
        for h in range(4):
            xa_s[b, h, rr, :] = _ln(x_v[b, h, rr, :].astype(f32), EPS).astype(bf16)

    for c in (wc["q"], wc["k"], xc[0]):
        c.start()
    for b in range(B):
        for h in range(4):
            x_v[b, h, TQ:, :] = jnp.zeros((nb * H - TQ, D), x_v.dtype)
    for k in range(x_s.shape[0]):
        x_s[k, nb * H2:, :] = jnp.zeros((x_s.shape[1] - nb * H2, D // 2), i32)
    for c in range(NL):
        for h in range(4):
            g_s[nb, h, c, HALO + H:, :] = jnp.zeros((HALO, 128), f32)
        dw_s[c] = jnp.zeros(dw_s.shape[1:], f32)
    for c in (wc["q"], wc["k"]):
        c.wait()
    xc[1].start()
    set_projection(0, _dot(wq[...], wk[...], NT) * (LOG2E * D ** -0.5))
    xc[2].start()

    @pl.loop(0, nb)
    def _(i):
        for k in range(len(xc)):
            @pl.when(i * H == cuts[k])
            def _():
                xc[k].wait()
                for c in ((), (xc[3],), (wc["g"],), ())[k]:
                    c.start()
        normalize(0, i * H, H)

    wc["g"].wait()
    for c in late:
        c.start()
    set_projection(2, wup[1].astype(f32))

    def prepare(b, i):
        dst = pl.ds(pl.multiple_of(i * H2, 8), H2)
        rr = pl.ds(pl.multiple_of(i * H, 16), H)
        never = i < 0
        zero = pl.multiple_of(jnp.minimum(i, 0), 8)

        def tile(h, c):
            v = xa_s[b, h, rr, (c // 2) * 256:(c // 2 + 1) * 256].astype(f32)
            return v[:, (c % 2) * 128:(c % 2 + 1) * 128]

        x1, xq, left = [], [], []
        for a in range(7):
            z = [[alpha_entry(a, lambda r1, c1: tile(2 * r1 + r2, 2 * c1 + c2)) for c2 in range(2)] for r2 in range(2)]
            x1.append(rows(cols(*z[0]), cols(*z[1])))
            for r2 in range(2):
                x_s[2 * a + r2, dst, :] = pack(cols(*z[r2]))
            l2 = left + [v for k, v in enumerate(alpha(z)) if k not in (2, 3)]
            if a == 6:
                l2.append(l2[-1])
            left = [l2.pop()] if len(l2) % 2 else []
            for k in range(len(l2) // 2):
                x_s[14 + 5 * a // 2 + k, dst, :] = pack(cols(l2[2 * k], l2[2 * k + 1]))
            xq.append(x_s[0, pl.ds(zero, 8), :128])
        xq = window(xq, *plan["XW"], 14)
        gpre = split(project(2, lambda j, k: tie(never, x1[k], xq[j]).astype(bf16)))
        gq, GR = [], plan["GR"]
        for p in range(0, H, GR):
            for h in range(4):
                gate = _ln(_gelu2(cols(*[t[p:p + GR] for t in gpre[h]])), 4 * EPS)
                for c in range(NL):
                    t = gate[:, c * 128:(c + 1) * 128]
                    g_s[i + 1, h, c, HALO + p:HALO + p + GR, :] = t
                    if p < HALO:
                        g_s[i, h, c, HALO + H + p:HALO + H + min(p + GR, HALO), :] = t[:HALO - p]
                    if p + GR > H - HALO:
                        o = max(H - HALO - p, 0)
                        g_s[i + 2, h, c, p + o - (H - HALO):p + GR - (H - HALO), :] = t[o:]
            gq.append(g_s[i + 1, 0, 0, pl.ds(zero + HALO, 8), :])
        gq = window(gq, *plan["GW"], 7)
        q = project(0, lambda j, k: unpack(tie(never, rows(x_s[2 * k, dst, :], x_s[2 * k + 1, dst, :]),
                                               gq[j] + xq[7 + k])), plan["QO"])
        qn = beta2(transpose(split(q)))
        for k in range(25):
            qc_s[i, k] = cols(qn[2 * k], qn[min(2 * k + 1, 48)]).astype(bf16)

    def connect_quarters():
        zero = jnp.zeros((HALO, 128), f32)
        for c in range(NL):
            for h in range(4):
                g_s[nb, h, c, HALO + HL:2 * HALO + HL, :] = g_s[1, h + 1, c, HALO:2 * HALO, :] if h < 3 else zero
                g_s[1, h, c, 0:HALO, :] = g_s[nb, h - 1, c, HL:HL + HALO, :] if h else zero

    def merge_weights(b0):
        for c in late:
            c.wait()
        zero = pl.multiple_of(jnp.minimum(b0, 0), 16)
        tq = []
        for b in range(1, B):
            for p in range(0, nb * H, plan["MR"]):
                normalize(b, p, plan["MR"])
                tq.append(pltpu.bitcast(xa_s[b, 0, pl.ds(zero, 16), :128], i32))
        tq = [list(t) for t in window(tq, *plan["MW"], 12)]
        set_projection(1, wup[0].astype(f32))
        for c in range(NL):
            dw_s[c, 0:K, :] = dwv[:, c * 128:(c + 1) * 128].astype(f32) * 0.5
        tq[10].append(wp_s[1, 0, pl.ds(zero, 8), :128])

        def product(n, a, w):
            return cols(*[_dot(unpack(tie(b0 < 0, a, tq[4 * n + c])), wb[w, :, c * 128:(c + 1) * 128])
                          for c in range(4)])

        t = product(0, pltpu.bitcast(wa[0], i32), 0)
        for k, v in enumerate(beta(quadrants(product(1, pltpu.bitcast(wa[1], i32), 2)))):
            wf_s[k, D // 4:, :] = pack(v)
        tq[11].append(wf_s[0, pl.ds(zero + D // 4, 8), :128])
        for k, v in enumerate(beta(quadrants(product(2, pack(t), 1)))):
            wf_s[k, :D // 4, :] = pack(v)

    def out_copy(slot, b, r, n):
        return pltpu.make_async_copy(ob_s.at[slot, :, pl.ds(0, n), :], o_hbm.at[b, :, pl.ds(r, n), :], osem.at[slot])

    def step(b, i):
        r = pl.multiple_of(i * H, 16)
        never = i < 0
        it = b * nb + i
        slot = it % 2
        short = (i == 1) & (b > 0)
        pl.when(short)(lambda: out_copy(slot, 0, 0, HL).wait())
        pl.when((it > 1) & jnp.logical_not(short))(lambda: out_copy(slot, 0, 0, H).wait())

        CR = plan["CR"]
        todo = [(h, c, p) for h in range(4) for c in range(NL) for p in range(0, H, CR)]
        conv = {}

        def conv_pieces(n):
            out = []
            for h, c, p in take(todo, n):
                w = dw_s[c]
                acc = None
                for t in sorted(range(K), key=lambda t: (t % 8, t)):
                    term = g_s[i + 1, h, c, pl.ds(p + HALO - K // 2 + t, CR), :] * w[t:t + 1, :]
                    acc = term if acc is None else acc + term
                conv[h, c, p] = acc
                out.append([acc[k:k + 8] for k in range(0, CR, 8)])
            return out

        def keys(a, c, lo, hi):
            t = 4 * a if c == 2 else 4 * a + 3 if c == 3 else 28 + 5 * a + (c if c < 2 else c - 2)
            return unpack(x_s[t // 2, lo * 64:hi * 64, (t % 2) * 128:(t % 2 + 1) * 128])

        def win(queue, w):
            return window(queue, 7 * w[0], 7 * w[1], 49)

        qc = [pltpu.bitcast(qc_s[i, k // 2], i32)[:, (k % 2) * 128:(k % 2 + 1) * 128] for k in range(49)]
        s = [[[None] * NT_ for _ in range(4)] for _ in range(4)]
        m, l, statq = [None] * 4, [None] * 4, []
        for t in range(NT_):
            st = win(statq, plan["QW"])
            cq = win(conv_pieces(plan["QC"] if t == 0 else 0), plan["QCW"])
            res = [None] * 49
            for p, k in enumerate([7 * a + c for a in plan["AO"] for c in plan["IO"]]):
                res[k] = _dot(unpack(tie(never, qc[k], st[p] + sum(cq[p], []))), keys(k // 7, k % 7, t, t + 1), NT)
            z = transpose(gamma2(res))
            for h in range(4):
                new = []
                for c in range(4):
                    v = z[h][c]
                    if (t + 1) * 128 > TQ:
                        v = jnp.where(t * 128 + lax.broadcasted_iota(i32, v.shape, 1) < TQ, v, -jnp.inf)
                    s[h][c][t] = v
                    new.append(v)
                mx = functools.reduce(jnp.maximum, new)
                tot = None
                if m[h] is not None:
                    mx = jnp.maximum(m[h], mx)
                    tot = l[h] * jnp.exp2(m[h] - mx)
                for v in new:
                    e = jnp.exp2(v - mx)
                    tot = e if tot is None else tot + e
                m[h], l[h] = mx, tot
            statq = [l[h][p:p + 8] for p in range(0, H, 8) for h in range(4)]
        shift = []
        for h in range(4):
            mr = jnp.max(m[h], axis=-1, keepdims=True)
            shift.append(mr + jnp.log2(jnp.sum(l[h] * jnp.exp2(m[h] - mr), axis=-1, keepdims=True)))

        edges = [sum(plan["VCH"][:n]) for n in range(len(plan["VCH"]) + 1)]

        def probabilities(n):
            tiles = range(edges[n], edges[n + 1])
            g = [[cols(*[jnp.exp2(s[h][c][t] - shift[h]) for t in tiles]) for c in range(4)] for h in range(4)]
            return alpha2(g), [g[h][c][p:p + 8, t * 128:(t + 1) * 128] for p in range(0, H, 8)
                               for h in range(4) for c in range(4) for t in range(len(tiles))]

        operands, pq = probabilities(0)
        st, pq = window(statq, *plan["SW"], 7), window(pq, *plan["FW"], 7)
        r2 = pl.ds(pl.multiple_of(i * H2, 8), H2)
        upre = split(project(1, lambda j, k: unpack(tie(never, rows(x_s[2 * k, r2, :], x_s[2 * k + 1, r2, :]),
                                                        st[j] + pq[j])), plan["UO"]))

        acc, uq, nv = [None] * 49, [], len(plan["VCH"])
        for n in range(nv):
            following, pq = probabilities(n + 1) if n + 1 < nv else (None, [])
            pq = win(pq, plan["PW"][n]) if n + 1 < nv else [[]] * 49
            ug = win(uq if n == plan["UJ"] else [], plan["UW"])
            cg = win(conv_pieces(plan["CJ"][n]), plan["CW"][n])
            outer = plan["PL"] if n == nv - 1 else plan["PA"]
            for p, k in enumerate([7 * a + c for a in outer for c in plan["PI"]]):
                d = _dot(tie(never, operands[k], pq[p] + ug[p] + sum(cg[p], [])).astype(bf16),
                         keys(PERM[k // 7], PERM[k % 7], edges[n], edges[n + 1]))
                acc[k] = d if acc[k] is None else acc[k] + d
                if n == 0 and p == 7 * plan["US"]:
                    started = d
            operands = following
            if n == 0:
                u = [[_gelu2(lax.select(never, started, v)) for v in row] for row in upre]
                uq = [v[p:p + 8] for row in u for v in row for p in range(0, H, 8)]

        cf = window(conv_pieces(len(todo)), *plan["FS"], 7)
        uc = [[u[h][c] * rows(*[conv[h, c, p] for p in range(0, H, CR)]) for c in range(4)] for h in range(4)]
        ao, ac = alpha(merge(gamma2(acc))), alpha(merge(uc))
        res = [None] * 7
        for n, k in enumerate(plan["FO"]):
            res[k] = _dot(tie(never, ao[k], sum(cf[n], [])).astype(bf16), unpack(wf_s[k, :D // 4, :]))
        for k in plan["FO"]:
            res[k] = res[k] + _dot(ac[k].astype(bf16), unpack(wf_s[k, D // 4:, :]))
        out = split(gamma(res))
        for h in range(4):
            ob_s[slot, h] = (x_v[b, h, pl.ds(r, H), :].astype(f32) + cols(*out[h])).astype(ob_s.dtype)
        pl.when(i < nb - 1)(lambda: out_copy(slot, b, r, H).start())
        pl.when(i == nb - 1)(lambda: out_copy(slot, b, r, HL).start())

    @pl.loop(0, B)
    def _(b):
        pl.loop(0, nb)(functools.partial(prepare, b))
        connect_quarters()
        pl.when(b == 0)(lambda: merge_weights(b))
        pl.loop(0, nb)(functools.partial(step, b))

    out_copy((B * nb) % 2, 0, 0, H).wait()
    out_copy((B * nb + 1) % 2, 0, 0, HL).wait()


def _call(x, w_q, w_k, w_v, w_ao, w_up, dw, w_dn, w_merge, plan):
    B, T, D = x.shape
    TQ = T // 4
    nb = -(-TQ // H)
    hbm = pl.BlockSpec(memory_space=pl.ANY)
    out = pl.pallas_call(
        functools.partial(_kernel, plan=plan),
        in_specs=[hbm] * 9,
        out_specs=hbm,
        out_shape=jax.ShapeDtypeStruct((B, 4, TQ, D), x.dtype),
        scratch_shapes=[
            pltpu.VMEM((B, 4, nb * H, D), x.dtype),
            pltpu.VMEM(w_q.shape, w_q.dtype),
            pltpu.VMEM(w_k.shape, w_k.dtype),
            pltpu.VMEM((2, D, D), w_up.dtype),
            pltpu.VMEM(dw.shape, dw.dtype),
            pltpu.VMEM((2, D, D), bf16),
            pltpu.VMEM((3, D, D), bf16),
            pltpu.VMEM((3, 7, D // 4, D // 2), i32),
            pltpu.VMEM((7, D // 2, D // 2), i32),
            pltpu.VMEM((B, 4, nb * H, D), bf16),
            pltpu.VMEM((32, 64 * sum(plan["VCH"]), D // 2), i32),
            pltpu.VMEM((nb, 32, H, D // 2), bf16),
            pltpu.VMEM((nb + 2, 4, D // 128, H + 2 * HALO, 128), f32),
            pltpu.VMEM((D // 128, 2 * HALO, 128), f32),
            pltpu.VMEM((2, 4, H, D), x.dtype),
            pltpu.SemaphoreType.DMA((10,)),
            pltpu.SemaphoreType.DMA((-(-nb // 2) + 1,)),
            pltpu.SemaphoreType.DMA((2,)),
        ],
        compiler_params=pltpu.CompilerParams(vmem_limit_bytes=112 * 1024 * 1024),
    )(x.reshape(B, 4, TQ, D), w_q, w_k, w_v, w_ao, w_up, dw, w_dn, w_merge)
    return out.reshape(B, T, D)


@jax.jit
def pallas_standalone__conformer_family_branchformer__speech_kernel(
    x: jax.Array,
    w_q: jax.Array,
    w_k: jax.Array,
    w_v: jax.Array,
    w_ao: jax.Array,
    w_up: jax.Array,
    dw: jax.Array,
    w_dn: jax.Array,
    w_merge: jax.Array,
):
    return _call(x, w_q, w_k, w_v, w_ao, w_up, dw, w_dn, w_merge, PLAN)
```

```python
import functools

import jax
import jax.numpy as jnp
import numpy as np
from jax import lax
import jax.experimental.pallas as pl
import jax.experimental.pallas.tpu as pltpu

bf16, f32, i32 = jnp.bfloat16, jnp.float32, jnp.int32
LOG2E = 1.4426950408889634
EPS = 1e-5
NN = (((1,), (0,)), ((), ()))
NT = (((1,), (1,)), ((), ()))

H = 144
HALO = 16
PERM = (0, 2, 6, 5, 3, 4, 1)
ALPHA_TERMS = (((0, 0, 1), (1, 1, 1)), ((1, 0, 1), (1, 1, 1)), ((0, 0, 1),), ((1, 1, 1),),
               ((0, 0, 1), (0, 1, 1)), ((1, 0, 1), (0, 0, -1)), ((0, 1, 1), (1, 1, -1)))

PLAN = dict(
    MR=48, MW=(1, 11),
    XW=(2, 14), GR=24, GW=(2, 5), QO=(0, 1, 2, 5, 4, 3, 6),
    AO=(0, 2, 1, 5, 4, 3, 6), IO=(0, 1, 3, 2, 5, 4, 6), QW=(2, 7), CR=48, QC=6, QCW=(0, 3),
    UO=(1, 3, 2, 4, 0, 5, 6), SW=(0, 2), FW=(5, 7),
    VCH=(2, 2, 4), PA=(0, 1, 2, 3, 4, 5, 6), PL=(0, 5, 2, 3, 4, 1, 6), PI=(2, 3, 0, 1, 4, 5, 6),
    PW=((4, 7), (4, 7)), CJ=(4, 8, 10), CW=((2, 4), (2, 4), (2, 4)), US=6, UJ=2, UW=(0, 2),
    FO=(1, 3, 6, 0, 2, 4, 5), CO=(2, 3, 0, 1, 5, 4, 6), FS=(2, 12),
    BO=((0, 0), (1, 1), (0, 1), (1, 0)),
)


def _ln(x, eps):
    d = x - jnp.mean(x, axis=-1, keepdims=True)
    v = jnp.mean(d * d, axis=-1, keepdims=True)
    return d * jnp.exp2(jnp.log(v + eps) * (-0.5 * LOG2E))


def _gelu2(x):
    c = float(np.sqrt(2.0 / np.pi))
    return x * jnp.tanh((x * x * (0.044715 * c) + c) * x) + x


def _dot(a, b, dims=NN):
    return lax.dot_general(a, b, dims, preferred_element_type=f32)


def rows(*parts):
    return lax.concatenate(parts, 0)


def cols(*parts):
    return lax.concatenate(parts, 1)


def pack(v):
    return pltpu.bitcast(v.astype(bf16), i32)


def unpack(v):
    return pltpu.bitcast(v, bf16)


def alpha(z):
    (a, b), (c, d) = z
    return [a + d, c + d, a, d, a + b, c - a, b - d]


def alpha_entry(k, z):
    (r0, c0, _), *rest = ALPHA_TERMS[k]
    v = z(r0, c0)
    for r, c, sign in rest:
        v = v + z(r, c) if sign > 0 else v - z(r, c)
    return v


def beta(z):
    t = alpha(z)
    return [t[k] for k in PERM]


def gamma(n):
    return [[n[0] + n[3] - n[4] + n[6], n[2] + n[4]], [n[1] + n[3], n[0] - n[1] + n[2] + n[5]]]


def alpha2(g):
    def pair(u, v):
        (x, sx), (y, sy) = u, v
        if sx > 0:
            return (x + y if sy > 0 else x - y), 1
        return (y - x, 1) if sy > 0 else (x + y, -1)

    out = []
    for a in range(7):
        for k in range(7):
            t = [[(g[2 * r1 + r2][2 * c1 + c2], s1 * s2) for r2, c2, s2 in ALPHA_TERMS[k]]
                 for r1, c1, s1 in ALPHA_TERMS[a]]
            if len(t) == 2 and len(t[0]) == 2:
                v, sign = pair(pair(t[0][0], t[1][1]), pair(t[0][1], t[1][0]))
            else:
                flat = [e for row in t for e in row]
                v, sign = pair(*flat) if len(flat) == 2 else flat[0]
            assert sign > 0
            out.append(v)
    return out


def beta2(g):
    t = [[beta([[g[2 * r1 + r2][2 * c1 + c2] for c1 in range(2)] for r1 in range(2)])
          for c2 in range(2)] for r2 in range(2)]
    return [v for a in range(7) for v in beta([[t[r2][c2][a] for c2 in range(2)] for r2 in range(2)])]


def gamma2(n):
    inner = [gamma(n[7 * a:7 * a + 7]) for a in range(7)]
    out = [[None] * 4 for _ in range(4)]
    for r2 in range(2):
        for c2 in range(2):
            z = gamma([inner[a][r2][c2] for a in range(7)])
            for r1 in range(2):
                for c1 in range(2):
                    out[2 * r1 + r2][2 * c1 + c2] = z[r1][c1]
    return out


def transpose(z):
    return [list(r) for r in zip(*z)]


def quadrants(w):
    n, m = w.shape[0] // 2, w.shape[1] // 2
    return [[w[i * n:(i + 1) * n, j * m:(j + 1) * m] for j in range(2)] for i in range(2)]


def merge(g):
    return [[rows(*[cols(g[2 * r1 + r2][2 * c1], g[2 * r1 + r2][2 * c1 + 1]) for r2 in range(2)])
             for c1 in range(2)] for r1 in range(2)]


def split(z):
    q = [[quadrants(v) for v in row] for row in z]
    return [[q[r // 2][c // 2][r % 2][c % 2] for c in range(4)] for r in range(4)]


def tie(never, a, tokens):
    if not tokens:
        return a
    nr, nc = a.shape[0] // 8, a.shape[1] // 128
    cells = {}
    for j, t in enumerate(tokens):
        p = j * nr * nc // len(tokens)
        cells[p] = jnp.maximum(cells[p], t) if p in cells else t
    out, done = [], 0
    for p in sorted({cell // nc for cell in cells}):
        if done < p:
            out.append(a[8 * done:8 * p])
        row = []
        for c in range(nc):
            v = a[8 * p:8 * p + 8, 128 * c:128 * c + 128]
            t = cells.get(p * nc + c)
            if t is not None:
                v = lax.select(never, t if t.dtype == a.dtype else pltpu.bitcast(t, a.dtype), v)
            row.append(v)
        out.append(cols(*row))
        done = p + 1
    if done < nr:
        out.append(a[8 * done:])
    return rows(*out)


def take(queue, n):
    out = queue[:n]
    del queue[:n]
    return out


def window(queue, lo, hi, n):
    m = hi - lo
    return [[]] * lo + [queue[k * len(queue) // m:(k + 1) * len(queue) // m] for k in range(m)] + [[]] * (n - hi)


def _kernel(x_hbm, wq_hbm, wk_hbm, wv_hbm, wao_hbm, wup_hbm, dw_hbm, wdn_hbm, wm_hbm, o_hbm,
            x_v, wq, wk, wup, dwv, wa, wb,
            wp_s,
            wf_s,
            xa_s,
            x_s,
            qc_s,
            g_s,
            dw_s, ob_s, wsem, xsem, osem, *, plan):
    B, _, TQ, D = x_hbm.shape
    K = dw_hbm.shape[0]
    NL = D // 128
    nb = -(-TQ // H)
    HL = TQ - (nb - 1) * H
    H2 = H // 2
    NT_ = sum(plan["VCH"])
    assert NL == 4 and K // 2 <= HALO <= HL and nb * H <= 128 * NT_

    wc = {n: pltpu.make_async_copy(s, d, wsem.at[k]) for k, (n, s, d) in enumerate([
        ("q", wq_hbm, wq), ("k", wk_hbm, wk), ("dw", dw_hbm, dwv),
        ("u", wup_hbm.at[:, 0:D], wup.at[0]), ("g", wup_hbm.at[:, D:2 * D], wup.at[1]),
        ("v", wv_hbm, wa.at[0]), ("dn", wdn_hbm, wa.at[1]),
        ("ao", wao_hbm, wb.at[0]), ("m0", wm_hbm.at[0:D], wb.at[1]), ("m1", wm_hbm.at[D:2 * D], wb.at[2])])}
    late = [wc[n] for n in ("v", "ao", "m0", "dn", "m1", "u", "dw")]
    cuts = [0] + list(range(H, nb * H, 2 * H)) + [TQ]
    xc = [pltpu.make_async_copy(x_hbm.at[0, :, pl.ds(a, e - a), :], x_v.at[0, :, pl.ds(a, e - a), :], xsem.at[n])
          for n, (a, e) in enumerate(zip(cuts[:-1], cuts[1:]))]
    late.append(pltpu.make_async_copy(x_hbm.at[pl.ds(1, B - 1)], x_v.at[pl.ds(1, B - 1), :, pl.ds(0, TQ), :],
                                      xsem.at[len(xc)]))

    def set_projection(n, w):
        for k, v in enumerate(beta(quadrants(w))):
            wp_s[n, k] = pack(v)

    def project(n, lhs, order=range(7)):
        res = [None] * 7
        for j, k in enumerate(order):
            res[k] = _dot(lhs(j, k), unpack(wp_s[n, k]))
        return gamma(res)

    def normalize(b, r, n):
        rr = pl.ds(r if isinstance(r, int) else pl.multiple_of(r, 16), n)
        for h in range(4):
            xa_s[b, h, rr, :] = _ln(x_v[b, h, rr, :].astype(f32), EPS).astype(bf16)

    for c in (wc["q"], wc["k"], xc[0]):
        c.start()
    for b in range(B):
        for h in range(4):
            x_v[b, h, TQ:, :] = jnp.zeros((nb * H - TQ, D), x_v.dtype)
    for k in range(x_s.shape[0]):
        x_s[k, nb * H2:, :] = jnp.zeros((x_s.shape[1] - nb * H2, D // 2), i32)
    for c in range(NL):
        for h in range(4):
            g_s[nb, h, c, HALO + H:, :] = jnp.zeros((HALO, 128), f32)
        dw_s[c] = jnp.zeros(dw_s.shape[1:], f32)
    for c in (wc["q"], wc["k"]):
        c.wait()
    xc[1].start()
    set_projection(0, _dot(wq[...], wk[...], NT) * (LOG2E * D ** -0.5))
    xc[2].start()

    @pl.loop(0, nb)
    def _(i):
        for k in range(len(xc)):
            @pl.when(i * H == cuts[k])
            def _():
                xc[k].wait()
                for c in ((), (xc[3],), (wc["g"],), ())[k]:
                    c.start()
        normalize(0, i * H, H)

    wc["g"].wait()
    for c in late:
        c.start()
    set_projection(2, wup[1].astype(f32))

    def prepare(b, i):
        dst = pl.ds(pl.multiple_of(i * H2, 8), H2)
        rr = pl.ds(pl.multiple_of(i * H, 16), H)
        never = i < 0
        zero = pl.multiple_of(jnp.minimum(i, 0), 8)

        def tile(h, c):
            v = xa_s[b, h, rr, (c // 2) * 256:(c // 2 + 1) * 256].astype(f32)
            return v[:, (c % 2) * 128:(c % 2 + 1) * 128]

        x1, xq, left = [], [], []
        for a in range(7):
            z = [[alpha_entry(a, lambda r1, c1: tile(2 * r1 + r2, 2 * c1 + c2)) for c2 in range(2)] for r2 in range(2)]
            x1.append(rows(cols(*z[0]), cols(*z[1])))
            for r2 in range(2):
                x_s[2 * a + r2, dst, :] = pack(cols(*z[r2]))
            l2 = left + [v for k, v in enumerate(alpha(z)) if k not in (2, 3)]
            if a == 6:
                l2.append(l2[-1])
            left = [l2.pop()] if len(l2) % 2 else []
            for k in range(len(l2) // 2):
                x_s[14 + 5 * a // 2 + k, dst, :] = pack(cols(l2[2 * k], l2[2 * k + 1]))
            xq.append(x_s[0, pl.ds(zero, 8), :128])
        xq = window(xq, *plan["XW"], 14)
        gpre = split(project(2, lambda j, k: tie(never, x1[k], xq[j]).astype(bf16)))
        gq, GR = [], plan["GR"]
        for p in range(0, H, GR):
            for h in range(4):
                gate = _ln(_gelu2(cols(*[t[p:p + GR] for t in gpre[h]])), 4 * EPS)
                for c in range(NL):
                    t = gate[:, c * 128:(c + 1) * 128]
                    g_s[i + 1, h, c, HALO + p:HALO + p + GR, :] = t
                    if p < HALO:
                        g_s[i, h, c, HALO + H + p:HALO + H + min(p + GR, HALO), :] = t[:HALO - p]
                    if p + GR > H - HALO:
                        o = max(H - HALO - p, 0)
                        g_s[i + 2, h, c, p + o - (H - HALO):p + GR - (H - HALO), :] = t[o:]
            gq.append(g_s[i + 1, 0, 0, pl.ds(zero + HALO, 8), :])
        gq = window(gq, *plan["GW"], 7)
        q = project(0, lambda j, k: unpack(tie(never, rows(x_s[2 * k, dst, :], x_s[2 * k + 1, dst, :]),
                                               gq[j] + xq[7 + k])), plan["QO"])
        qn = beta2(transpose(split(q)))
        for k in range(25):
            qc_s[i, k] = cols(qn[2 * k], qn[min(2 * k + 1, 48)]).astype(bf16)

    def connect_quarters():
        zero = jnp.zeros((HALO, 128), f32)
        for c in range(NL):
            for h in range(4):
                g_s[nb, h, c, HALO + HL:2 * HALO + HL, :] = g_s[1, h + 1, c, HALO:2 * HALO, :] if h < 3 else zero
                g_s[1, h, c, 0:HALO, :] = g_s[nb, h - 1, c, HL:HL + HALO, :] if h else zero

    def merge_weights(b0):
        for c in late:
            c.wait()
        zero = pl.multiple_of(jnp.minimum(b0, 0), 16)
        tq = []
        for b in range(1, B):
            for p in range(0, nb * H, plan["MR"]):
                normalize(b, p, plan["MR"])
                tq.append(pltpu.bitcast(xa_s[b, 0, pl.ds(zero, 16), :128], i32))
        tq = [list(t) for t in window(tq, *plan["MW"], 12)]
        set_projection(1, wup[0].astype(f32))
        for c in range(NL):
            dw_s[c, 0:K, :] = dwv[:, c * 128:(c + 1) * 128].astype(f32) * 0.5
        tq[10].append(wp_s[1, 0, pl.ds(zero, 8), :128])

        def product(n, a, w):
            return cols(*[_dot(unpack(tie(b0 < 0, a, tq[4 * n + c])), wb[w, :, c * 128:(c + 1) * 128])
                          for c in range(4)])

        t = product(0, pltpu.bitcast(wa[0], i32), 0)
        for k, v in enumerate(beta(quadrants(product(1, pltpu.bitcast(wa[1], i32), 2)))):
            wf_s[k, D // 4:, :] = pack(v)
        tq[11].append(wf_s[0, pl.ds(zero + D // 4, 8), :128])
        for k, v in enumerate(beta(quadrants(product(2, pack(t), 1)))):
            wf_s[k, :D // 4, :] = pack(v)

    def out_copy(slot, b, r, n):
        return pltpu.make_async_copy(ob_s.at[slot, :, pl.ds(0, n), :], o_hbm.at[b, :, pl.ds(r, n), :], osem.at[slot])

    def step(b, i):
        r = pl.multiple_of(i * H, 16)
        never = i < 0
        it = b * nb + i
        slot = it % 2
        short = (i == 1) & (b > 0)
        pl.when(short)(lambda: out_copy(slot, 0, 0, HL).wait())
        pl.when((it > 1) & jnp.logical_not(short))(lambda: out_copy(slot, 0, 0, H).wait())

        CR = plan["CR"]
        todo = [(2 * r1 + h, 2 * c1 + c, p) for r1, c1 in plan["BO"]
                for h in range(2) for c in range(2) for p in range(0, H, CR)]
        conv = {}

        def conv_pieces(n):
            out = []
            for h, c, p in take(todo, n):
                w = dw_s[c]
                acc = None
                for t in sorted(range(K), key=lambda t: (t % 8, t)):
                    term = g_s[i + 1, h, c, pl.ds(p + HALO - K // 2 + t, CR), :] * w[t:t + 1, :]
                    acc = term if acc is None else acc + term
                conv[h, c, p] = acc
                out.append([acc[k:k + 8] for k in range(0, CR, 8)])
            return out

        def keys(a, c, lo, hi):
            t = 4 * a if c == 2 else 4 * a + 3 if c == 3 else 28 + 5 * a + (c if c < 2 else c - 2)
            return unpack(x_s[t // 2, lo * 64:hi * 64, (t % 2) * 128:(t % 2 + 1) * 128])

        def win(queue, w):
            return window(queue, 7 * w[0], 7 * w[1], 49)

        qc = [pltpu.bitcast(qc_s[i, k // 2], i32)[:, (k % 2) * 128:(k % 2 + 1) * 128] for k in range(49)]
        s = [[[None] * NT_ for _ in range(4)] for _ in range(4)]
        m, l, statq = [None] * 4, [None] * 4, []
        for t in range(NT_):
            st = win(statq, plan["QW"])
            cq = win(conv_pieces(plan["QC"] if t == 0 else 0), plan["QCW"])
            res = [None] * 49
            for p, k in enumerate([7 * a + c for a in plan["AO"] for c in plan["IO"]]):
                res[k] = _dot(unpack(tie(never, qc[k], st[p] + sum(cq[p], []))), keys(k // 7, k % 7, t, t + 1), NT)
            z = transpose(gamma2(res))
            for h in range(4):
                new = []
                for c in range(4):
                    v = z[h][c]
                    if (t + 1) * 128 > TQ:
                        v = jnp.where(t * 128 + lax.broadcasted_iota(i32, v.shape, 1) < TQ, v, -jnp.inf)
                    s[h][c][t] = v
                    new.append(v)
                mx = functools.reduce(jnp.maximum, new)
                tot = None
                if m[h] is not None:
                    mx = jnp.maximum(m[h], mx)
                    tot = l[h] * jnp.exp2(m[h] - mx)
                for v in new:
                    e = jnp.exp2(v - mx)
                    tot = e if tot is None else tot + e
                m[h], l[h] = mx, tot
            statq = [l[h][p:p + 8] for p in range(0, H, 8) for h in range(4)]
        shift = []
        for h in range(4):
            mr = jnp.max(m[h], axis=-1, keepdims=True)
            shift.append(mr + jnp.log2(jnp.sum(l[h] * jnp.exp2(m[h] - mr), axis=-1, keepdims=True)))

        edges = [sum(plan["VCH"][:n]) for n in range(len(plan["VCH"]) + 1)]

        def probabilities(n):
            tiles = range(edges[n], edges[n + 1])
            g = [[cols(*[jnp.exp2(s[h][c][t] - shift[h]) for t in tiles]) for c in range(4)] for h in range(4)]
            return alpha2(g), [g[h][c][p:p + 8, t * 128:(t + 1) * 128] for p in range(0, H, 8)
                               for h in range(4) for c in range(4) for t in range(len(tiles))]

        operands, pq = probabilities(0)
        st, pq = window(statq, *plan["SW"], 7), window(pq, *plan["FW"], 7)
        r2 = pl.ds(pl.multiple_of(i * H2, 8), H2)
        upre = split(project(1, lambda j, k: unpack(tie(never, rows(x_s[2 * k, r2, :], x_s[2 * k + 1, r2, :]),
                                                        st[j] + pq[j])), plan["UO"]))

        acc, uq, nv = [None] * 49, [], len(plan["VCH"])
        for n in range(nv):
            following, pq = probabilities(n + 1) if n + 1 < nv else (None, [])
            pq = win(pq, plan["PW"][n]) if n + 1 < nv else [[]] * 49
            ug = win(uq if n == plan["UJ"] else [], plan["UW"])
            cg = win(conv_pieces(plan["CJ"][n]), plan["CW"][n])
            outer = plan["PL"] if n == nv - 1 else plan["PA"]
            for p, k in enumerate([7 * a + c for a in outer for c in plan["PI"]]):
                d = _dot(tie(never, operands[k], pq[p] + ug[p] + sum(cg[p], [])).astype(bf16),
                         keys(PERM[k // 7], PERM[k % 7], edges[n], edges[n + 1]))
                acc[k] = d if acc[k] is None else acc[k] + d
                if n == 0 and p == 7 * plan["US"]:
                    started = d
            operands = following
            if n == 0:
                u = [[_gelu2(lax.select(never, started, v)) for v in row] for row in upre]
                uq = [v[p:p + 8] for row in u for v in row for p in range(0, H, 8)]

        cf = window(conv_pieces(len(todo)), *plan["FS"], 14)
        uc = [[u[h][c] * rows(*[conv[h, c, p] for p in range(0, H, CR)]) for c in range(4)] for h in range(4)]
        ao, ac = alpha(merge(gamma2(acc))), alpha(merge(uc))
        res = [None] * 7
        for n, k in enumerate(plan["FO"]):
            res[k] = _dot(tie(never, ao[k], sum(cf[n], [])).astype(bf16), unpack(wf_s[k, :D // 4, :]))
        for n, k in enumerate(plan["CO"]):
            res[k] = res[k] + _dot(tie(never, ac[k], sum(cf[7 + n], [])).astype(bf16), unpack(wf_s[k, D // 4:, :]))
        out = split(gamma(res))
        for h in range(4):
            ob_s[slot, h] = (x_v[b, h, pl.ds(r, H), :].astype(f32) + cols(*out[h])).astype(ob_s.dtype)
        pl.when(i < nb - 1)(lambda: out_copy(slot, b, r, H).start())
        pl.when(i == nb - 1)(lambda: out_copy(slot, b, r, HL).start())

    @pl.loop(0, B)
    def _(b):
        pl.loop(0, nb)(functools.partial(prepare, b))
        connect_quarters()
        pl.when(b == 0)(lambda: merge_weights(b))
        pl.loop(0, nb)(functools.partial(step, b))

    out_copy((B * nb) % 2, 0, 0, H).wait()
    out_copy((B * nb + 1) % 2, 0, 0, HL).wait()


def _call(x, w_q, w_k, w_v, w_ao, w_up, dw, w_dn, w_merge, plan):
    B, T, D = x.shape
    TQ = T // 4
    nb = -(-TQ // H)
    hbm = pl.BlockSpec(memory_space=pl.ANY)
    out = pl.pallas_call(
        functools.partial(_kernel, plan=plan),
        in_specs=[hbm] * 9,
        out_specs=hbm,
        out_shape=jax.ShapeDtypeStruct((B, 4, TQ, D), x.dtype),
        scratch_shapes=[
            pltpu.VMEM((B, 4, nb * H, D), x.dtype),
            pltpu.VMEM(w_q.shape, w_q.dtype),
            pltpu.VMEM(w_k.shape, w_k.dtype),
            pltpu.VMEM((2, D, D), w_up.dtype),
            pltpu.VMEM(dw.shape, dw.dtype),
            pltpu.VMEM((2, D, D), bf16),
            pltpu.VMEM((3, D, D), bf16),
            pltpu.VMEM((3, 7, D // 4, D // 2), i32),
            pltpu.VMEM((7, D // 2, D // 2), i32),
            pltpu.VMEM((B, 4, nb * H, D), bf16),
            pltpu.VMEM((32, 64 * sum(plan["VCH"]), D // 2), i32),
            pltpu.VMEM((nb, 32, H, D // 2), bf16),
            pltpu.VMEM((nb + 2, 4, D // 128, H + 2 * HALO, 128), f32),
            pltpu.VMEM((D // 128, 2 * HALO, 128), f32),
            pltpu.VMEM((2, 4, H, D), x.dtype),
            pltpu.SemaphoreType.DMA((10,)),
            pltpu.SemaphoreType.DMA((-(-nb // 2) + 1,)),
            pltpu.SemaphoreType.DMA((2,)),
        ],
        compiler_params=pltpu.CompilerParams(vmem_limit_bytes=112 * 1024 * 1024),
    )(x.reshape(B, 4, TQ, D), w_q, w_k, w_v, w_ao, w_up, dw, w_dn, w_merge)
    return out.reshape(B, T, D)


@jax.jit
def pallas_standalone__conformer_family_branchformer__speech_kernel(
    x: jax.Array,
    w_q: jax.Array,
    w_k: jax.Array,
    w_v: jax.Array,
    w_ao: jax.Array,
    w_up: jax.Array,
    dw: jax.Array,
    w_dn: jax.Array,
    w_merge: jax.Array,
):
    return _call(x, w_q, w_k, w_v, w_ao, w_up, dw, w_dn, w_merge, PLAN)
```
